```python
import jax
import jax.numpy as jnp

def _softmax(x, axis=-1):
    return jax.nn.softmax(x, axis=axis)

def _gelu(x):
    return jax.nn.gelu(x, approximate=True)

def _silu(x):
    return jax.nn.silu(x)

def _sigmoid(x):
    return jax.nn.sigmoid(x)

def _layernorm(x, axis=-1, eps=1e-05):
    m = jnp.mean(x, axis=axis, keepdims=True)
    v = jnp.var(x, axis=axis, keepdims=True)
    return (x - m) / jnp.sqrt(v + eps)

def _scatter_add(tgt, idx, src, axis=0):
    return tgt.at[idx].add(src)

def _segment_sum(src, seg, n):
    return jax.ops.segment_sum(src, seg, n)

class _Rng:

    def __init__(self, key):
        self._k = key

    def _next(self):
        self._k, sub = jax.random.split(self._k)
        return sub

    def normal(self, shape):
        return jax.random.normal(self._next(), shape, dtype=jnp.bfloat16)

    def randint(self, lo, hi, shape):
        return jax.random.randint(self._next(), shape, lo, hi, dtype=jnp.int32)

    def uniform(self, shape, lo=0.0, hi=1.0):
        return jax.random.uniform(self._next(), shape, jnp.bfloat16, lo, hi)

    def permutation(self, n):
        return jax.random.permutation(self._next(), n)
kernel_name = 'parallel_sum__memory_aug_recurrent_mem_tr__moe_arch_mod__prompt'

def setup_inputs():
    _rng = _Rng(jax.random.key(int.from_bytes(__import__("os").urandom(4), "little")))
    _w = lambda a: (lambda t: t.astype(jnp.bfloat16) if jnp.issubdtype(t.dtype, jnp.floating) else t)(jnp.asarray(a))

    def _A_setup():
        B, S, Dm = (1, 2048, 1024)
        H, Dh = (32, 128)
        M, seg = (8, 32)
        seg = min(seg, S)
        S = S // seg * seg
        return {'x': _w((lambda *s: _rng.normal(s) * 0.05)(B, S, Dm)), 'mem0': _w((lambda *s: _rng.normal(s) * 0.05)(B, M, Dm)), 'Wq': _w((lambda *s: _rng.normal(s) * 0.05)(Dm, H, Dh) * Dm ** (-0.5)), 'Wk': _w((lambda *s: _rng.normal(s) * 0.05)(Dm, H, Dh) * Dm ** (-0.5)), 'Wv': _w((lambda *s: _rng.normal(s) * 0.05)(Dm, H, Dh) * Dm ** (-0.5)), 'Wo': _w((lambda *s: _rng.normal(s) * 0.05)(H, Dh, Dm) * (H * Dh) ** (-0.5)), 'seg_len': seg}
    _A_in = _A_setup()

    def _B_setup():
        B, S, D, F, C = (1, 2048, 1024, 3584, 2)
        return {'x': _w((lambda *s: _rng.normal(s) * 0.05)(B, S, D)), 'w_r': _w((lambda *s: _rng.normal(s) * 0.05)(D)), 'w_gate': _w((lambda *s: _rng.normal(s) * 0.05)(D, F)), 'w_up': _w((lambda *s: _rng.normal(s) * 0.05)(D, F)), 'w_down': _w((lambda *s: _rng.normal(s) * 0.05)(F, D))}
    _B_in = _B_setup()
    return {'A_x': _A_in['x'], 'A_mem0': _A_in['mem0'], 'A_Wq': _A_in['Wq'], 'A_Wk': _A_in['Wk'], 'A_Wv': _A_in['Wv'], 'A_Wo': _A_in['Wo'], 'A_seg_len': _A_in['seg_len'], 'B_x': _B_in['x'], 'B_w_r': _B_in['w_r'], 'B_w_gate': _B_in['w_gate'], 'B_w_up': _B_in['w_up'], 'B_w_down': _B_in['w_down']}

def reference(A_x, A_mem0, A_Wq, A_Wk, A_Wv, A_Wo, A_seg_len, B_x, B_w_r, B_w_gate, B_w_up, B_w_down):

    def _A_ref(x, mem0, Wq, Wk, Wv, Wo, seg_len):
        B, S, Dm = x.shape
        H, Dh = (Wq.shape[1], Wq.shape[2])
        M = mem0.shape[1]
        scale = Dh ** (-0.5)
        n_seg = S // seg_len
        L = M + seg_len
        idx = jnp.arange(L)
        mask = (idx[:, None] < M) | (idx[:, None] >= idx[None, :])
        mem = mem0
        outs = []
        for s in range(n_seg):
            xs = x[:, s * seg_len:(s + 1) * seg_len, :].copy()
            h = jnp.concatenate([mem, xs], axis=1)
            q = jnp.einsum('btd,dhe->bhte', h, Wq)
            k = jnp.einsum('btd,dhe->bhte', h, Wk)
            v = jnp.einsum('btd,dhe->bhte', h, Wv)
            scores = jnp.einsum('bhqe,bhke->bhqk', q, k) * scale
            scores = jnp.where(mask[None, None], scores, -1000000000.0)
            p = _softmax(scores, axis=-1)
            o = jnp.einsum('bhqk,bhke->bhqe', p, v)
            o = jnp.einsum('bhte,hed->btd', o, Wo)
            mem = o[:, :M, :].copy()
            outs.append(o[:, M:, :])
        return jnp.concatenate(outs, axis=1)

    def _B_ref(x, w_r, w_gate, w_up, w_down):
        B, S, D = x.shape
        C = 2
        r = x @ w_r
        idx = jnp.argsort(-r, axis=-1)[:, :C]
        idx_e = jnp.repeat(idx.reshape(B, C, 1), D, axis=2)
        x_sel = jnp.take_along_axis(x, idx_e, axis=1)
        g = _silu(x_sel @ w_gate)
        u = x_sel @ w_up
        y = g * u @ w_down
        r_sel = _sigmoid(jnp.take_along_axis(r, idx, axis=1))
        y = y * r_sel.reshape(B, C, 1)
        b_off = (jnp.arange(B) * S).reshape(B, 1)
        flat_idx = (idx + b_off).reshape(B * C)
        zero = (x * 0.0).reshape(B * S, D)
        upd = _scatter_add(zero, flat_idx, y.reshape(B * C, D), axis=0)
        return x + upd.reshape(B, S, D)
    x = A_x
    xn = _layernorm(x, axis=-1)
    return x + _A_ref(xn, A_mem0, A_Wq, A_Wk, A_Wv, A_Wo, A_seg_len) + _B_ref(xn, B_w_r, B_w_gate, B_w_up, B_w_down)
```

```python
import jax
import jax.numpy as jnp
from jax import lax
import jax.experimental.pallas as pl
import jax.experimental.pallas.tpu as pltpu

bf16 = jnp.bfloat16
f32 = jnp.float32
u32 = jnp.uint32

S, DM, H, DH, NMEM, SEG, FF = 2048, 1024, 32, 128, 8, 32, 3584
NSEG = S // SEG
TOK = 24
PRE = S - NSEG * TOK
RQ = 544
RO = 768
NG = 4
KT = DM // 128
FT = FF // 128
L2 = 2 * (SEG + NMEM)
SCALE = DH ** -0.5
EPS_BF16 = 1.0013580322265625e-05

SEM_W0, SEM_W1, SEM_XA, SEM_XB, SEM_XC, SEM_WO, SEM_WG, SEM_WU, SEM_WD, SEM_OUT, SEM_P0, SEM_P1, SEM_OUT2 = range(13)
XA_ROWS, XB_ROWS = 640, 384


def _as_bf16(x):
    return pltpu.bitcast(x, bf16)


def _as_u32(x):
    return pltpu.bitcast(x, u32)


def _rnd(x):
    return x.astype(bf16).astype(f32)


def _dot(a, b):
    return jnp.dot(a, b, preferred_element_type=f32)


def _head(g, c, hh):
    return 8 * c + 2 * g + hh


def _kernel(x_hbm, mem0_ref, wq_hbm, wk_hbm, wv_hbm, wo_hbm, wr_ref, wg_hbm, wu_hbm, wd_hbm,
            out_hbm,
            x_scr, xn_scr, xpn_scr, lhs_pre, stage, wqkv, wo,
            qr0, qr1, qr2, qr3, or0, or1, or2, or3, lo0, lo1, lo2, lo3,
            mem_scr, fill_scr, racc, wg, wu, wd, out_stage, sems):
    qrings = (qr0, qr1, qr2, qr3)
    orings = (or0, or1, or2, or3)
    lhs_os = (lo0, lo1, lo2, lo3)
    w32 = [w.bitcast(u32) for w in (wq_hbm, wk_hbm, wv_hbm)]
    wo32 = wo_hbm.bitcast(u32)
    wg32 = wg_hbm.bitcast(u32)
    wu32 = wu_hbm.bitcast(u32)
    wd32 = wd_hbm.bitcast(u32)

    def x_copy(r0, n, sem):
        return pltpu.make_async_copy(x_hbm.at[0, pl.ds(r0, n)], x_scr.at[pl.ds(r0, n)], sems.at[sem])

    def w_copy(k):
        return pltpu.make_async_copy(w32[k // 2].at[:, pl.ds(8 * (k % 2), 8), :], stage.at[k % 2],
                                     sems.at[SEM_W0 + k % 2])

    def col_tiles_start(src, dst, sem, lo, hi):
        for j in range(lo, hi):
            pltpu.make_async_copy(src.at[:, pl.ds(128 * j, 128)], dst.at[j], sems.at[sem]).start()

    def wait_all(buf, sem):
        pltpu.make_async_copy(buf, buf, sems.at[sem]).wait()

    x_copy(0, XA_ROWS, SEM_XA).start()
    w_copy(0).start()

    mem_scr[...] = mem0_ref[0].astype(f32)
    racc[...] = jnp.full(racc.shape, -jnp.inf, f32)
    qi = lax.broadcasted_iota(jnp.int32, (L2, L2), 0)
    ki = lax.broadcasted_iota(jnp.int32, (L2, L2), 1)
    q_mem, k_mem = qi >= 2 * SEG, ki >= 2 * SEG
    q_head = jnp.where(q_mem, (qi - 2 * SEG) // NMEM, qi // SEG)
    k_head = jnp.where(k_mem, (ki - 2 * SEG) // NMEM, ki // SEG)
    visible = q_mem | k_mem | (qi >= ki)
    fill_scr[...] = jnp.where(q_head == k_head, jnp.where(visible, 0.0, -1e9), -jnp.inf).astype(f32)

    def ln_chunk(c, to_lhs):
        wr = wr_ref[...].astype(f32).reshape(1, DM)
        lane = lax.broadcasted_iota(jnp.int32, (16, 128), 1)
        for i in range(8):
            r0 = pl.multiple_of(c * 128 + 16 * i, 16)
            x = x_scr[pl.ds(r0, 16), :].astype(f32)
            mean = jnp.sum(x, axis=-1, keepdims=True) * (1.0 / DM)
            xc = x - mean
            var = jnp.sum(xc * xc, axis=-1, keepdims=True) * (1.0 / DM)
            den = _rnd(jnp.sqrt(_rnd(_rnd(var) + EPS_BF16)))
            xnb = (_rnd(x - _rnd(mean)) * (1.0 / den)).astype(bf16)
            xn = xnb.astype(f32)
            xn_scr[pl.ds(r0, 16), :] = xn
            xpn_scr[pl.ds(r0, 16), :] = x + xn
            r = _rnd(jnp.sum(xn * wr, axis=-1, keepdims=True))
            racc[16 * i:16 * i + 16, :] = jnp.where(lane == c, r, racc[16 * i:16 * i + 16, :])
            if to_lhs:
                p0 = pl.multiple_of(c * 64 + 8 * i, 8)
                for k in range(KT):
                    lhs_pre[k, pl.ds(p0, 8), :] = _as_u32(xnb[:, 128 * k:128 * (k + 1)])

    x_copy(0, XA_ROWS, SEM_XA).wait()

    def ln_first(c, carry):
        ln_chunk(c, True)
        return carry
    lax.fori_loop(0, PRE // 128, ln_first, 0)

    stage2d = stage.reshape(2 * DM * 8, 128)

    def pro_body(t, carry):
        m = t // 4
        c8 = t % 4
        slot = (t // 2) % 2

        for k in range(6):
            @pl.when(t == 2 * k)
            def _():
                w_copy(k).wait()
                if k + 1 < 6:
                    w_copy(k + 1).start()
                if k == 0:
                    x_copy(XA_ROWS, XB_ROWS, SEM_XB).start()
                if k == 1:
                    col_tiles_start(wo32, wo, SEM_WO, 0, 4)
                if k == 2:
                    x_copy(XA_ROWS + XB_ROWS, S - XA_ROWS - XB_ROWS, SEM_XC).wait()
                    col_tiles_start(wo32, wo, SEM_WO, 4, 8)
                if k == 5:
                    col_tiles_start(wg32, wg, SEM_WG, 0, FT)
                    col_tiles_start(wu32, wu, SEM_WU, 0, FT)
                    col_tiles_start(wd32, wd, SEM_WD, 0, KT)

        @pl.when(t == 1)
        def _():
            x_copy(XA_ROWS, XB_ROWS, SEM_XB).wait()
            x_copy(XA_ROWS + XB_ROWS, S - XA_ROWS - XB_ROWS, SEM_XC).start()

        sc = jnp.where(m == 0, SCALE, 1.0).astype(f32)
        for g in range(NG):
            base = slot * (DM * 8) + 4 * (t % 2) + g
            a = stage2d[pl.ds(base, DM // 2, stride=16), :]
            b = stage2d[pl.ds(base + 8, DM // 2, stride=16), :]
            pair = ((a & jnp.uint32(0xFFFF)) | (b << 16), (a >> 16) | (b & jnp.uint32(0xFFFF0000)))
            for hh in range(2):
                wqkv[_head(g, c8, hh) * 3 + m] = pair[hh]
                lhs = jnp.concatenate([_as_bf16(lhs_pre[k]) for k in range(KT)], axis=1)
                y = _dot(lhs, _as_bf16(pair[hh])) * sc
                qrings[g][(2 * c8 + hh) * 3 + m, 0:PRE // 2, :] = _as_u32(y.astype(bf16))
            if g == 0:
                ln_chunk(PRE // 128 + t, False)
        return carry
    lax.fori_loop(0, 12, pro_body, 0)
    wait_all(wo, SEM_WO)

    def step(s, carry):
        xrow = pl.multiple_of(PRE + TOK * s, 8)
        wr_pos = [pl.multiple_of(lax.rem(PRE + TOK * s + 8 * i, RQ) // 2, 4) for i in range(3)]
        rd = pl.multiple_of(lax.rem(SEG * s, RQ) // 2, 16)
        owr = pl.multiple_of(lax.rem(SEG * s, RO) // 2, 16)
        ord_ = pl.multiple_of(lax.rem(TOK * s, RO) // 2, 4)
        orow = pl.multiple_of(TOK * s, 8)
        lhs = jnp.concatenate([xn_scr[pl.ds(xrow, TOK), :], mem_scr[...]], axis=0).astype(bf16)

        mem_parts, probs, acc = {}, {}, []

        def qkv(g, c):
            res = []
            for m in range(3):
                ms = []
                for hh in range(2):
                    y = _dot(lhs, _as_bf16(wqkv[_head(g, c, hh) * 3 + m]))
                    if m == 0:
                        y = y * SCALE
                    yp = _as_u32(y.astype(bf16))
                    for i in range(3):
                        qrings[g][(2 * c + hh) * 3 + m, pl.ds(wr_pos[i], 4), :] = yp[4 * i:4 * i + 4]
                    ms.append(y[TOK:])
                res.append(jnp.concatenate(ms, axis=0).astype(bf16))
            mem_parts[g, c] = res

        def pair_rows(g, c, m, mem_rows):
            t0 = _as_bf16(qrings[g][(2 * c) * 3 + m, pl.ds(rd, SEG // 2), :])
            t1 = _as_bf16(qrings[g][(2 * c + 1) * 3 + m, pl.ds(rd, SEG // 2), :])
            return jnp.concatenate([t0, t1, mem_rows], axis=0)

        def scores(g, c):
            qm, km, vm = mem_parts.pop((g, c))
            sc = lax.dot_general(pair_rows(g, c, 0, qm), pair_rows(g, c, 1, km),
                                 (((1,), (1,)), ((), ())), preferred_element_type=f32)
            fill = fill_scr[...]
            sc = jnp.where(fill == 0.0, sc, fill)
            e = jnp.exp(sc - jnp.max(sc, axis=-1, keepdims=True))
            den = jnp.sum(e, axis=-1, keepdims=True)
            r = pl.reciprocal(den, approx=True)
            r = r * (2.0 - den * r)
            probs[g, c] = (e.astype(bf16), r, vm)

        def pv(g, c):
            e, r, vm = probs.pop((g, c))
            o = _dot(e, pair_rows(g, c, 2, vm)) * r
            for hh in range(2):
                h = 2 * c + hh
                orings[g][h, pl.ds(owr, SEG // 2), :] = _as_u32(o[SEG * hh:SEG * (hh + 1)].astype(bf16))
                tok = _as_bf16(orings[g][h, pl.ds(ord_, TOK // 2), :])
                om = o[2 * SEG + NMEM * hh:2 * SEG + NMEM * (hh + 1)]
                last = jnp.concatenate([tok[16:TOK].astype(f32), om], axis=0).astype(bf16)
                lhs_os[g][h] = _as_u32(jnp.concatenate([tok[0:16], last], axis=0))

        def out_proj(g):
            cols = []
            for j in range(KT):
                l = jnp.concatenate([_as_bf16(lhs_os[g][k]) for k in range(8)], axis=1)
                w = jnp.concatenate(
                    [_as_bf16(wo[j, 64 * _head(g, c, 0):64 * _head(g, c, 0) + 128, :]) for c in range(4)], axis=0)
                cols.append(_dot(l, w))
            a = jnp.concatenate(cols, axis=1)
            acc[:] = [a if not acc else acc[0] + a]

        for item in "q0 q1 s0 q2 s1 p0 q3 s2 p1 w0 s3 p2 w1 p3 w2 w3".split():
            g = int(item[1])
            if item[0] == "w":
                out_proj(g)
            else:
                for c in range(4):
                    {"q": qkv, "s": scores, "p": pv}[item[0]](g, c)
        a = acc[0]
        mem_scr[...] = _rnd(a[TOK:])
        out_stage[pl.ds(orow, TOK), :] = (a[:TOK] + xpn_scr[pl.ds(orow, TOK), :]).astype(bf16)
        pltpu.make_async_copy(out_stage.at[pl.ds(orow, TOK)], out_hbm.at[0, pl.ds(orow, TOK)],
                              sems.at[SEM_OUT]).start()
        return carry
    lax.fori_loop(0, NSEG, step, 0)

    rv = racc[...]
    ridx = (lax.broadcasted_iota(jnp.int32, rv.shape, 0)
            + 128 * lax.broadcasted_iota(jnp.int32, rv.shape, 1)).astype(f32)
    m0 = jnp.max(rv)
    f0 = jnp.min(jnp.where(rv == m0, ridx, 1e9))
    rv2 = jnp.where(ridx == f0, -jnp.inf, rv)
    m1 = jnp.max(rv2)
    f1 = jnp.min(jnp.where(rv2 == m1, ridx, 1e9))
    i0 = jnp.clip(f0.astype(jnp.int32), 0, S - 1)
    i1 = jnp.clip(f1.astype(jnp.int32), 0, S - 1)
    row16 = lax.broadcasted_iota(jnp.int32, (16, DM), 0)
    xsel = jnp.where(row16 == 0, xn_scr[pl.ds(i0, 1), :],
                     jnp.where(row16 == 1, xn_scr[pl.ds(i1, 1), :], 0.0)).astype(bf16)
    wait_all(wg, SEM_WG)
    wait_all(wu, SEM_WU)
    wait_all(wd, SEM_WD)
    hs = []
    for j in range(FT):
        gate = _dot(xsel, _as_bf16(wg[j]))
        up = _dot(xsel, _as_bf16(wu[j]))
        hs.append((gate * jax.nn.sigmoid(gate) * up).astype(bf16))
    hid = jnp.concatenate(hs, axis=1)
    y = jnp.concatenate([_dot(hid, _as_bf16(wd[j])) for j in range(KT)], axis=1)
    rsel = jnp.where(lax.broadcasted_iota(jnp.int32, (16, 1), 0) == 0, m0, m1)
    y = y * jax.nn.sigmoid(rsel)
    y0, y1 = y[0:1], y[1:2]

    xpn_scr[pl.ds(i0, 1), :] = xpn_scr[pl.ds(i0, 1), :] + y0
    xpn_scr[pl.ds(i1, 1), :] = xpn_scr[pl.ds(i1, 1), :] + y1
    done = NSEG * TOK
    wait_all(out_stage.at[pl.ds(0, done)], SEM_OUT)
    g0 = pl.multiple_of((i0 // 16) * 16, 16)
    g1 = pl.multiple_of((i1 // 16) * 16, 16)
    redo0 = i0 < done
    redo1 = i1 < done
    send1 = jnp.logical_and(redo1, g1 != g0)

    def patch(i, gst, yy):
        blk = out_stage[pl.ds(gst, 16), :].astype(f32)
        out_stage[pl.ds(gst, 16), :] = (blk + jnp.where(row16 == i - gst, yy, 0.0)).astype(bf16)

    def patch_copy(gst, sem):
        return pltpu.make_async_copy(out_stage.at[pl.ds(gst, 16)], out_hbm.at[0, pl.ds(gst, 16)], sems.at[sem])

    @pl.when(redo0)
    def _():
        patch(i0, g0, y0)

    @pl.when(redo1)
    def _():
        patch(i1, g1, y1)

    @pl.when(redo0)
    def _():
        patch_copy(g0, SEM_P0).start()

    @pl.when(send1)
    def _():
        patch_copy(g1, SEM_P1).start()

    def epi_body(b, carry):
        pos = pl.multiple_of(64 * b, 64)
        r0 = pl.multiple_of(done + 128 * b, 128)
        for j in range(KT):
            l = jnp.concatenate(
                [_as_bf16(orings[(h % 8) // 2][2 * (h // 8) + h % 2, pl.ds(pos, 64), :]) for h in range(H)], axis=1)
            a = _dot(l, _as_bf16(wo[j]))
            cs = slice(128 * j, 128 * (j + 1))
            out_stage[pl.ds(r0, 128), cs] = (a + xpn_scr[pl.ds(r0, 128), cs]).astype(bf16)
        pltpu.make_async_copy(out_stage.at[pl.ds(r0, 128)], out_hbm.at[0, pl.ds(r0, 128)],
                              sems.at[SEM_OUT2]).start()
        return carry
    lax.fori_loop(0, PRE // 128, epi_body, 0)

    wait_all(out_stage.at[pl.ds(done, PRE)], SEM_OUT2)

    @pl.when(redo0)
    def _():
        patch_copy(g0, SEM_P0).wait()

    @pl.when(send1)
    def _():
        patch_copy(g1, SEM_P1).wait()


@jax.jit
def pallas_parallel_sum__memory_aug_recurrent_mem_tr__moe_arch_mod__prompt_kernel(
    A_x: jax.Array,
    A_mem0: jax.Array,
    A_Wq: jax.Array,
    A_Wk: jax.Array,
    A_Wv: jax.Array,
    A_Wo: jax.Array,
    A_seg_len: jax.Array,
    B_x: jax.Array,
    B_w_r: jax.Array,
    B_w_gate: jax.Array,
    B_w_up: jax.Array,
    B_w_down: jax.Array,
):
    del A_seg_len, B_x
    assert A_x.shape == (1, S, DM) and A_mem0.shape == (1, NMEM, DM)
    assert A_Wq.shape == (DM, H, DH) and A_Wo.shape == (H, DH, DM) and B_w_gate.shape == (DM, FF)
    hbm = pl.BlockSpec(memory_space=pl.ANY)
    vmem = pl.BlockSpec(memory_space=pltpu.VMEM)
    scratch = [
        pltpu.VMEM((S, DM), bf16),
        pltpu.VMEM((S, DM), f32),
        pltpu.VMEM((S, DM), f32),
        pltpu.VMEM((KT, PRE // 2, 128), u32),
        pltpu.VMEM((2, DM, 8, 128), u32),
        pltpu.VMEM((3 * H, DM // 2, 128), u32),
        pltpu.VMEM((KT, H * DH // 2, 128), u32),
    ]
    scratch += [pltpu.VMEM((24, RQ // 2, 128), u32)] * NG
    scratch += [pltpu.VMEM((8, RO // 2, 128), u32)] * NG
    scratch += [pltpu.VMEM((8, 16, 128), u32)] * NG
    scratch += [
        pltpu.VMEM((NMEM, DM), f32),
        pltpu.VMEM((L2, L2), f32),
        pltpu.VMEM((128, 128), f32),
        pltpu.VMEM((FT, DM // 2, 128), u32),
        pltpu.VMEM((FT, DM // 2, 128), u32),
        pltpu.VMEM((KT, FF // 2, 128), u32),
        pltpu.VMEM((S, DM), bf16),
        pltpu.SemaphoreType.DMA((13,)),
    ]
    return pl.pallas_call(
        _kernel,
        out_shape=jax.ShapeDtypeStruct((1, S, DM), bf16),
        in_specs=[hbm, vmem, hbm, hbm, hbm, hbm, vmem, hbm, hbm, hbm],
        out_specs=hbm,
        scratch_shapes=scratch,
        compiler_params=pltpu.CompilerParams(vmem_limit_bytes=124 * 1024 * 1024),
    )(A_x, A_mem0, A_Wq, A_Wk, A_Wv, A_Wo.reshape(H * DH, DM), B_w_r, B_w_gate, B_w_up, B_w_down)
```

```python
import jax
import jax.numpy as jnp
from jax import lax
import jax.experimental.pallas as pl
import jax.experimental.pallas.tpu as pltpu

bf16 = jnp.bfloat16
f32 = jnp.float32
u32 = jnp.uint32

S, DM, H, DH, NMEM, SEG, FF = 2048, 1024, 32, 128, 8, 32, 3584
NSEG = S // SEG
TOK = 24
PRE = S - NSEG * TOK
RQ = 544
RO = 768
NG = 4
KT = DM // 128
FT = FF // 128
L2 = 2 * (SEG + NMEM)
SCALE = DH ** -0.5
EPS_BF16 = 1.0013580322265625e-05

NSLOT = 6
SEM_W0 = 0
SEM_X0 = NSLOT
SEM_XB, SEM_XC, SEM_WO, SEM_WG, SEM_WU, SEM_WD, SEM_OUT, SEM_P0, SEM_P1, SEM_OUT2 = range(NSLOT + 4, NSLOT + 14)
NSEM = NSLOT + 14
XB_ROWS = 384


def _as_bf16(x):
    return pltpu.bitcast(x, bf16)


def _as_u32(x):
    return pltpu.bitcast(x, u32)


def _rnd(x):
    return x.astype(bf16).astype(f32)


def _dot(a, b):
    return jnp.dot(a, b, preferred_element_type=f32)


def _head(g, c, hh):
    return 8 * c + 2 * g + hh


def _kernel(x_hbm, mem0_ref, wq_hbm, wk_hbm, wv_hbm, wo_hbm, wr_ref, wg_hbm, wu_hbm, wd_hbm,
            out_hbm,
            x_scr, xn_scr, xpn_scr, lhs_pre, stage, wqkv, wo,
            qr0, qr1, qr2, qr3, or0, or1, or2, or3, lo0, lo1, lo2, lo3,
            mem_scr, fill_scr, racc, wg, wu, wd, out_stage, sems):
    qrings = (qr0, qr1, qr2, qr3)
    orings = (or0, or1, or2, or3)
    lhs_os = (lo0, lo1, lo2, lo3)
    w32 = [w.bitcast(u32) for w in (wq_hbm, wk_hbm, wv_hbm)]
    wo32 = wo_hbm.bitcast(u32)
    wg32 = wg_hbm.bitcast(u32)
    wu32 = wu_hbm.bitcast(u32)
    wd32 = wd_hbm.bitcast(u32)

    def x_copy(r0, n, sem):
        return pltpu.make_async_copy(x_hbm.at[0, pl.ds(r0, n)], x_scr.at[pl.ds(r0, n)], sems.at[sem])

    def w_copy(t, lo, n, sem, e):
        return pltpu.make_async_copy(w32[t // 4].at[:, e, pl.ds(4 * (t % 4) + lo, n), :],
                                     stage.at[t % 4, :, pl.ds(4 * e + lo, n), :], sems.at[SEM_W0 + sem])

    def w_start(t, lo=0, n=4, sem=None):
        for e in range(2):
            w_copy(t, lo, n, t % 4 if sem is None else sem, e).start()

    def w_wait(t, lo=0, n=4, sem=None):
        for e in range(2):
            w_copy(t, lo, n, t % 4 if sem is None else sem, e).wait()

    def col_tiles_start(src, dst, sem, lo, hi):
        for j in range(lo, hi):
            pltpu.make_async_copy(src.at[:, pl.ds(128 * j, 128)], dst.at[j], sems.at[sem]).start()

    def wait_all(buf, sem):
        pltpu.make_async_copy(buf, buf, sems.at[sem]).wait()

    for c in range(4):
        x_copy(128 * c, 128, SEM_X0 + c).start()
    w_start(0, 0, 2, 4)
    w_start(0, 2, 2, 5)

    mem_scr[...] = mem0_ref[0].astype(f32)
    racc[...] = jnp.full(racc.shape, -jnp.inf, f32)
    qi = lax.broadcasted_iota(jnp.int32, (L2, L2), 0)
    ki = lax.broadcasted_iota(jnp.int32, (L2, L2), 1)
    q_mem, k_mem = qi >= 2 * SEG, ki >= 2 * SEG
    q_head = jnp.where(q_mem, (qi - 2 * SEG) // NMEM, qi // SEG)
    k_head = jnp.where(k_mem, (ki - 2 * SEG) // NMEM, ki // SEG)
    visible = q_mem | k_mem | (qi >= ki)
    fill_scr[...] = jnp.where(q_head == k_head, jnp.where(visible, 0.0, -1e9), -jnp.inf).astype(f32)

    def ln_rows(r0, n, racc_row, lane_id):
        wr = wr_ref[...].astype(f32).reshape(1, DM)
        lane = lax.broadcasted_iota(jnp.int32, (n, 128), 1)
        x = x_scr[pl.ds(r0, n), :].astype(f32)
        mean = jnp.sum(x, axis=-1, keepdims=True) * (1.0 / DM)
        xc = x - mean
        var = jnp.sum(xc * xc, axis=-1, keepdims=True) * (1.0 / DM)
        den = _rnd(jnp.sqrt(_rnd(_rnd(var) + EPS_BF16)))
        xnb = (_rnd(x - _rnd(mean)) * (1.0 / den)).astype(bf16)
        xn = xnb.astype(f32)
        xn_scr[pl.ds(r0, n), :] = xn
        xpn_scr[pl.ds(r0, n), :] = x + xn
        r = _rnd(jnp.sum(xn * wr, axis=-1, keepdims=True))
        racc[racc_row:racc_row + n, :] = jnp.where(lane == lane_id, r, racc[racc_row:racc_row + n, :])
        return xnb

    def ln_chunk(c):
        for i in range(8):
            xnb = ln_rows(pl.multiple_of(c * 128 + 16 * i, 16), 16, 16 * i, c)
            p0 = pl.multiple_of(c * 64 + 8 * i, 8)
            for k in range(KT):
                lhs_pre[k, pl.ds(p0, 8), :] = _as_u32(xnb[:, 128 * k:128 * (k + 1)])

    def ln_first(c, carry):
        r0 = pl.multiple_of(128 * c, 128)
        pltpu.make_async_copy(x_hbm.at[0, pl.ds(r0, 128)], x_scr.at[pl.ds(r0, 128)], sems.at[SEM_X0 + c]).wait()
        ln_chunk(c)
        return carry
    with jax.named_scope("ln_first"):
        lax.fori_loop(0, PRE // 128, ln_first, 0)

    stage2d = stage.reshape(4 * DM * 4, 128)

    def pro_pairs(t, gs):
        m, c8 = t // 4, t % 4
        sc = (SCALE if m == 0 else None) if isinstance(t, int) else jnp.where(m == 0, SCALE, 1.0).astype(f32)
        for g in gs:
            both = stage2d[pl.ds(c8 * (DM * 4) + g, DM, stride=4), :]
            pair = (pltpu.bitcast(both << 16, f32).astype(bf16),
                    pltpu.bitcast(both & jnp.uint32(0xFFFF0000), f32).astype(bf16))
            for hh in range(2):
                wqkv[_head(g, c8, hh) * 3 + m] = _as_u32(pair[hh])
                lhs = jnp.concatenate([_as_bf16(lhs_pre[k]) for k in range(KT)], axis=1)
                y = _dot(lhs, pair[hh])
                if sc is not None:
                    y = y * sc
                qrings[g][(2 * c8 + hh) * 3 + m, 0:PRE // 2, :] = _as_u32(y.astype(bf16))

    with jax.named_scope("pro_a"):
        w_start(1)
        w_wait(0, 0, 2, 4)
        pro_pairs(0, (0, 1))
    with jax.named_scope("pro_b"):
        w_start(2)
        w_start(3)
        w_wait(0, 2, 2, 5)
        pro_pairs(0, (2, 3))
    with jax.named_scope("pro_c"):
        w_wait(1)
        pro_pairs(1, range(NG))

    def pro_body(i, carry):
        for k in range(5):
            @pl.when(i == k)
            def _():
                w_wait(2 + 2 * k)
                w_wait(3 + 2 * k)
                if k < 4:
                    w_start(4 + 2 * k)
                    w_start(5 + 2 * k)
                if k == 0:
                    x_copy(PRE, S - PRE, SEM_XB).start()
                if k in (1, 2):
                    col_tiles_start(wo32, wo, SEM_WO, 4 * (k - 1), 4 * k)
                if k == 4:
                    col_tiles_start(wg32, wg, SEM_WG, 0, FT)
                    col_tiles_start(wu32, wu, SEM_WU, 0, FT)
                    col_tiles_start(wd32, wd, SEM_WD, 0, KT)
        pro_pairs(2 + 2 * i, range(NG))
        pro_pairs(3 + 2 * i, range(NG))
        return carry
    with jax.named_scope("prologue"):
        lax.fori_loop(0, 5, pro_body, 0)
    with jax.named_scope("wait_wo"):
        wait_all(wo, SEM_WO)
        x_copy(PRE, S - PRE, SEM_XB).wait()
    ln_rows(PRE, TOK, 128, 0)

    def step(s, mem_in):
        xrow = pl.multiple_of(PRE + TOK * s, 8)
        wr_pos = [pl.multiple_of(lax.rem(PRE + TOK * s + 8 * i, RQ) // 2, 4) for i in range(3)]
        rd = pl.multiple_of(lax.rem(SEG * s, RQ) // 2, 16)
        owr = pl.multiple_of(lax.rem(SEG * s, RO) // 2, 16)
        ord_ = pl.multiple_of(lax.rem(TOK * s, RO) // 2, 4)
        orow = pl.multiple_of(TOK * s, 8)
        lhs = jnp.concatenate([xn_scr[pl.ds(xrow, TOK), :], mem_in], axis=0).astype(bf16)

        mem_parts, probs = {}, {}

        def qkv(g, c):
            res = []
            for m in range(3):
                ms = []
                for hh in range(2):
                    y = _dot(lhs, _as_bf16(wqkv[_head(g, c, hh) * 3 + m]))
                    if m == 0:
                        y = y * SCALE
                    yp = _as_u32(y.astype(bf16))
                    for i in range(3):
                        qrings[g][(2 * c + hh) * 3 + m, pl.ds(wr_pos[i], 4), :] = yp[4 * i:4 * i + 4]
                    ms.append(y[TOK:])
                res.append(jnp.concatenate(ms, axis=0).astype(bf16))
            mem_parts[g, c] = res

        def pair_rows(g, c, m, mem_rows):
            t0 = _as_bf16(qrings[g][(2 * c) * 3 + m, pl.ds(rd, SEG // 2), :])
            t1 = _as_bf16(qrings[g][(2 * c + 1) * 3 + m, pl.ds(rd, SEG // 2), :])
            return jnp.concatenate([t0, t1, mem_rows], axis=0)

        def scores(g, c):
            qm, km, vm = mem_parts.pop((g, c))
            sc = lax.dot_general(pair_rows(g, c, 0, qm), pair_rows(g, c, 1, km),
                                 (((1,), (1,)), ((), ())), preferred_element_type=f32)
            fill = fill_scr[...]
            sc = jnp.where(fill == 0.0, sc, fill)
            e = jnp.exp(sc - jnp.max(sc, axis=-1, keepdims=True))
            den = jnp.sum(e, axis=-1, keepdims=True)
            r = pl.reciprocal(den, approx=True)
            r = r * (2.0 - den * r)
            probs[g, c] = (e.astype(bf16), r, vm)

        def pv(g, c):
            e, r, vm = probs.pop((g, c))
            o = _dot(e, pair_rows(g, c, 2, vm)) * r
            for hh in range(2):
                h = 2 * c + hh
                orings[g][h, pl.ds(owr, SEG // 2), :] = _as_u32(o[SEG * hh:SEG * (hh + 1)].astype(bf16))
                tok = _as_bf16(orings[g][h, pl.ds(ord_, TOK // 2), :])
                om = o[2 * SEG + NMEM * hh:2 * SEG + NMEM * (hh + 1)]
                last = jnp.concatenate([tok[16:TOK].astype(f32), om], axis=0).astype(bf16)
                lhs_os[g][h] = _as_u32(jnp.concatenate([tok[0:16], last], axis=0))

        acc = [None] * KT

        def out_proj(g, js):
            for j in js:
                l = jnp.concatenate([_as_bf16(lhs_os[g][k]) for k in range(8)], axis=1)
                w = jnp.concatenate(
                    [_as_bf16(wo[j, 64 * _head(g, c, 0):64 * _head(g, c, 0) + 128, :]) for c in range(4)], axis=0)
                a = _dot(l, w)
                if acc[j] is None:
                    cs = slice(128 * j, 128 * (j + 1))
                    acc[j] = a + jnp.concatenate([xpn_scr[pl.ds(orow, TOK), cs], jnp.zeros((NMEM, 128), f32)], axis=0)
                else:
                    acc[j] = acc[j] + a

        for item in "q0 q1 s0 q2 p0 s1 q3 p1 s2 w0 L0 p2 s3 w1 w2a p3 w2b w3".split():
            g = int(item[1])
            if item[0] == "w":
                out_proj(g, {"": range(8), "a": range(4), "b": range(4, 8)}[item[2:]])
            elif item[0] == "L":
                nxt = jnp.minimum(s + 1, NSEG - 1)
                ln_rows(pl.multiple_of(PRE + TOK * nxt, 8), TOK, 128, nxt)
            else:
                for c in range(4):
                    {"q": qkv, "s": scores, "p": pv}[item[0]](g, c)
        a = jnp.concatenate(acc, axis=1)
        out_stage[pl.ds(orow, TOK), :] = a[:TOK].astype(bf16)
        return _rnd(a[TOK:])

    def body(s, carry):
        mem_scr[...] = step(s, mem_scr[...])
        orow = pl.multiple_of(TOK * s, 8)
        pltpu.make_async_copy(out_stage.at[pl.ds(orow, TOK)], out_hbm.at[0, pl.ds(orow, TOK)],
                              sems.at[SEM_OUT]).start()
        return carry
    with jax.named_scope("chain"):
        lax.fori_loop(0, NSEG, body, 0)

    rv = racc[...]
    rrow = lax.broadcasted_iota(jnp.int32, rv.shape, 0)
    rlane = lax.broadcasted_iota(jnp.int32, rv.shape, 1)
    ridx = jnp.where(rrow < 128, rrow + 128 * rlane, PRE + (rrow - 128) + TOK * rlane).astype(f32)
    m0 = jnp.max(rv)
    f0 = jnp.min(jnp.where(rv == m0, ridx, 1e9))
    rv2 = jnp.where(ridx == f0, -jnp.inf, rv)
    m1 = jnp.max(rv2)
    f1 = jnp.min(jnp.where(rv2 == m1, ridx, 1e9))
    i0 = jnp.clip(f0.astype(jnp.int32), 0, S - 1)
    i1 = jnp.clip(f1.astype(jnp.int32), 0, S - 1)
    row16 = lax.broadcasted_iota(jnp.int32, (16, DM), 0)
    xsel = jnp.where(row16 == 0, xn_scr[pl.ds(i0, 1), :],
                     jnp.where(row16 == 1, xn_scr[pl.ds(i1, 1), :], 0.0)).astype(bf16)
    wait_all(wg, SEM_WG)
    wait_all(wu, SEM_WU)
    wait_all(wd, SEM_WD)
    hs = []
    for j in range(FT):
        gate = _dot(xsel, _as_bf16(wg[j]))
        up = _dot(xsel, _as_bf16(wu[j]))
        hs.append((gate * jax.nn.sigmoid(gate) * up).astype(bf16))
    hid = jnp.concatenate(hs, axis=1)
    y = jnp.concatenate([_dot(hid, _as_bf16(wd[j])) for j in range(KT)], axis=1)
    rsel = jnp.where(lax.broadcasted_iota(jnp.int32, (16, 1), 0) == 0, m0, m1)
    y = y * jax.nn.sigmoid(rsel)
    y0, y1 = y[0:1], y[1:2]

    xpn_scr[pl.ds(i0, 1), :] = xpn_scr[pl.ds(i0, 1), :] + y0
    xpn_scr[pl.ds(i1, 1), :] = xpn_scr[pl.ds(i1, 1), :] + y1
    done = NSEG * TOK
    wait_all(out_stage.at[pl.ds(0, done)], SEM_OUT)
    g0 = pl.multiple_of((i0 // 16) * 16, 16)
    g1 = pl.multiple_of((i1 // 16) * 16, 16)
    redo0 = i0 < done
    redo1 = i1 < done
    send1 = jnp.logical_and(redo1, g1 != g0)

    def patch(i, gst, yy):
        blk = out_stage[pl.ds(gst, 16), :].astype(f32)
        out_stage[pl.ds(gst, 16), :] = (blk + jnp.where(row16 == i - gst, yy, 0.0)).astype(bf16)

    def patch_copy(gst, sem):
        return pltpu.make_async_copy(out_stage.at[pl.ds(gst, 16)], out_hbm.at[0, pl.ds(gst, 16)], sems.at[sem])

    @pl.when(redo0)
    def _():
        patch(i0, g0, y0)

    @pl.when(redo1)
    def _():
        patch(i1, g1, y1)

    @pl.when(redo0)
    def _():
        patch_copy(g0, SEM_P0).start()

    @pl.when(send1)
    def _():
        patch_copy(g1, SEM_P1).start()

    def epi_body(b, carry):
        pos = pl.multiple_of(64 * b, 64)
        r0 = pl.multiple_of(done + 128 * b, 128)
        for j in range(KT):
            l = jnp.concatenate(
                [_as_bf16(orings[(h % 8) // 2][2 * (h // 8) + h % 2, pl.ds(pos, 64), :]) for h in range(H)], axis=1)
            a = _dot(l, _as_bf16(wo[j]))
            cs = slice(128 * j, 128 * (j + 1))
            out_stage[pl.ds(r0, 128), cs] = (a + xpn_scr[pl.ds(r0, 128), cs]).astype(bf16)
        pltpu.make_async_copy(out_stage.at[pl.ds(r0, 128)], out_hbm.at[0, pl.ds(r0, 128)],
                              sems.at[SEM_OUT2]).start()
        return carry
    with jax.named_scope("epilogue"):
        lax.fori_loop(0, PRE // 128, epi_body, 0)

    with jax.named_scope("wait_out"):
        wait_all(out_stage.at[pl.ds(done, PRE)], SEM_OUT2)

    @pl.when(redo0)
    def _():
        patch_copy(g0, SEM_P0).wait()

    @pl.when(send1)
    def _():
        patch_copy(g1, SEM_P1).wait()


@jax.jit
def pallas_parallel_sum__memory_aug_recurrent_mem_tr__moe_arch_mod__prompt_kernel(
    A_x: jax.Array,
    A_mem0: jax.Array,
    A_Wq: jax.Array,
    A_Wk: jax.Array,
    A_Wv: jax.Array,
    A_Wo: jax.Array,
    A_seg_len: jax.Array,
    B_x: jax.Array,
    B_w_r: jax.Array,
    B_w_gate: jax.Array,
    B_w_up: jax.Array,
    B_w_down: jax.Array,
):
    del A_seg_len, B_x
    assert A_x.shape == (1, S, DM) and A_mem0.shape == (1, NMEM, DM)
    assert A_Wq.shape == (DM, H, DH) and A_Wo.shape == (H, DH, DM) and B_w_gate.shape == (DM, FF)
    hbm = pl.BlockSpec(memory_space=pl.ANY)
    vmem = pl.BlockSpec(memory_space=pltpu.VMEM)
    scratch = [
        pltpu.VMEM((S, DM), bf16),
        pltpu.VMEM((S, DM), f32),
        pltpu.VMEM((S, DM), f32),
        pltpu.VMEM((KT, PRE // 2, 128), u32),
        pltpu.VMEM((4, DM // 2, 8, 128), u32),
        pltpu.VMEM((3 * H, DM // 2, 128), u32),
        pltpu.VMEM((KT, H * DH // 2, 128), u32),
    ]
    scratch += [pltpu.VMEM((24, RQ // 2, 128), u32)] * NG
    scratch += [pltpu.VMEM((8, RO // 2, 128), u32)] * NG
    scratch += [pltpu.VMEM((8, 16, 128), u32)] * NG
    scratch += [
        pltpu.VMEM((NMEM, DM), f32),
        pltpu.VMEM((L2, L2), f32),
        pltpu.VMEM((128 + TOK, 128), f32),
        pltpu.VMEM((FT, DM // 2, 128), u32),
        pltpu.VMEM((FT, DM // 2, 128), u32),
        pltpu.VMEM((KT, FF // 2, 128), u32),
        pltpu.VMEM((S, DM), bf16),
        pltpu.SemaphoreType.DMA((NSEM,)),
    ]
    return pl.pallas_call(
        _kernel,
        out_shape=jax.ShapeDtypeStruct((1, S, DM), bf16),
        in_specs=[hbm, vmem, hbm, hbm, hbm, hbm, vmem, hbm, hbm, hbm],
        out_specs=hbm,
        scratch_shapes=scratch,
        compiler_params=pltpu.CompilerParams(vmem_limit_bytes=124 * 1024 * 1024),
    )(A_x, A_mem0, *[w.reshape(DM // 2, 2, H, DH) for w in (A_Wq, A_Wk, A_Wv)], A_Wo.reshape(H * DH, DM), B_w_r, B_w_gate, B_w_up, B_w_down)
```

```python
import jax
import jax.numpy as jnp
from jax import lax
import jax.experimental.pallas as pl
import jax.experimental.pallas.tpu as pltpu

bf16 = jnp.bfloat16
f32 = jnp.float32
u32 = jnp.uint32

S, DM, H, DH, NMEM, SEG, FF = 2048, 1024, 32, 128, 8, 32, 3584
NSEG = S // SEG
TOK = 24
PRE = S - NSEG * TOK
RQ = 544
RO = 832
NG = 4
KT = DM // 128
FT = FF // 128
L2 = 2 * (SEG + NMEM)
LOG2E = 1.4426950408889634
SCALE = DH ** -0.5 * LOG2E
PADK = 0
LK = 128 if PADK else L2
EPS_BF16 = 1.0013580322265625e-05

NSLOT = 6
SEM_W0 = 0
SEM_X0 = NSLOT
SEM_XB, SEM_XC, SEM_WO, SEM_WG, SEM_WU, SEM_WD, SEM_OUT, SEM_P0, SEM_P1, SEM_OUT2 = range(NSLOT + 4, NSLOT + 14)
NSEM = NSLOT + 14
XB_ROWS = 384


def _as_bf16(x):
    return pltpu.bitcast(x, bf16)


def _as_u32(x):
    return pltpu.bitcast(x, u32)


def _rnd(x):
    return x.astype(bf16).astype(f32)


def _dot(a, b):
    return jnp.dot(a, b, preferred_element_type=f32)


def _head(g, c, hh):
    return 8 * c + 2 * g + hh


def _kernel(x_hbm, mem0_ref, wq_hbm, wk_hbm, wv_hbm, wo_hbm, wr_ref, wg_hbm, wu_hbm, wd_hbm,
            out_hbm,
            x_scr, xn_scr, xpn_scr, lhs_pre, stage, wqkv, wo,
            qr0, qr1, qr2, qr3, or0, or1, or2, or3, lo0, lo1, lo2, lo3,
            mem_scr, fill_scr, racc, wg, wu, wd, out_stage, sems):
    qrings = (qr0, qr1, qr2, qr3)
    orings = (or0, or1, or2, or3)
    lhs_os = (lo0, lo1, lo2, lo3)
    w32 = [w.bitcast(u32) for w in (wq_hbm, wk_hbm, wv_hbm)]
    wo32 = wo_hbm.bitcast(u32)
    wg32 = wg_hbm.bitcast(u32)
    wu32 = wu_hbm.bitcast(u32)
    wd32 = wd_hbm.bitcast(u32)

    def x_copy(r0, n, sem):
        return pltpu.make_async_copy(x_hbm.at[0, pl.ds(r0, n)], x_scr.at[pl.ds(r0, n)], sems.at[sem])

    def w_copy(t, lo, n, sem, e):
        return pltpu.make_async_copy(w32[t // 4].at[:, e, pl.ds(4 * (t % 4) + lo, n), :],
                                     stage.at[t % 4, :, pl.ds(4 * e + lo, n), :], sems.at[SEM_W0 + sem])

    def w_start(t, lo=0, n=4, sem=None):
        for e in range(2):
            w_copy(t, lo, n, t % 4 if sem is None else sem, e).start()

    def w_wait(t, lo=0, n=4, sem=None):
        for e in range(2):
            w_copy(t, lo, n, t % 4 if sem is None else sem, e).wait()

    def col_tiles_start(src, dst, sem, lo, hi):
        for j in range(lo, hi):
            pltpu.make_async_copy(src.at[:, pl.ds(128 * j, 128)], dst.at[j], sems.at[sem]).start()

    def wait_all(buf, sem):
        pltpu.make_async_copy(buf, buf, sems.at[sem]).wait()

    for c in range(4):
        x_copy(128 * c, 128, SEM_X0 + c).start()
    w_start(0, 0, 2, 4)
    w_start(0, 2, 2, 5)

    mem_scr[...] = mem0_ref[0].astype(f32)
    racc[...] = jnp.full(racc.shape, -jnp.inf, f32)
    qi = lax.broadcasted_iota(jnp.int32, (L2, LK), 0)
    ki = lax.broadcasted_iota(jnp.int32, (L2, LK), 1)
    q_mem, k_mem = qi >= 2 * SEG, ki >= 2 * SEG
    q_head = jnp.where(q_mem, (qi - 2 * SEG) // NMEM, qi // SEG)
    k_head = jnp.where(k_mem, (ki - 2 * SEG) // NMEM, ki // SEG)
    visible = q_mem | k_mem | (qi >= ki)
    fill_scr[...] = jnp.where(q_head == k_head, jnp.where(visible, 0.0, -1e9 * LOG2E), -jnp.inf).astype(f32)

    def ln_rows(r0, n, racc_row, lane_id):
        wr = wr_ref[...].astype(f32).reshape(1, DM)
        lane = lax.broadcasted_iota(jnp.int32, (n, 128), 1)
        x = x_scr[pl.ds(r0, n), :].astype(f32)
        mean = jnp.sum(x, axis=-1, keepdims=True) * (1.0 / DM)
        xc = x - mean
        var = jnp.sum(xc * xc, axis=-1, keepdims=True) * (1.0 / DM)
        den = _rnd(jnp.sqrt(_rnd(_rnd(var) + EPS_BF16)))
        xnb = (_rnd(x - _rnd(mean)) * (1.0 / den)).astype(bf16)
        xn = xnb.astype(f32)
        xn_scr[pl.ds(r0, n), :] = xn
        xpn_scr[pl.ds(r0, n), :] = x + xn
        r = _rnd(jnp.sum(xn * wr, axis=-1, keepdims=True))
        racc[racc_row:racc_row + n, :] = jnp.where(lane == lane_id, r, racc[racc_row:racc_row + n, :])
        return xnb

    def ln_chunk(c):
        for i in range(8):
            xnb = ln_rows(pl.multiple_of(c * 128 + 16 * i, 16), 16, 16 * i, c)
            p0 = pl.multiple_of(c * 64 + 8 * i, 8)
            for k in range(KT):
                lhs_pre[k, pl.ds(p0, 8), :] = _as_u32(xnb[:, 128 * k:128 * (k + 1)])

    def ln_first(c, carry):
        r0 = pl.multiple_of(128 * c, 128)
        pltpu.make_async_copy(x_hbm.at[0, pl.ds(r0, 128)], x_scr.at[pl.ds(r0, 128)], sems.at[SEM_X0 + c]).wait()
        ln_chunk(c)
        return carry
    with jax.named_scope("ln_first"):
        lax.fori_loop(0, PRE // 128, ln_first, 0)

    stage2d = stage.reshape(4 * DM * 4, 128)

    def pro_pairs(t, gs):
        m, c8 = t // 4, t % 4
        sc = (SCALE if m == 0 else None) if isinstance(t, int) else jnp.where(m == 0, SCALE, 1.0).astype(f32)
        for g in gs:
            both = stage2d[pl.ds(c8 * (DM * 4) + g, DM, stride=4), :]
            pair = (pltpu.bitcast(both << 16, f32).astype(bf16),
                    pltpu.bitcast(both & jnp.uint32(0xFFFF0000), f32).astype(bf16))
            for hh in range(2):
                wqkv[_head(g, c8, hh) * 3 + m] = _as_u32(pair[hh])
                lhs = jnp.concatenate([_as_bf16(lhs_pre[k]) for k in range(KT)], axis=1)
                y = _dot(lhs, pair[hh])
                if sc is not None:
                    y = y * sc
                qrings[g][(2 * c8 + hh) * 3 + m, 0:PRE // 2, :] = _as_u32(y.astype(bf16))

    with jax.named_scope("pro_a"):
        w_start(1)
        w_wait(0, 0, 2, 4)
        pro_pairs(0, (0, 1))
    with jax.named_scope("pro_b"):
        w_start(2)
        w_start(3)
        w_wait(0, 2, 2, 5)
        pro_pairs(0, (2, 3))
    with jax.named_scope("pro_c"):
        w_wait(1)
        pro_pairs(1, range(NG))

    def pro_body(i, carry):
        for k in range(5):
            @pl.when(i == k)
            def _():
                w_wait(2 + 2 * k)
                w_wait(3 + 2 * k)
                if k < 4:
                    w_start(4 + 2 * k)
                    w_start(5 + 2 * k)
                if k == 0:
                    x_copy(PRE, S - PRE, SEM_XB).start()
                if k in (1, 2):
                    col_tiles_start(wo32, wo, SEM_WO, 4 * (k - 1), 4 * k)
                if k == 4:
                    col_tiles_start(wg32, wg, SEM_WG, 0, FT)
                    col_tiles_start(wu32, wu, SEM_WU, 0, FT)
                    col_tiles_start(wd32, wd, SEM_WD, 0, KT)
        pro_pairs(2 + 2 * i, range(NG))
        pro_pairs(3 + 2 * i, range(NG))
        return carry
    with jax.named_scope("prologue"):
        lax.fori_loop(0, 5, pro_body, 0)
    with jax.named_scope("wait_wo"):
        wait_all(wo, SEM_WO)
        x_copy(PRE, S - PRE, SEM_XB).wait()
    ln_rows(PRE, TOK, 128, 0)
    for g in range(NG):
        orings[g][:, 48:64, :] = jnp.zeros((8, 16, 128), u32)

    def out_row(s):
        return TOK * s + SEG * ((s + 16) // 20)

    def o_rows(pos, n):
        return jnp.concatenate(
            [_as_bf16(orings[(h % 8) // 2][2 * (h // 8) + h % 2, pl.ds(pos, n), :]) for h in range(H)], axis=1)

    def filler(u):
        k = jnp.maximum(u - 2, 0)
        j = k % 8
        r0 = pl.multiple_of(SEG * (16 * (k // 8) + 3), SEG)
        pos = pl.multiple_of(lax.rem(r0, RO) // 2, 16)
        cs = pl.ds(pl.multiple_of(128 * j, 128), 128)
        a = _dot(o_rows(pos, SEG // 2), _as_bf16(wo[j]))
        out_stage[pl.ds(r0, SEG), cs] = (a + xpn_scr[pl.ds(r0, SEG), cs]).astype(bf16)

    def step(s, mem_in):
        xrow = pl.multiple_of(PRE + TOK * s, 8)
        wr_pos = [pl.multiple_of(lax.rem(PRE + TOK * s + 8 * i, RQ) // 2, 4) for i in range(3)]
        rd = pl.multiple_of(lax.rem(SEG * s, RQ) // 2, 16)
        owr = pl.multiple_of(lax.rem(SEG * s, RO) // 2, 16)
        orow = pl.multiple_of(out_row(s), 8)
        ord_ = pl.multiple_of(lax.rem(orow, RO) // 2, 4)
        lhs_box = []

        def load_lhs():
            lhs_box[:] = [jnp.concatenate([xn_scr[pl.ds(xrow, TOK), :], mem_in], axis=0).astype(bf16)]
        load_lhs()

        mem_parts, probs = {}, {}

        def qkv(g, c):
            lhs = lhs_box[0]
            res = []
            for m in range(3):
                ms = []
                for hh in range(2):
                    y = _dot(lhs, _as_bf16(wqkv[_head(g, c, hh) * 3 + m]))
                    if m == 0:
                        y = y * SCALE
                    yp = _as_u32(y.astype(bf16))
                    for i in range(3):
                        qrings[g][(2 * c + hh) * 3 + m, pl.ds(wr_pos[i], 4), :] = yp[4 * i:4 * i + 4]
                    ms.append(y[TOK:])
                res.append(jnp.concatenate(ms, axis=0).astype(bf16))
            mem_parts[g, c] = res

        def pair_rows(g, c, m, mem_rows):
            t0 = _as_bf16(qrings[g][(2 * c) * 3 + m, pl.ds(rd, SEG // 2), :])
            t1 = _as_bf16(qrings[g][(2 * c + 1) * 3 + m, pl.ds(rd, SEG // 2), :])
            pad = [jnp.zeros((LK - L2, 128), bf16)] if (m > 0 and LK > L2) else []
            return jnp.concatenate([t0, t1, mem_rows] + pad, axis=0)

        def scores(g, c):
            qm, km, vm = mem_parts.pop((g, c))
            sc = lax.dot_general(pair_rows(g, c, 0, qm), pair_rows(g, c, 1, km),
                                 (((1,), (1,)), ((), ())), preferred_element_type=f32)
            fill = fill_scr[...]
            sc = jnp.where(fill == 0.0, sc, fill)
            e = jnp.exp2(sc - jnp.max(sc, axis=-1, keepdims=True))
            r = pl.reciprocal(jnp.sum(e, axis=-1, keepdims=True), approx=True)
            probs[g, c] = (e.astype(bf16), r, vm)

        def pv(g, c):
            e, r, vm = probs.pop((g, c))
            o = _dot(e, pair_rows(g, c, 2, vm)) * r
            for hh in range(2):
                h = 2 * c + hh
                orings[g][h, pl.ds(owr, SEG // 2), :] = _as_u32(o[SEG * hh:SEG * (hh + 1)].astype(bf16))
                tok = _as_bf16(orings[g][h, pl.ds(ord_, TOK // 2), :])
                om = o[2 * SEG + NMEM * hh:2 * SEG + NMEM * (hh + 1)]
                last = jnp.concatenate([tok[16:TOK].astype(f32), om], axis=0).astype(bf16)
                lhs_os[g][h] = _as_u32(jnp.concatenate([tok[0:16], last], axis=0))

        acc = [None] * KT

        def out_proj(gs, js):
            for j in js:
                l = jnp.concatenate([_as_bf16(lhs_os[g][k]) for g in gs for k in range(8)], axis=1)
                w = jnp.concatenate(
                    [_as_bf16(wo[j, 64 * _head(g, c, 0):64 * _head(g, c, 0) + 128, :])
                     for g in gs for c in range(4)], axis=0)
                a = _dot(l, w)
                if acc[j] is None:
                    cs = slice(128 * j, 128 * (j + 1))
                    acc[j] = a + jnp.concatenate([xpn_scr[pl.ds(orow, TOK), cs], jnp.zeros((NMEM, 128), f32)], axis=0)
                else:
                    acc[j] = acc[j] + a

        for item in "q0 q1 s0 q2 p0 s1 q3 p1 s2 w01a p2 s3 w012b L0 p3 w2a w3".split():
            g = int(item[1])
            if item[0] == "L":
                nxt = jnp.minimum(s + 1, NSEG - 1)
                ln_rows(pl.multiple_of(PRE + TOK * nxt, 8), TOK, 128, nxt)
            elif item[0] == "w":
                out_proj([int(ch) for ch in item[1:] if ch.isdigit()],
                         {"a": range(4), "b": range(4, 8)}.get(item[-1], range(8)))
            else:
                for c in range(4):
                    {"q": qkv, "s": scores, "p": pv}[item[0]](g, c)
        a = jnp.concatenate(acc, axis=1)
        out_stage[pl.ds(orow, TOK), :] = a[:TOK].astype(bf16)
        return _rnd(a[TOK:])

    def body(u, carry):
        mem = step(2 * u, mem_scr[...])
        filler(u)
        mem_scr[...] = step(2 * u + 1, mem)
        orow = pl.multiple_of(out_row(2 * u), 8)
        pltpu.make_async_copy(out_stage.at[pl.ds(orow, 2 * TOK)], out_hbm.at[0, pl.ds(orow, 2 * TOK)],
                              sems.at[SEM_OUT]).start()
        return carry
    with jax.named_scope("chain"):
        lax.fori_loop(0, NSEG // 2, body, 0)

    def out_copy(r0, n, sem):
        return pltpu.make_async_copy(out_stage.at[pl.ds(r0, n)], out_hbm.at[0, pl.ds(r0, n)], sems.at[sem])

    wait_all(wg, SEM_WG)
    wait_all(wu, SEM_WU)
    wait_all(wd, SEM_WD)
    for f in (3, 19, 35):
        out_copy(SEG * f, SEG, SEM_OUT).start()

    rv = racc[...]
    rrow = lax.broadcasted_iota(jnp.int32, rv.shape, 0)
    rlane = lax.broadcasted_iota(jnp.int32, rv.shape, 1)
    ridx = jnp.where(rrow < 128, rrow + 128 * rlane, PRE + (rrow - 128) + TOK * rlane).astype(f32)
    m0 = jnp.max(rv, keepdims=True)
    f0 = jnp.min(jnp.where(rv == m0, ridx, 1e9), keepdims=True)
    rv2 = jnp.where(ridx == f0, -jnp.inf, rv)
    m1 = jnp.max(rv2, keepdims=True)
    f1 = jnp.min(jnp.where(rv2 == m1, ridx, 1e9), keepdims=True)
    i0 = jnp.clip(f0[0, 0].astype(jnp.int32), 0, S - 1)
    i1 = jnp.clip(f1[0, 0].astype(jnp.int32), 0, S - 1)
    row16 = lax.broadcasted_iota(jnp.int32, (16, DM), 0)
    xsel = jnp.where(row16 == 0, xn_scr[pl.ds(i0, 1), :],
                     jnp.where(row16 == 1, xn_scr[pl.ds(i1, 1), :], 0.0)).astype(bf16)

    r51 = 51 * SEG
    for j in (6, 7):
        cs = slice(128 * j, 128 * (j + 1))
        a = _dot(o_rows((r51 % RO) // 2, SEG // 2), _as_bf16(wo[j]))
        out_stage[r51:r51 + SEG, cs] = (a + xpn_scr[r51:r51 + SEG, cs]).astype(bf16)
    out_copy(r51, SEG, SEM_OUT).start()

    e0 = r51 + SEG
    last = S - 128
    part = {}

    def add(key, v):
        part[key] = v if key not in part else v + part[key]

    def e_round(b, j, r):
        l = jnp.concatenate(
            [_as_bf16(orings[(h % 8) // 2][2 * (h // 8) + h % 2, 64 * b:64 * (b + 1), :])
             for h in range(4 * r, 4 * r + 4)], axis=1)
        add(("e", b, j), _dot(l, _as_bf16(wo[j, 256 * r:256 * (r + 1), :])))
        if r == 7:
            rows, cs = slice(e0 + 128 * b, e0 + 128 * (b + 1)), slice(128 * j, 128 * (j + 1))
            out_stage[rows, cs] = (part.pop(("e", b, j)) + xpn_scr[rows, cs]).astype(bf16)
            if j == KT - 1:
                out_copy(e0 + 128 * b, 128, SEM_OUT if b < 2 else SEM_OUT2).start()

    def up_round(w, name, j, r):
        add((name, j), _dot(xsel[:, 512 * r:512 * (r + 1)], _as_bf16(w[j, 256 * r:256 * (r + 1), :])))
        if name == "u" and r == 1:
            gate = part.pop(("g", j))
            part["h", j] = (gate * jax.nn.sigmoid(gate) * part.pop(("u", j))).astype(bf16)

    def down_round(j, r):
        hid = jnp.concatenate([part["h", k] for k in range(4 * r, 4 * r + 4)], axis=1)
        add(("y", j), _dot(hid, _as_bf16(wd[j, 256 * r:256 * (r + 1), :])))

    e_rounds = [(b, j, r) for b in range(3) for j in range(KT) for r in range(8)]
    m_rounds = [lambda j=j, r=r, w=w, n=n: up_round(w, n, j, r)
                for j in range(FT) for (w, n) in ((wg, "g"), (wu, "u")) for r in range(2)]
    m_rounds += [None] * 4
    m_rounds += [lambda j=j, r=r: down_round(j, r) for r in range(FT // 4) for j in range(KT)]
    m_rounds = [None] * 8 + m_rounds
    NM = 2
    for n, er in enumerate(e_rounds[:128]):
        e_round(*er)
        for mr in m_rounds[NM * n:NM * n + NM]:
            if mr is not None:
                mr()
    assert len(m_rounds) <= NM * 128
    rsel = jnp.where(lax.broadcasted_iota(jnp.int32, (16, 1), 0) == 0, m0, m1)
    y = jnp.concatenate([part.pop(("y", j)) for j in range(KT)], axis=1) * jax.nn.sigmoid(rsel)
    y0, y1 = y[0:1], y[1:2]
    xpn_scr[pl.ds(i0, 1), :] = xpn_scr[pl.ds(i0, 1), :] + jnp.where(i0 >= last, y0, 0.0)
    xpn_scr[pl.ds(i1, 1), :] = xpn_scr[pl.ds(i1, 1), :] + jnp.where(i1 >= last, y1, 0.0)
    for er in e_rounds[128:]:
        e_round(*er)

    with jax.named_scope("wait_out"):
        wait_all(out_stage.at[pl.ds(0, last)], SEM_OUT)
    g0 = pl.multiple_of((i0 // 16) * 16, 16)
    g1 = pl.multiple_of((i1 // 16) * 16, 16)
    redo0 = i0 < last
    redo1 = i1 < last
    send1 = jnp.logical_and(redo1, g1 != g0)

    def patch(i, gst, yy):
        blk = out_stage[pl.ds(gst, 16), :].astype(f32)
        out_stage[pl.ds(gst, 16), :] = (blk + jnp.where(row16 == i - gst, yy, 0.0)).astype(bf16)

    @pl.when(redo0)
    def _():
        patch(i0, g0, y0)

    @pl.when(redo1)
    def _():
        patch(i1, g1, y1)

    @pl.when(redo0)
    def _():
        out_copy(g0, 16, SEM_P0).start()

    @pl.when(send1)
    def _():
        out_copy(g1, 16, SEM_P1).start()

    with jax.named_scope("wait_out2"):
        out_copy(last, 128, SEM_OUT2).wait()

    @pl.when(redo0)
    def _():
        out_copy(g0, 16, SEM_P0).wait()

    @pl.when(send1)
    def _():
        out_copy(g1, 16, SEM_P1).wait()


@jax.jit
def pallas_parallel_sum__memory_aug_recurrent_mem_tr__moe_arch_mod__prompt_kernel(
    A_x: jax.Array,
    A_mem0: jax.Array,
    A_Wq: jax.Array,
    A_Wk: jax.Array,
    A_Wv: jax.Array,
    A_Wo: jax.Array,
    A_seg_len: jax.Array,
    B_x: jax.Array,
    B_w_r: jax.Array,
    B_w_gate: jax.Array,
    B_w_up: jax.Array,
    B_w_down: jax.Array,
):
    del A_seg_len, B_x
    assert A_x.shape == (1, S, DM) and A_mem0.shape == (1, NMEM, DM)
    assert A_Wq.shape == (DM, H, DH) and A_Wo.shape == (H, DH, DM) and B_w_gate.shape == (DM, FF)
    hbm = pl.BlockSpec(memory_space=pl.ANY)
    vmem = pl.BlockSpec(memory_space=pltpu.VMEM)
    scratch = [
        pltpu.VMEM((S, DM), bf16),
        pltpu.VMEM((S, DM), f32),
        pltpu.VMEM((S, DM), f32),
        pltpu.VMEM((KT, PRE // 2, 128), u32),
        pltpu.VMEM((4, DM // 2, 8, 128), u32),
        pltpu.VMEM((3 * H, DM // 2, 128), u32),
        pltpu.VMEM((KT, H * DH // 2, 128), u32),
    ]
    scratch += [pltpu.VMEM((24, RQ // 2, 128), u32)] * NG
    scratch += [pltpu.VMEM((8, RO // 2, 128), u32)] * NG
    scratch += [pltpu.VMEM((8, 16, 128), u32)] * NG
    scratch += [
        pltpu.VMEM((NMEM, DM), f32),
        pltpu.VMEM((L2, LK), f32),
        pltpu.VMEM((128 + TOK, 128), f32),
        pltpu.VMEM((FT, DM // 2, 128), u32),
        pltpu.VMEM((FT, DM // 2, 128), u32),
        pltpu.VMEM((KT, FF // 2, 128), u32),
        pltpu.VMEM((S, DM), bf16),
        pltpu.SemaphoreType.DMA((NSEM,)),
    ]
    return pl.pallas_call(
        _kernel,
        out_shape=jax.ShapeDtypeStruct((1, S, DM), bf16),
        in_specs=[hbm, vmem, hbm, hbm, hbm, hbm, vmem, hbm, hbm, hbm],
        out_specs=hbm,
        scratch_shapes=scratch,
        compiler_params=pltpu.CompilerParams(vmem_limit_bytes=124 * 1024 * 1024),
    )(A_x, A_mem0, *[w.reshape(DM // 2, 2, H, DH) for w in (A_Wq, A_Wk, A_Wv)], A_Wo.reshape(H * DH, DM), B_w_r, B_w_gate, B_w_up, B_w_down)
```

```python
import jax
import jax.numpy as jnp
from jax import lax
import jax.experimental.pallas as pl
import jax.experimental.pallas.tpu as pltpu

bf16 = jnp.bfloat16
f32 = jnp.float32
u32 = jnp.uint32

S, DM, H, DH, NMEM, SEG, FF = 2048, 1024, 32, 128, 8, 32, 3584
NSEG = S // SEG
TOK = 24
PRE = S - NSEG * TOK
RQ = 544
RO = 832
NG = 4
KT = DM // 128
FT = FF // 128
L2 = 2 * (SEG + NMEM)
LOG2E = 1.4426950408889634
SCALE = DH ** -0.5 * LOG2E
PADK = 0
LK = 128 if PADK else L2
EPS_BF16 = 1.0013580322265625e-05

NSLOT = 7
SEM_W0 = 0
SEM_X0 = NSLOT
SEM_XB, SEM_XC, SEM_WO, SEM_WG, SEM_WU, SEM_WD, SEM_OUT, SEM_P0, SEM_P1, SEM_OUT2 = range(NSLOT + 4, NSLOT + 14)
NSEM = NSLOT + 14
XB_ROWS = 384


def _as_bf16(x):
    return pltpu.bitcast(x, bf16)


def _as_u32(x):
    return pltpu.bitcast(x, u32)


def _rnd(x):
    return x.astype(bf16).astype(f32)


def _dot(a, b):
    return jnp.dot(a, b, preferred_element_type=f32)


def _head(g, c, hh):
    return 8 * c + 2 * g + hh


def _kernel(x_hbm, mem0_ref, wq_hbm, wk_hbm, wv_hbm, wo_hbm, wr_ref, wg_hbm, wu_hbm, wd_hbm,
            out_hbm,
            x_scr, xpn_scr, xn_pk, wr_scr, stage, wqkv, wo,
            qr0, qr1, qr2, qr3, or0, or1, or2, or3, lo0, lo1, lo2, lo3,
            mem_scr, zero_scr, fill_scr, racc, wg, wu, wd, out_stage, sems):
    qrings = (qr0, qr1, qr2, qr3)
    orings = (or0, or1, or2, or3)
    lhs_os = (lo0, lo1, lo2, lo3)
    w32 = [w.bitcast(u32) for w in (wq_hbm, wk_hbm, wv_hbm)]
    wo32 = wo_hbm.bitcast(u32)
    wg32 = wg_hbm.bitcast(u32)
    wu32 = wu_hbm.bitcast(u32)
    wd32 = wd_hbm.bitcast(u32)

    def x_copy(r0, n, sem):
        return pltpu.make_async_copy(x_hbm.at[0, pl.ds(r0, n)], x_scr.at[pl.ds(r0, n)], sems.at[sem])

    def w_copy(t, lo, n, sem, e):
        return pltpu.make_async_copy(w32[t // 4].at[:, e, pl.ds(4 * (t % 4) + lo, n), :],
                                     stage.at[t % 4, :, pl.ds(4 * e + lo, n), :], sems.at[SEM_W0 + sem])

    def w_start(t, lo=0, n=4, sem=None, prio=0):
        for e in range(2):
            w_copy(t, lo, n, t % 4 if sem is None else sem, e).start(priority=prio)

    def w_wait(t, lo=0, n=4, sem=None):
        for e in range(2):
            w_copy(t, lo, n, t % 4 if sem is None else sem, e).wait()

    def col_tiles_start(src, dst, sem, lo, hi):
        for j in range(lo, hi):
            pltpu.make_async_copy(src.at[:, pl.ds(128 * j, 128)], dst.at[j], sems.at[sem]).start()

    def wait_all(buf, sem):
        pltpu.make_async_copy(buf, buf, sems.at[sem]).wait()

    for c in range(4):
        x_copy(128 * c, 128, SEM_X0 + c).start()
    w_start(0, 0, 1, 4)
    w_start(0, 1, 1, 5)
    w_start(0, 2, 2, 6)
    w_start(1)
    x_copy(PRE, TOK, SEM_XC).start()
    w_start(2)
    w_start(3)

    mem_scr[...] = mem0_ref[0].astype(f32)
    zero_scr[...] = jnp.zeros(zero_scr.shape, u32)
    wr_row = wr_ref[...].astype(f32).reshape(1, DM)
    wr_scr[0:8, :] = jnp.broadcast_to(wr_row, (8, DM))
    wr_scr[8:16, :] = jnp.broadcast_to(jnp.sum(wr_row, axis=-1, keepdims=True), (8, DM))
    racc[...] = jnp.full(racc.shape, -jnp.inf, f32)
    qi = lax.broadcasted_iota(jnp.int32, (L2, LK), 0)
    ki = lax.broadcasted_iota(jnp.int32, (L2, LK), 1)
    q_mem, k_mem = qi >= 2 * SEG, ki >= 2 * SEG
    q_head = jnp.where(q_mem, (qi - 2 * SEG) // NMEM, qi // SEG)
    k_head = jnp.where(k_mem, (ki - 2 * SEG) // NMEM, ki // SEG)
    visible = q_mem | k_mem | (qi >= ki)
    fill_scr[...] = jnp.where(q_head == k_head, jnp.where(visible, 0.0, -1e9 * LOG2E), -jnp.inf).astype(f32)

    def ln_rows(r0, n, racc_row, lane_id):
        lane = lax.broadcasted_iota(jnp.int32, (n, 128), 1)
        wr = jnp.concatenate([wr_scr[0:8, :]] * (n // 8), axis=0)
        wr_sum = jnp.concatenate([wr_scr[8:16, 0:1]] * (n // 8), axis=0)
        x = x_scr[pl.ds(r0, n), :].astype(f32)
        mean = jnp.sum(x, axis=-1, keepdims=True) * (1.0 / DM)
        msq = jnp.sum(x * x, axis=-1, keepdims=True) * (1.0 / DM)
        xw = jnp.sum(x * wr, axis=-1, keepdims=True)
        var = jnp.maximum(msq - mean * mean, 0.0)
        inv = 1.0 / _rnd(jnp.sqrt(_rnd(_rnd(var) + EPS_BF16)))
        mean = _rnd(mean)
        xnb = ((x - mean) * inv).astype(bf16)
        xpn_scr[pl.ds(r0, n), :] = x + xnb.astype(f32)
        xnp = _as_u32(xnb)
        p0 = r0 // 2 if isinstance(r0, int) else pl.multiple_of(r0 // 2, 4)
        for k in range(KT):
            xn_pk[k, pl.ds(p0, n // 2), :] = xnp[:, 128 * k:128 * (k + 1)]
        r = _rnd((xw - mean * wr_sum) * inv)
        racc[racc_row:racc_row + n, :] = jnp.where(lane == lane_id, r, racc[racc_row:racc_row + n, :])

    def ln_chunk(c):
        for i in range(8):
            ln_rows(pl.multiple_of(c * 128 + 16 * i, 16), 16, 16 * i, c)

    def ln_first(c, carry):
        r0 = pl.multiple_of(128 * c, 128)
        pltpu.make_async_copy(x_hbm.at[0, pl.ds(r0, 128)], x_scr.at[pl.ds(r0, 128)], sems.at[SEM_X0 + c]).wait()
        ln_chunk(c)
        return carry
    with jax.named_scope("ln_first"):
        lax.fori_loop(0, PRE // 128, ln_first, 0)

    stage2d = stage.reshape(4 * DM * 4, 128)

    def pro_pairs(t, gs):
        m, c8 = t // 4, t % 4
        sc = (SCALE if m == 0 else None) if isinstance(t, int) else jnp.where(m == 0, SCALE, 1.0).astype(f32)
        for g in gs:
            both = stage2d[pl.ds(c8 * (DM * 4) + g, DM, stride=4), :]
            pair = (pltpu.bitcast(both << 16, f32).astype(bf16),
                    pltpu.bitcast(both & jnp.uint32(0xFFFF0000), f32).astype(bf16))
            for hh in range(2):
                wqkv[_head(g, c8, hh) * 3 + m] = _as_u32(pair[hh])
                lhs = jnp.concatenate([_as_bf16(xn_pk[k, 0:PRE // 2, :]) for k in range(KT)], axis=1)
                y = _dot(lhs, pair[hh])
                if sc is not None:
                    y = y * sc
                qrings[g][(2 * c8 + hh) * 3 + m, 0:PRE // 2, :] = _as_u32(y.astype(bf16))

    with jax.named_scope("pro_a"):
        w_wait(0, 0, 1, 4)
        pro_pairs(0, (0,))
    with jax.named_scope("pro_a2"):
        w_wait(0, 1, 1, 5)
        pro_pairs(0, (1,))
    with jax.named_scope("pro_b"):
        w_wait(0, 2, 2, 6)
        pro_pairs(0, (2, 3))
    with jax.named_scope("pro_c"):
        w_wait(1)
        x_copy(PRE, TOK, SEM_XC).wait()
        pro_pairs(1, range(NG))
        ln_rows(PRE, TOK, 128, 0)
        for g in range(NG):
            orings[g][:, 48:64, :] = jnp.zeros((8, 16, 128), u32)

    def pro_body(i, carry):
        for k in range(5):
            @pl.when(i == k)
            def _():
                w_wait(2 + 2 * k)
                w_wait(3 + 2 * k)
                if k < 4:
                    w_start(4 + 2 * k)
                    w_start(5 + 2 * k)
                if k == 0:
                    x_copy(PRE + TOK, S - PRE - TOK, SEM_XB).start()
                if k in (1, 2):
                    col_tiles_start(wo32, wo, SEM_WO, 4 * (k - 1), 4 * k)
                if k == 4:
                    col_tiles_start(wg32, wg, SEM_WG, 0, FT)
                    col_tiles_start(wu32, wu, SEM_WU, 0, FT)
                    col_tiles_start(wd32, wd, SEM_WD, 0, KT)
        pro_pairs(2 + 2 * i, range(NG))
        pro_pairs(3 + 2 * i, range(NG))
        return carry
    with jax.named_scope("prologue"):
        lax.fori_loop(0, 5, pro_body, 0)
    with jax.named_scope("wait_wo"):
        wait_all(wo, SEM_WO)
        x_copy(PRE + TOK, S - PRE - TOK, SEM_XB).wait()

    def out_row(s):
        return TOK * s + SEG * ((s + 16) // 20)

    def o_rows(pos, n):
        return jnp.concatenate(
            [_as_bf16(orings[(h % 8) // 2][2 * (h // 8) + h % 2, pl.ds(pos, n), :]) for h in range(H)], axis=1)

    def filler(u):
        k = jnp.maximum(u - 2, 0)
        j = k % 8
        r0 = pl.multiple_of(SEG * (16 * (k // 8) + 3), SEG)
        pos = pl.multiple_of(lax.rem(r0, RO) // 2, 16)
        cs = pl.ds(pl.multiple_of(128 * j, 128), 128)
        a = _dot(o_rows(pos, SEG // 2), _as_bf16(wo[j]))
        out_stage[pl.ds(r0, SEG), cs] = (a + xpn_scr[pl.ds(r0, SEG), cs]).astype(bf16)

    def step(s, mem_in):
        xpos = pl.multiple_of((PRE + TOK * s) // 2, 4)
        wr_pos = [pl.multiple_of(lax.rem(PRE + TOK * s + 8 * i, RQ) // 2, 4) for i in range(3)]
        rd = pl.multiple_of(lax.rem(SEG * s, RQ) // 2, 16)
        owr = pl.multiple_of(lax.rem(SEG * s, RO) // 2, 16)
        orow = pl.multiple_of(out_row(s), 8)
        ord_ = pl.multiple_of(lax.rem(orow, RO) // 2, 4)
        def with_mem(tok_u32, mem_rows):
            tok = _as_bf16(tok_u32)
            last = jnp.concatenate([tok[16:TOK].astype(f32), mem_rows], axis=0).astype(bf16)
            return jnp.concatenate([tok[0:16], last], axis=0)

        zero = zero_scr[0:TOK // 2, :]
        lhs = jnp.concatenate(
            [with_mem(xn_pk[k, pl.ds(xpos, TOK // 2), :] ^ zero, mem_in[:, 128 * k:128 * (k + 1)])
             for k in range(KT)], axis=1)

        mem_parts, probs = {}, {}

        def qkv(g, c):
            res = []
            for m in range(3):
                ms = []
                for hh in range(2):
                    y = _dot(lhs, _as_bf16(wqkv[_head(g, c, hh) * 3 + m]))
                    if m == 0:
                        y = y * SCALE
                    yp = _as_u32(y.astype(bf16))
                    for i in range(3):
                        qrings[g][(2 * c + hh) * 3 + m, pl.ds(wr_pos[i], 4), :] = yp[4 * i:4 * i + 4]
                    ms.append(y[TOK:])
                res.append(jnp.concatenate(ms, axis=0).astype(bf16))
            mem_parts[g, c] = res

        def pair_rows(g, c, m, mem_rows):
            t0 = _as_bf16(qrings[g][(2 * c) * 3 + m, pl.ds(rd, SEG // 2), :])
            t1 = _as_bf16(qrings[g][(2 * c + 1) * 3 + m, pl.ds(rd, SEG // 2), :])
            pad = [jnp.zeros((LK - L2, 128), bf16)] if (m > 0 and LK > L2) else []
            return jnp.concatenate([t0, t1, mem_rows] + pad, axis=0)

        def scores(g, c):
            qm, km, vm = mem_parts.pop((g, c))
            sc = lax.dot_general(pair_rows(g, c, 0, qm), pair_rows(g, c, 1, km),
                                 (((1,), (1,)), ((), ())), preferred_element_type=f32)
            fill = fill_scr[...]
            sc = jnp.where(fill == 0.0, sc, fill)
            e = jnp.exp2(sc - jnp.max(sc, axis=-1, keepdims=True))
            r = pl.reciprocal(jnp.sum(e, axis=-1, keepdims=True), approx=True)
            probs[g, c] = (e.astype(bf16), r, vm)

        def pv(g, c):
            e, r, vm = probs.pop((g, c))
            o = _dot(e, pair_rows(g, c, 2, vm)) * r
            for hh in range(2):
                h = 2 * c + hh
                orings[g][h, pl.ds(owr, SEG // 2), :] = _as_u32(o[SEG * hh:SEG * (hh + 1)].astype(bf16))
                om = o[2 * SEG + NMEM * hh:2 * SEG + NMEM * (hh + 1)]
                lhs_os[g][h] = _as_u32(with_mem(orings[g][h, pl.ds(ord_, TOK // 2), :], om))

        acc = [None] * KT

        def out_proj(gs, js):
            for j in js:
                l = jnp.concatenate([_as_bf16(lhs_os[g][k]) for g in gs for k in range(8)], axis=1)
                w = jnp.concatenate(
                    [_as_bf16(wo[j, 64 * _head(g, c, 0):64 * _head(g, c, 0) + 128, :])
                     for g in gs for c in range(4)], axis=0)
                a = _dot(l, w)
                if acc[j] is None:
                    cs = slice(128 * j, 128 * (j + 1))
                    acc[j] = a + jnp.concatenate([xpn_scr[pl.ds(orow, TOK), cs], jnp.zeros((NMEM, 128), f32)], axis=0)
                else:
                    acc[j] = acc[j] + a

        for item in "q0 q1 s0 q2 p0 s1 q3 p1 s2 w01a p2 s3 w012b L0 p3 w2a w3".split():
            g = int(item[1])
            if item[0] == "L":
                nxt = jnp.minimum(s + 1, NSEG - 1)
                ln_rows(pl.multiple_of(PRE + TOK * nxt, 8), TOK, 128, nxt)
            elif item[0] == "w":
                out_proj([int(ch) for ch in item[1:] if ch.isdigit()],
                         {"a": range(4), "b": range(4, 8)}.get(item[-1], range(8)))
            else:
                for c in {"a": range(2), "b": range(2, 4), "x": range(1), "y": range(1, 4), "u": range(3), "v": range(3, 4)}.get(item[-1], range(4)):
                    {"q": qkv, "s": scores, "p": pv}[item[0]](g, c)
        a = jnp.concatenate(acc, axis=1)
        out_stage[pl.ds(orow, TOK), :] = a[:TOK].astype(bf16)
        return _rnd(a[TOK:])

    def body(u, carry):
        mem = step(2 * u, mem_scr[...])
        filler(u)
        mem_scr[...] = step(2 * u + 1, mem)
        orow = pl.multiple_of(out_row(2 * u), 8)
        pltpu.make_async_copy(out_stage.at[pl.ds(orow, 2 * TOK)], out_hbm.at[0, pl.ds(orow, 2 * TOK)],
                              sems.at[SEM_OUT]).start()
        return carry
    with jax.named_scope("chain"):
        lax.fori_loop(0, NSEG // 2, body, 0)

    def out_copy(r0, n, sem):
        return pltpu.make_async_copy(out_stage.at[pl.ds(r0, n)], out_hbm.at[0, pl.ds(r0, n)], sems.at[sem])

    wait_all(wg, SEM_WG)
    wait_all(wu, SEM_WU)
    wait_all(wd, SEM_WD)
    for f in (3, 19, 35):
        out_copy(SEG * f, SEG, SEM_OUT).start()

    rv = racc[...]
    rrow = lax.broadcasted_iota(jnp.int32, rv.shape, 0)
    rlane = lax.broadcasted_iota(jnp.int32, rv.shape, 1)
    ridx = jnp.where(rrow < 128, rrow + 128 * rlane, PRE + (rrow - 128) + TOK * rlane).astype(f32)
    m0 = jnp.max(rv, keepdims=True)
    f0 = jnp.min(jnp.where(rv == m0, ridx, 1e9), keepdims=True)
    rv2 = jnp.where(ridx == f0, -jnp.inf, rv)
    m1 = jnp.max(rv2, keepdims=True)
    f1 = jnp.min(jnp.where(rv2 == m1, ridx, 1e9), keepdims=True)
    i0 = jnp.clip(f0[0, 0].astype(jnp.int32), 0, S - 1)
    i1 = jnp.clip(f1[0, 0].astype(jnp.int32), 0, S - 1)
    row16 = lax.broadcasted_iota(jnp.int32, (16, DM), 0)

    def xn_row(i):
        w = jnp.concatenate([xn_pk[k, pl.ds(i // 2, 1), :] for k in range(KT)], axis=1)
        return pltpu.bitcast(jnp.where(i % 2 == 0, w << 16, w & jnp.uint32(0xFFFF0000)), f32)
    xsel = jnp.where(row16 == 0, xn_row(i0), jnp.where(row16 == 1, xn_row(i1), 0.0)).astype(bf16)

    r51 = 51 * SEG
    for j in (6, 7):
        cs = slice(128 * j, 128 * (j + 1))
        a = _dot(o_rows((r51 % RO) // 2, SEG // 2), _as_bf16(wo[j]))
        out_stage[r51:r51 + SEG, cs] = (a + xpn_scr[r51:r51 + SEG, cs]).astype(bf16)
    out_copy(r51, SEG, SEM_OUT).start()

    e0 = r51 + SEG
    last = S - 128
    part = {}

    def add(key, v):
        part[key] = v if key not in part else v + part[key]

    def e_round(b, j, r):
        l = jnp.concatenate(
            [_as_bf16(orings[(h % 8) // 2][2 * (h // 8) + h % 2, 64 * b:64 * (b + 1), :])
             for h in range(4 * r, 4 * r + 4)], axis=1)
        add(("e", b, j), _dot(l, _as_bf16(wo[j, 256 * r:256 * (r + 1), :])))
        if r == 7:
            rows, cs = slice(e0 + 128 * b, e0 + 128 * (b + 1)), slice(128 * j, 128 * (j + 1))
            out_stage[rows, cs] = (part.pop(("e", b, j)) + xpn_scr[rows, cs]).astype(bf16)
            if j == KT - 1:
                out_copy(e0 + 128 * b, 128, SEM_OUT if b < 2 else SEM_OUT2).start()

    def up_round(w, name, j, r):
        add((name, j), _dot(xsel[:, 512 * r:512 * (r + 1)], _as_bf16(w[j, 256 * r:256 * (r + 1), :])))
        if name == "u" and r == 1:
            gate = part.pop(("g", j))
            part["h", j] = (gate * jax.nn.sigmoid(gate) * part.pop(("u", j))).astype(bf16)

    def down_round(j, r):
        hid = jnp.concatenate([part["h", k] for k in range(4 * r, 4 * r + 4)], axis=1)
        add(("y", j), _dot(hid, _as_bf16(wd[j, 256 * r:256 * (r + 1), :])))

    e_rounds = [(b, j, r) for b in range(3) for j in range(KT) for r in range(8)]
    m_rounds = [lambda j=j, r=r, w=w, n=n: up_round(w, n, j, r)
                for j in range(FT) for (w, n) in ((wg, "g"), (wu, "u")) for r in range(2)]
    m_rounds += [None] * 4
    m_rounds += [lambda j=j, r=r: down_round(j, r) for r in range(FT // 4) for j in range(KT)]
    m_rounds = [None] * 8 + m_rounds
    NM = 2
    for n, er in enumerate(e_rounds[:128]):
        e_round(*er)
        for mr in m_rounds[NM * n:NM * n + NM]:
            if mr is not None:
                mr()
    assert len(m_rounds) <= NM * 128
    rsel = jnp.where(lax.broadcasted_iota(jnp.int32, (16, 1), 0) == 0, m0, m1)
    y = jnp.concatenate([part.pop(("y", j)) for j in range(KT)], axis=1) * jax.nn.sigmoid(rsel)
    y0, y1 = y[0:1], y[1:2]
    xpn_scr[pl.ds(i0, 1), :] = xpn_scr[pl.ds(i0, 1), :] + jnp.where(i0 >= last, y0, 0.0)
    xpn_scr[pl.ds(i1, 1), :] = xpn_scr[pl.ds(i1, 1), :] + jnp.where(i1 >= last, y1, 0.0)
    for er in e_rounds[128:]:
        e_round(*er)

    with jax.named_scope("wait_out"):
        wait_all(out_stage.at[pl.ds(0, last)], SEM_OUT)
    g0 = pl.multiple_of((i0 // 16) * 16, 16)
    g1 = pl.multiple_of((i1 // 16) * 16, 16)
    redo0 = i0 < last
    redo1 = i1 < last
    send1 = jnp.logical_and(redo1, g1 != g0)

    def patch(i, gst, yy):
        blk = out_stage[pl.ds(gst, 16), :].astype(f32)
        out_stage[pl.ds(gst, 16), :] = (blk + jnp.where(row16 == i - gst, yy, 0.0)).astype(bf16)

    @pl.when(redo0)
    def _():
        patch(i0, g0, y0)

    @pl.when(redo1)
    def _():
        patch(i1, g1, y1)

    @pl.when(redo0)
    def _():
        out_copy(g0, 16, SEM_P0).start()

    @pl.when(send1)
    def _():
        out_copy(g1, 16, SEM_P1).start()

    with jax.named_scope("wait_out2"):
        out_copy(last, 128, SEM_OUT2).wait()

    @pl.when(redo0)
    def _():
        out_copy(g0, 16, SEM_P0).wait()

    @pl.when(send1)
    def _():
        out_copy(g1, 16, SEM_P1).wait()


@jax.jit
def pallas_parallel_sum__memory_aug_recurrent_mem_tr__moe_arch_mod__prompt_kernel(
    A_x: jax.Array,
    A_mem0: jax.Array,
    A_Wq: jax.Array,
    A_Wk: jax.Array,
    A_Wv: jax.Array,
    A_Wo: jax.Array,
    A_seg_len: jax.Array,
    B_x: jax.Array,
    B_w_r: jax.Array,
    B_w_gate: jax.Array,
    B_w_up: jax.Array,
    B_w_down: jax.Array,
):
    del A_seg_len, B_x
    assert A_x.shape == (1, S, DM) and A_mem0.shape == (1, NMEM, DM)
    assert A_Wq.shape == (DM, H, DH) and A_Wo.shape == (H, DH, DM) and B_w_gate.shape == (DM, FF)
    hbm = pl.BlockSpec(memory_space=pl.ANY)
    vmem = pl.BlockSpec(memory_space=pltpu.VMEM)
    scratch = [
        pltpu.VMEM((S, DM), bf16),
        pltpu.VMEM((S, DM), f32),
        pltpu.VMEM((KT, S // 2, 128), u32),
        pltpu.VMEM((16, DM), f32),
        pltpu.VMEM((4, DM // 2, 8, 128), u32),
        pltpu.VMEM((3 * H, DM // 2, 128), u32),
        pltpu.VMEM((KT, H * DH // 2, 128), u32),
    ]
    scratch += [pltpu.VMEM((24, RQ // 2, 128), u32)] * NG
    scratch += [pltpu.VMEM((8, RO // 2, 128), u32)] * NG
    scratch += [pltpu.VMEM((8, 16, 128), u32)] * NG
    scratch += [
        pltpu.VMEM((NMEM, DM), f32),
        pltpu.VMEM((16, 128), u32),
        pltpu.VMEM((L2, LK), f32),
        pltpu.VMEM((128 + TOK, 128), f32),
        pltpu.VMEM((FT, DM // 2, 128), u32),
        pltpu.VMEM((FT, DM // 2, 128), u32),
        pltpu.VMEM((KT, FF // 2, 128), u32),
        pltpu.VMEM((S, DM), bf16),
        pltpu.SemaphoreType.DMA((NSEM,)),
    ]
    return pl.pallas_call(
        _kernel,
        out_shape=jax.ShapeDtypeStruct((1, S, DM), bf16),
        in_specs=[hbm, vmem, hbm, hbm, hbm, hbm, vmem, hbm, hbm, hbm],
        out_specs=hbm,
        scratch_shapes=scratch,
        compiler_params=pltpu.CompilerParams(vmem_limit_bytes=124 * 1024 * 1024,
                                             disable_bounds_checks=True),
    )(A_x, A_mem0, *[w.reshape(DM // 2, 2, H, DH) for w in (A_Wq, A_Wk, A_Wv)], A_Wo.reshape(H * DH, DM), B_w_r, B_w_gate, B_w_up, B_w_down)
```

```python
import jax
import jax.numpy as jnp
from jax import lax
import jax.experimental.pallas as pl
import jax.experimental.pallas.tpu as pltpu

bf16 = jnp.bfloat16
f32 = jnp.float32
u32 = jnp.uint32

S, DM, H, DH, NMEM, SEG, FF = 2048, 1024, 32, 128, 8, 32, 3584
NSEG = S // SEG
TOK = 24
PRE = S - NSEG * TOK
RQ = 544
RO = 832
NG = 4
KT = DM // 128
FT = FF // 128
L2 = 2 * (SEG + NMEM)
LOG2E = 1.4426950408889634
SCALE = DH ** -0.5 * LOG2E
PADK = 0
LK = 128 if PADK else L2
EPS_BF16 = 1.0013580322265625e-05

SEM_W0 = 0
SEM_X0 = 9
SEM_XB, SEM_XC, SEM_WO, SEM_FFN, SEM_OUT, SEM_P0, SEM_P1, SEM_OUT2 = range(13, 21)
NSEM = 21
G0, U0, D0 = 0, FT * DM // 2, 2 * FT * DM // 2
FFN_ROWS = D0 + KT * FF // 2


def _as_bf16(x):
    return pltpu.bitcast(x, bf16)


def _as_u32(x):
    return pltpu.bitcast(x, u32)


def _rnd(x):
    return x.astype(bf16).astype(f32)


def _dot(a, b):
    return jnp.dot(a, b, preferred_element_type=f32)


def _head(g, c, hh):
    return 8 * c + 2 * g + hh


def _kernel(x_hbm, mem0_ref, wq_hbm, wk_hbm, wv_hbm, wo_hbm, wr_ref, wg_hbm, wu_hbm, wd_hbm,
            out_hbm,
            x_scr, xpn_scr, xn_pk, wr_scr, pool, wqkv, wo,
            qr0, qr1, qr2, qr3, or0, or1, or2, or3, lo0, lo1, lo2, lo3,
            mem_scr, zero_scr, fill_scr, racc, out_stage, sems):
    qrings = (qr0, qr1, qr2, qr3)
    orings = (or0, or1, or2, or3)
    lhs_os = (lo0, lo1, lo2, lo3)
    w32 = [w.bitcast(u32) for w in (wq_hbm, wk_hbm, wv_hbm)]
    wo32 = wo_hbm.bitcast(u32)
    wg32 = wg_hbm.bitcast(u32)
    wu32 = wu_hbm.bitcast(u32)
    wd32 = wd_hbm.bitcast(u32)

    def x_copy(r0, n, sem):
        return pltpu.make_async_copy(x_hbm.at[0, pl.ds(r0, n)], x_scr.at[pl.ds(r0, n)], sems.at[sem])

    def w_start(lo, hi, sem):
        for p in range(lo, hi):
            pltpu.make_async_copy(w32[p // 16].at[:, p % 16, :], pool.at[pl.ds(DM * p, DM)],
                                  sems.at[SEM_W0 + sem]).start()

    def w_wait(n, sem):
        wait_all(pool.at[pl.ds(0, DM * n)], SEM_W0 + sem)

    def col_tiles_start(src, dst_of, sem, n):
        for j in range(n):
            pltpu.make_async_copy(src.at[:, pl.ds(128 * j, 128)], dst_of(j), sems.at[sem]).start()

    def wait_all(buf, sem):
        pltpu.make_async_copy(buf, buf, sems.at[sem]).wait()

    for c in range(4):
        x_copy(128 * c, 128, SEM_X0 + c).start()
    w_start(0, 1, 0)
    w_start(1, 2, 1)
    w_start(2, 4, 2)
    w_start(4, 8, 3)
    x_copy(PRE, TOK, SEM_XC).start()
    for i in range(5):
        w_start(8 + 8 * i, 16 + 8 * i, 4 + i)
    x_copy(PRE + TOK, S - PRE - TOK, SEM_XB).start()
    col_tiles_start(wo32, lambda j: wo.at[j], SEM_WO, KT)

    mem_scr[...] = mem0_ref[0].astype(f32)
    zero_scr[...] = jnp.zeros(zero_scr.shape, u32)
    wr_row = wr_ref[...].astype(f32).reshape(1, DM)
    wr_scr[0:8, :] = jnp.broadcast_to(wr_row, (8, DM))
    wr_scr[8:16, :] = jnp.broadcast_to(jnp.sum(wr_row, axis=-1, keepdims=True), (8, DM))
    racc[...] = jnp.full(racc.shape, -jnp.inf, f32)
    qi = lax.broadcasted_iota(jnp.int32, (L2, LK), 0)
    ki = lax.broadcasted_iota(jnp.int32, (L2, LK), 1)
    q_mem, k_mem = qi >= 2 * SEG, ki >= 2 * SEG
    q_head = jnp.where(q_mem, (qi - 2 * SEG) // NMEM, qi // SEG)
    k_head = jnp.where(k_mem, (ki - 2 * SEG) // NMEM, ki // SEG)
    visible = q_mem | k_mem | (qi >= ki)
    fill_scr[...] = jnp.where(q_head == k_head, jnp.where(visible, 0.0, -1e9 * LOG2E), -jnp.inf).astype(f32)

    def ln_rows(r0, n, racc_row, lane_id):
        lane = lax.broadcasted_iota(jnp.int32, (n, 128), 1)
        wr = jnp.concatenate([wr_scr[0:8, :]] * (n // 8), axis=0)
        wr_sum = jnp.concatenate([wr_scr[8:16, 0:1]] * (n // 8), axis=0)
        x = x_scr[pl.ds(r0, n), :].astype(f32)
        mean = jnp.sum(x, axis=-1, keepdims=True) * (1.0 / DM)
        msq = jnp.sum(x * x, axis=-1, keepdims=True) * (1.0 / DM)
        xw = jnp.sum(x * wr, axis=-1, keepdims=True)
        var = jnp.maximum(msq - mean * mean, 0.0)
        inv = 1.0 / _rnd(jnp.sqrt(_rnd(_rnd(var) + EPS_BF16)))
        mean = _rnd(mean)
        xnb = ((x - mean) * inv).astype(bf16)
        xpn_scr[pl.ds(r0, n), :] = x + xnb.astype(f32)
        xnp = _as_u32(xnb)
        p0 = r0 // 2 if isinstance(r0, int) else pl.multiple_of(r0 // 2, 4)
        for k in range(KT):
            xn_pk[k, pl.ds(p0, n // 2), :] = xnp[:, 128 * k:128 * (k + 1)]
        r = _rnd((xw - mean * wr_sum) * inv)
        racc[racc_row:racc_row + n, :] = jnp.where(lane == lane_id, r, racc[racc_row:racc_row + n, :])

    def ln_chunk(c):
        for i in range(8):
            ln_rows(pl.multiple_of(c * 128 + 16 * i, 16), 16, 16 * i, c)

    def ln_first(c, carry):
        r0 = pl.multiple_of(128 * c, 128)
        pltpu.make_async_copy(x_hbm.at[0, pl.ds(r0, 128)], x_scr.at[pl.ds(r0, 128)], sems.at[SEM_X0 + c]).wait()
        ln_chunk(c)
        return carry
    with jax.named_scope("ln_first"):
        lax.fori_loop(0, PRE // 128, ln_first, 0)

    def pro_pairs(t, gs):
        m, c8 = t // 4, t % 4
        sc = (SCALE if m == 0 else None) if isinstance(t, int) else jnp.where(m == 0, SCALE, 1.0).astype(f32)
        for g in gs:
            p0 = DM * (4 * t + g)
            both = pool[pl.ds(p0 if isinstance(t, int) else pl.multiple_of(p0, DM), DM), :]
            pair = (pltpu.bitcast(both << 16, f32).astype(bf16),
                    pltpu.bitcast(both & jnp.uint32(0xFFFF0000), f32).astype(bf16))
            for hh in range(2):
                wqkv[_head(g, c8, hh) * 3 + m] = _as_u32(pair[hh])
                lhs = jnp.concatenate([_as_bf16(xn_pk[k, 0:PRE // 2, :]) for k in range(KT)], axis=1)
                y = _dot(lhs, pair[hh])
                if sc is not None:
                    y = y * sc
                qrings[g][(2 * c8 + hh) * 3 + m, 0:PRE // 2, :] = _as_u32(y.astype(bf16))

    with jax.named_scope("pro_a"):
        w_wait(1, 0)
        pro_pairs(0, (0,))
    with jax.named_scope("pro_a2"):
        w_wait(1, 1)
        pro_pairs(0, (1,))
    with jax.named_scope("pro_b"):
        w_wait(2, 2)
        pro_pairs(0, (2, 3))
    with jax.named_scope("pro_c"):
        w_wait(4, 3)
        x_copy(PRE, TOK, SEM_XC).wait()
        pro_pairs(1, range(NG))
        ln_rows(PRE, TOK, 128, 0)
        for g in range(NG):
            orings[g][:, 48:64, :] = jnp.zeros((8, 16, 128), u32)

    def pro_body(i, carry):
        w_wait(8, 4 + i)
        pro_pairs(2 + 2 * i, range(NG))
        pro_pairs(3 + 2 * i, range(NG))
        return carry
    with jax.named_scope("prologue"):
        lax.fori_loop(0, 5, pro_body, 0)
    with jax.named_scope("wait_wo"):
        wait_all(wo, SEM_WO)
        x_copy(PRE + TOK, S - PRE - TOK, SEM_XB).wait()
    col_tiles_start(wg32, lambda j: pool.at[pl.ds(G0 + 512 * j, 512)], SEM_FFN, FT)
    col_tiles_start(wu32, lambda j: pool.at[pl.ds(U0 + 512 * j, 512)], SEM_FFN, FT)
    col_tiles_start(wd32, lambda j: pool.at[pl.ds(D0 + FF // 2 * j, FF // 2)], SEM_FFN, KT)

    def out_row(s):
        return TOK * s + SEG * ((s + 16) // 20)

    def o_rows(pos, n):
        return jnp.concatenate(
            [_as_bf16(orings[(h % 8) // 2][2 * (h // 8) + h % 2, pl.ds(pos, n), :]) for h in range(H)], axis=1)

    def filler(u):
        k = jnp.maximum(u - 2, 0)
        j = k % 8
        r0 = pl.multiple_of(SEG * (16 * (k // 8) + 3), SEG)
        pos = pl.multiple_of(lax.rem(r0, RO) // 2, 16)
        cs = pl.ds(pl.multiple_of(128 * j, 128), 128)
        a = _dot(o_rows(pos, SEG // 2), _as_bf16(wo[j]))
        out_stage[pl.ds(r0, SEG), cs] = (a + xpn_scr[pl.ds(r0, SEG), cs]).astype(bf16)

    def step(s, mem_in):
        xpos = pl.multiple_of((PRE + TOK * s) // 2, 4)
        wr_pos = [pl.multiple_of(lax.rem(PRE + TOK * s + 8 * i, RQ) // 2, 4) for i in range(3)]
        rd = pl.multiple_of(lax.rem(SEG * s, RQ) // 2, 16)
        owr = pl.multiple_of(lax.rem(SEG * s, RO) // 2, 16)
        orow = pl.multiple_of(out_row(s), 8)
        ord_ = pl.multiple_of(lax.rem(orow, RO) // 2, 4)
        def with_mem(tok_u32, mem_rows):
            tok = _as_bf16(tok_u32)
            last = jnp.concatenate([tok[16:TOK].astype(f32), mem_rows], axis=0).astype(bf16)
            return jnp.concatenate([tok[0:16], last], axis=0)

        zero = zero_scr[0:TOK // 2, :]
        lhs = jnp.concatenate(
            [with_mem(xn_pk[k, pl.ds(xpos, TOK // 2), :] ^ zero, mem_in[:, 128 * k:128 * (k + 1)])
             for k in range(KT)], axis=1)

        mem_parts, probs = {}, {}

        def qkv(g, c):
            res = []
            for m in range(3):
                ms = []
                for hh in range(2):
                    y = _dot(lhs, _as_bf16(wqkv[_head(g, c, hh) * 3 + m]))
                    if m == 0:
                        y = y * SCALE
                    yp = _as_u32(y.astype(bf16))
                    for i in range(3):
                        qrings[g][(2 * c + hh) * 3 + m, pl.ds(wr_pos[i], 4), :] = yp[4 * i:4 * i + 4]
                    ms.append(y[TOK:])
                res.append(jnp.concatenate(ms, axis=0).astype(bf16))
            mem_parts[g, c] = res

        def pair_rows(g, c, m, mem_rows):
            t0 = _as_bf16(qrings[g][(2 * c) * 3 + m, pl.ds(rd, SEG // 2), :])
            t1 = _as_bf16(qrings[g][(2 * c + 1) * 3 + m, pl.ds(rd, SEG // 2), :])
            pad = [jnp.zeros((LK - L2, 128), bf16)] if (m > 0 and LK > L2) else []
            return jnp.concatenate([t0, t1, mem_rows] + pad, axis=0)

        def scores(g, c):
            qm, km, vm = mem_parts.pop((g, c))
            sc = lax.dot_general(pair_rows(g, c, 0, qm), pair_rows(g, c, 1, km),
                                 (((1,), (1,)), ((), ())), preferred_element_type=f32)
            fill = fill_scr[...]
            sc = jnp.where(fill == 0.0, sc, fill)
            e = jnp.exp2(sc - jnp.max(sc, axis=-1, keepdims=True))
            r = pl.reciprocal(jnp.sum(e, axis=-1, keepdims=True), approx=True)
            probs[g, c] = (e.astype(bf16), r, vm)

        def pv(g, c):
            e, r, vm = probs.pop((g, c))
            o = _dot(e, pair_rows(g, c, 2, vm)) * r
            for hh in range(2):
                h = 2 * c + hh
                orings[g][h, pl.ds(owr, SEG // 2), :] = _as_u32(o[SEG * hh:SEG * (hh + 1)].astype(bf16))
                om = o[2 * SEG + NMEM * hh:2 * SEG + NMEM * (hh + 1)]
                lhs_os[g][h] = _as_u32(with_mem(orings[g][h, pl.ds(ord_, TOK // 2), :], om))

        acc = [None] * KT

        def out_proj(gs, js):
            for j in js:
                l = jnp.concatenate([_as_bf16(lhs_os[g][k]) for g in gs for k in range(8)], axis=1)
                w = jnp.concatenate(
                    [_as_bf16(wo[j, 64 * _head(g, c, 0):64 * _head(g, c, 0) + 128, :])
                     for g in gs for c in range(4)], axis=0)
                a = _dot(l, w)
                if acc[j] is None:
                    cs = slice(128 * j, 128 * (j + 1))
                    acc[j] = a + jnp.concatenate([xpn_scr[pl.ds(orow, TOK), cs], jnp.zeros((NMEM, 128), f32)], axis=0)
                else:
                    acc[j] = acc[j] + a

        for item in "q0 q1 s0 q2 p0 s1 q3 p1 s2 w01a p2 s3 w012b L0 p3 w2a w3".split():
            g = int(item[1])
            if item[0] == "L":
                nxt = jnp.minimum(s + 1, NSEG - 1)
                ln_rows(pl.multiple_of(PRE + TOK * nxt, 8), TOK, 128, nxt)
            elif item[0] == "w":
                out_proj([int(ch) for ch in item[1:] if ch.isdigit()],
                         {"a": range(4), "b": range(4, 8)}.get(item[-1], range(8)))
            else:
                for c in {"a": range(2), "b": range(2, 4), "x": range(1), "y": range(1, 4), "u": range(3), "v": range(3, 4)}.get(item[-1], range(4)):
                    {"q": qkv, "s": scores, "p": pv}[item[0]](g, c)
        a = jnp.concatenate(acc, axis=1)
        out_stage[pl.ds(orow, TOK), :] = a[:TOK].astype(bf16)
        return _rnd(a[TOK:])

    def body(u, carry):
        mem = step(2 * u, mem_scr[...])
        filler(u)
        mem_scr[...] = step(2 * u + 1, mem)
        orow = pl.multiple_of(out_row(2 * u), 8)
        pltpu.make_async_copy(out_stage.at[pl.ds(orow, 2 * TOK)], out_hbm.at[0, pl.ds(orow, 2 * TOK)],
                              sems.at[SEM_OUT]).start()
        return carry
    with jax.named_scope("chain"):
        lax.fori_loop(0, NSEG // 2, body, 0)

    def out_copy(r0, n, sem):
        return pltpu.make_async_copy(out_stage.at[pl.ds(r0, n)], out_hbm.at[0, pl.ds(r0, n)], sems.at[sem])

    wait_all(pool.at[pl.ds(0, FFN_ROWS)], SEM_FFN)
    for f in (3, 19, 35):
        out_copy(SEG * f, SEG, SEM_OUT).start()

    rv = racc[...]
    rrow = lax.broadcasted_iota(jnp.int32, rv.shape, 0)
    rlane = lax.broadcasted_iota(jnp.int32, rv.shape, 1)
    ridx = jnp.where(rrow < 128, rrow + 128 * rlane, PRE + (rrow - 128) + TOK * rlane).astype(f32)
    m0 = jnp.max(rv, keepdims=True)
    f0 = jnp.min(jnp.where(rv == m0, ridx, 1e9), keepdims=True)
    rv2 = jnp.where(ridx == f0, -jnp.inf, rv)
    m1 = jnp.max(rv2, keepdims=True)
    f1 = jnp.min(jnp.where(rv2 == m1, ridx, 1e9), keepdims=True)
    i0 = jnp.clip(f0[0, 0].astype(jnp.int32), 0, S - 1)
    i1 = jnp.clip(f1[0, 0].astype(jnp.int32), 0, S - 1)
    row16 = lax.broadcasted_iota(jnp.int32, (16, DM), 0)

    def xn_row(i):
        w = jnp.concatenate([xn_pk[k, pl.ds(i // 2, 1), :] for k in range(KT)], axis=1)
        return pltpu.bitcast(jnp.where(i % 2 == 0, w << 16, w & jnp.uint32(0xFFFF0000)), f32)
    xsel = jnp.where(row16 == 0, xn_row(i0), jnp.where(row16 == 1, xn_row(i1), 0.0)).astype(bf16)

    r51 = 51 * SEG
    for j in (6, 7):
        cs = slice(128 * j, 128 * (j + 1))
        a = _dot(o_rows((r51 % RO) // 2, SEG // 2), _as_bf16(wo[j]))
        out_stage[r51:r51 + SEG, cs] = (a + xpn_scr[r51:r51 + SEG, cs]).astype(bf16)
    out_copy(r51, SEG, SEM_OUT).start()

    e0 = r51 + SEG
    last = S - 128
    part = {}

    def add(key, v):
        part[key] = v if key not in part else v + part[key]

    def e_round(b, j, r):
        l = jnp.concatenate(
            [_as_bf16(orings[(h % 8) // 2][2 * (h // 8) + h % 2, 64 * b:64 * (b + 1), :])
             for h in range(4 * r, 4 * r + 4)], axis=1)
        add(("e", b, j), _dot(l, _as_bf16(wo[j, 256 * r:256 * (r + 1), :])))
        if r == 7:
            rows, cs = slice(e0 + 128 * b, e0 + 128 * (b + 1)), slice(128 * j, 128 * (j + 1))
            out_stage[rows, cs] = (part.pop(("e", b, j)) + xpn_scr[rows, cs]).astype(bf16)
            if j == KT - 1:
                out_copy(e0 + 128 * b, 128, SEM_OUT if b < 2 else SEM_OUT2).start()

    def up_round(w, name, j, r):
        add((name, j), _dot(xsel[:, 512 * r:512 * (r + 1)], _as_bf16(pool[pl.ds(w + 512 * j + 256 * r, 256), :])))
        if name == "u" and r == 1:
            gate = part.pop(("g", j))
            part["h", j] = (gate * jax.nn.sigmoid(gate) * part.pop(("u", j))).astype(bf16)

    def down_round(j, r):
        hid = jnp.concatenate([part["h", k] for k in range(4 * r, 4 * r + 4)], axis=1)
        add(("y", j), _dot(hid, _as_bf16(pool[pl.ds(D0 + FF // 2 * j + 256 * r, 256), :])))

    e_rounds = [(b, j, r) for b in range(3) for j in range(KT) for r in range(8)]
    m_rounds = [lambda j=j, r=r, w=w, n=n: up_round(w, n, j, r)
                for j in range(FT) for (w, n) in ((G0, "g"), (U0, "u")) for r in range(2)]
    m_rounds += [None] * 4
    m_rounds += [lambda j=j, r=r: down_round(j, r) for r in range(FT // 4) for j in range(KT)]
    m_rounds = [None] * 8 + m_rounds
    NM = 2
    for n, er in enumerate(e_rounds[:128]):
        e_round(*er)
        for mr in m_rounds[NM * n:NM * n + NM]:
            if mr is not None:
                mr()
    assert len(m_rounds) <= NM * 128
    rsel = jnp.where(lax.broadcasted_iota(jnp.int32, (16, 1), 0) == 0, m0, m1)
    y = jnp.concatenate([part.pop(("y", j)) for j in range(KT)], axis=1) * jax.nn.sigmoid(rsel)
    y0, y1 = y[0:1], y[1:2]
    xpn_scr[pl.ds(i0, 1), :] = xpn_scr[pl.ds(i0, 1), :] + jnp.where(i0 >= last, y0, 0.0)
    xpn_scr[pl.ds(i1, 1), :] = xpn_scr[pl.ds(i1, 1), :] + jnp.where(i1 >= last, y1, 0.0)
    for er in e_rounds[128:]:
        e_round(*er)

    with jax.named_scope("wait_out"):
        wait_all(out_stage.at[pl.ds(0, last)], SEM_OUT)
    g0 = pl.multiple_of((i0 // 16) * 16, 16)
    g1 = pl.multiple_of((i1 // 16) * 16, 16)
    redo0 = i0 < last
    redo1 = i1 < last
    send1 = jnp.logical_and(redo1, g1 != g0)

    def patch(i, gst, yy):
        blk = out_stage[pl.ds(gst, 16), :].astype(f32)
        out_stage[pl.ds(gst, 16), :] = (blk + jnp.where(row16 == i - gst, yy, 0.0)).astype(bf16)

    @pl.when(redo0)
    def _():
        patch(i0, g0, y0)

    @pl.when(redo1)
    def _():
        patch(i1, g1, y1)

    @pl.when(redo0)
    def _():
        out_copy(g0, 16, SEM_P0).start()

    @pl.when(send1)
    def _():
        out_copy(g1, 16, SEM_P1).start()

    with jax.named_scope("wait_out2"):
        out_copy(last, 128, SEM_OUT2).wait()

    @pl.when(redo0)
    def _():
        out_copy(g0, 16, SEM_P0).wait()

    @pl.when(send1)
    def _():
        out_copy(g1, 16, SEM_P1).wait()


@jax.jit
def pallas_parallel_sum__memory_aug_recurrent_mem_tr__moe_arch_mod__prompt_kernel(
    A_x: jax.Array,
    A_mem0: jax.Array,
    A_Wq: jax.Array,
    A_Wk: jax.Array,
    A_Wv: jax.Array,
    A_Wo: jax.Array,
    A_seg_len: jax.Array,
    B_x: jax.Array,
    B_w_r: jax.Array,
    B_w_gate: jax.Array,
    B_w_up: jax.Array,
    B_w_down: jax.Array,
):
    del A_seg_len, B_x
    assert A_x.shape == (1, S, DM) and A_mem0.shape == (1, NMEM, DM)
    assert A_Wq.shape == (DM, H, DH) and A_Wo.shape == (H, DH, DM) and B_w_gate.shape == (DM, FF)
    hbm = pl.BlockSpec(memory_space=pl.ANY)
    vmem = pl.BlockSpec(memory_space=pltpu.VMEM)
    scratch = [
        pltpu.VMEM((S, DM), bf16),
        pltpu.VMEM((S, DM), f32),
        pltpu.VMEM((KT, S // 2, 128), u32),
        pltpu.VMEM((16, DM), f32),
        pltpu.VMEM((48 * DM, 128), u32),
        pltpu.VMEM((3 * H, DM // 2, 128), u32),
        pltpu.VMEM((KT, H * DH // 2, 128), u32),
    ]
    scratch += [pltpu.VMEM((24, RQ // 2, 128), u32)] * NG
    scratch += [pltpu.VMEM((8, RO // 2, 128), u32)] * NG
    scratch += [pltpu.VMEM((8, 16, 128), u32)] * NG
    scratch += [
        pltpu.VMEM((NMEM, DM), f32),
        pltpu.VMEM((16, 128), u32),
        pltpu.VMEM((L2, LK), f32),
        pltpu.VMEM((128 + TOK, 128), f32),
        pltpu.VMEM((S, DM), bf16),
        pltpu.SemaphoreType.DMA((NSEM,)),
    ]
    return pl.pallas_call(
        _kernel,
        out_shape=jax.ShapeDtypeStruct((1, S, DM), bf16),
        in_specs=[hbm, vmem, hbm, hbm, hbm, hbm, vmem, hbm, hbm, hbm],
        out_specs=hbm,
        scratch_shapes=scratch,
        compiler_params=pltpu.CompilerParams(vmem_limit_bytes=124 * 1024 * 1024,
                                             disable_bounds_checks=True),
    )(A_x, A_mem0, A_Wq, A_Wk, A_Wv, A_Wo.reshape(H * DH, DM), B_w_r, B_w_gate, B_w_up, B_w_down)
```

```python
import jax
import jax.numpy as jnp
from jax import lax
import jax.experimental.pallas as pl
import jax.experimental.pallas.tpu as pltpu

bf16 = jnp.bfloat16
f32 = jnp.float32
u32 = jnp.uint32

S, DM, H, DH, NMEM, SEG, FF = 2048, 1024, 32, 128, 8, 32, 3584
NSEG = S // SEG
TOK = 24
PRE = S - NSEG * TOK
RQ = 544
RO = 832
NG = 4
KT = DM // 128
FT = FF // 128
L2 = 2 * (SEG + NMEM)
LOG2E = 1.4426950408889634
SCALE = DH ** -0.5 * LOG2E
PADK = 0
LK = 128 if PADK else L2
EPS_BF16 = 1.0013580322265625e-05

SEM_W0 = 0
SEM_X0 = 9
SEM_XB, SEM_XC, SEM_WO, SEM_FFN, SEM_OUT, SEM_P0, SEM_P1, SEM_OUT2 = range(13, 21)
NSEM = 21
G0, U0, D0 = 0, FT * DM // 2, 2 * FT * DM // 2
FFN_ROWS = D0 + KT * FF // 2


def _as_bf16(x):
    return pltpu.bitcast(x, bf16)


def _as_u32(x):
    return pltpu.bitcast(x, u32)


def _rnd(x):
    return x.astype(bf16).astype(f32)


def _dot(a, b):
    return jnp.dot(a, b, preferred_element_type=f32)


def _head(g, c, hh):
    return 8 * c + 2 * g + hh


def _kernel(x_hbm, mem0_ref, wq_hbm, wk_hbm, wv_hbm, wo_hbm, wr_ref, wg_hbm, wu_hbm, wd_hbm,
            out_hbm,
            x_scr, xpn_scr, xn_pk, wr_scr, pool, wqkv, wo,
            qr0, qr1, qr2, qr3, or0, or1, or2, or3, lo0, lo1, lo2, lo3,
            mem_scr, zero_scr, fill_scr, racc, out_stage, sems):
    qrings = (qr0, qr1, qr2, qr3)
    orings = (or0, or1, or2, or3)
    lhs_os = (lo0, lo1, lo2, lo3)
    w32 = [w.bitcast(u32) for w in (wq_hbm, wk_hbm, wv_hbm)]
    wo32 = wo_hbm.bitcast(u32)
    wg32 = wg_hbm.bitcast(u32)
    wu32 = wu_hbm.bitcast(u32)
    wd32 = wd_hbm.bitcast(u32)

    def x_copy(r0, n, sem):
        return pltpu.make_async_copy(x_hbm.at[0, pl.ds(r0, n)], x_scr.at[pl.ds(r0, n)], sems.at[sem])

    def out_copy(r0, n, sem):
        return pltpu.make_async_copy(out_stage.at[pl.ds(r0, n)], out_hbm.at[0, pl.ds(r0, n)], sems.at[sem])

    def w_start(lo, hi, sem):
        for p in range(lo, hi):
            pltpu.make_async_copy(w32[p // 16].at[:, p % 16, :], pool.at[pl.ds(DM * p, DM)],
                                  sems.at[SEM_W0 + sem]).start()

    def w_wait(lo, n, sem):
        r0 = DM * lo if isinstance(lo, int) else pl.multiple_of(DM * lo, DM)
        wait_all(pool.at[pl.ds(r0, DM * n)], SEM_W0 + sem)

    def col_tiles_start(src, dst_of, sem, n):
        for j in range(n):
            pltpu.make_async_copy(src.at[:, pl.ds(128 * j, 128)], dst_of(j), sems.at[sem]).start()

    def wait_all(buf, sem):
        pltpu.make_async_copy(buf, buf, sems.at[sem]).wait()

    for c in range(4):
        x_copy(128 * c, 128, SEM_X0 + c).start()
    w_start(0, 1, 0)
    w_start(1, 2, 1)
    w_start(2, 4, 2)
    w_start(4, 8, 3)
    x_copy(PRE, SEG, SEM_XC).start()
    for i in range(5):
        w_start(8 + 8 * i, 16 + 8 * i, 4 + i)
    x_copy(PRE + SEG, S - PRE - SEG, SEM_XB).start()
    col_tiles_start(wo32, lambda j: wo.at[j], SEM_WO, KT)

    mem_scr[...] = mem0_ref[0].astype(f32)
    zero_scr[...] = jnp.zeros(zero_scr.shape, u32)
    wr_row = wr_ref[...].astype(f32).reshape(1, DM)
    wr_scr[0:8, :] = jnp.broadcast_to(wr_row, (8, DM))
    wr_scr[8:16, :] = jnp.broadcast_to(jnp.sum(wr_row, axis=-1, keepdims=True), (8, DM))
    racc[...] = jnp.full(racc.shape, -jnp.inf, f32)
    qi = lax.broadcasted_iota(jnp.int32, (L2, LK), 0)
    ki = lax.broadcasted_iota(jnp.int32, (L2, LK), 1)
    q_mem, k_mem = qi >= 2 * SEG, ki >= 2 * SEG
    q_head = jnp.where(q_mem, (qi - 2 * SEG) // NMEM, qi // SEG)
    k_head = jnp.where(k_mem, (ki - 2 * SEG) // NMEM, ki // SEG)
    visible = q_mem | k_mem | (qi >= ki)
    fill_scr[...] = jnp.where(q_head == k_head, jnp.where(visible, 0.0, -1e9 * LOG2E), -jnp.inf).astype(f32)

    def ln_rows(r0, n, racc_row, lane_id):
        lane = lax.broadcasted_iota(jnp.int32, (n, 128), 1)
        wr = jnp.concatenate([wr_scr[0:8, :]] * (n // 8), axis=0)
        wr_sum = jnp.concatenate([wr_scr[8:16, 0:1]] * (n // 8), axis=0)
        x = x_scr[pl.ds(r0, n), :].astype(f32)
        mean = jnp.sum(x, axis=-1, keepdims=True) * (1.0 / DM)
        msq = jnp.sum(x * x, axis=-1, keepdims=True) * (1.0 / DM)
        xw = jnp.sum(x * wr, axis=-1, keepdims=True)
        var = jnp.maximum(msq - mean * mean, 0.0)
        inv = 1.0 / _rnd(jnp.sqrt(_rnd(_rnd(var) + EPS_BF16)))
        mean = _rnd(mean)
        xnb = ((x - mean) * inv).astype(bf16)
        xpn_scr[pl.ds(r0, n), :] = x + xnb.astype(f32)
        xnp = _as_u32(xnb)
        p0 = r0 // 2 if isinstance(r0, int) else pl.multiple_of(r0 // 2, 4)
        for k in range(KT):
            xn_pk[k, pl.ds(p0, n // 2), :] = xnp[:, 128 * k:128 * (k + 1)]
        r = _rnd((xw - mean * wr_sum) * inv)
        racc[racc_row:racc_row + n, :] = jnp.where(lane == lane_id, r, racc[racc_row:racc_row + n, :])

    def ln_first(c, carry):
        x_copy(pl.multiple_of(128 * c, 128), 128, SEM_X0 + c).wait()
        for i in range(8):
            ln_rows(pl.multiple_of(c * 128 + 16 * i, 16), 16, 16 * i, c)
        return carry
    lax.fori_loop(0, PRE // 128, ln_first, 0)

    def pro_pairs(t, gs):
        m, c8 = t // 4, t % 4
        sc = (SCALE if m == 0 else None) if isinstance(t, int) else jnp.where(m == 0, SCALE, 1.0).astype(f32)
        for g in gs:
            p0 = DM * (4 * t + g)
            both = pool[pl.ds(p0 if isinstance(t, int) else pl.multiple_of(p0, DM), DM), :]
            pair = (pltpu.bitcast(both << 16, f32).astype(bf16),
                    pltpu.bitcast(both & jnp.uint32(0xFFFF0000), f32).astype(bf16))
            for hh in range(2):
                wqkv[_head(g, c8, hh) * 3 + m] = _as_u32(pair[hh])
                lhs = jnp.concatenate([_as_bf16(xn_pk[k, 0:PRE // 2, :]) for k in range(KT)], axis=1)
                y = _dot(lhs, pair[hh])
                if sc is not None:
                    y = y * sc
                qrings[g][(2 * c8 + hh) * 3 + m, 0:PRE // 2, :] = _as_u32(y.astype(bf16))

    w_wait(0, 1, 0)
    pro_pairs(0, (0,))
    w_wait(1, 1, 1)
    pro_pairs(0, (1,))
    w_wait(2, 2, 2)
    pro_pairs(0, (2, 3))
    w_wait(4, 4, 3)
    x_copy(PRE, SEG, SEM_XC).wait()
    pro_pairs(1, range(NG))
    ln_rows(PRE, TOK, 128, 0)
    for g in range(NG):
        orings[g][:, 48:64, :] = jnp.zeros((8, 16, 128), u32)

    def pro_body(i, carry):
        w_wait(8 + 8 * i, 8, 4 + i)
        pro_pairs(2 + 2 * i, range(NG))
        pro_pairs(3 + 2 * i, range(NG))
        return carry
    lax.fori_loop(0, 5, pro_body, 0)
    wait_all(wo, SEM_WO)
    x_copy(PRE + SEG, S - PRE - SEG, SEM_XB).wait()
    col_tiles_start(wg32, lambda j: pool.at[pl.ds(G0 + 512 * j, 512)], SEM_FFN, FT)
    col_tiles_start(wu32, lambda j: pool.at[pl.ds(U0 + 512 * j, 512)], SEM_FFN, FT)
    col_tiles_start(wd32, lambda j: pool.at[pl.ds(D0 + FF // 2 * j, FF // 2)], SEM_FFN, KT)

    def out_row(s):
        return TOK * s + SEG * ((s + 16) // 20)

    def o_rows(pos, n):
        return jnp.concatenate(
            [_as_bf16(orings[(h % 8) // 2][2 * (h // 8) + h % 2, pl.ds(pos, n), :]) for h in range(H)], axis=1)

    def filler(u):
        k = jnp.maximum(u - 2, 0)
        j = k % 8
        r0 = pl.multiple_of(SEG * (16 * (k // 8) + 3), SEG)
        pos = pl.multiple_of(lax.rem(r0, RO) // 2, 16)
        cs = pl.ds(pl.multiple_of(128 * j, 128), 128)
        a = _dot(o_rows(pos, SEG // 2), _as_bf16(wo[j]))
        out_stage[pl.ds(r0, SEG), cs] = (a + xpn_scr[pl.ds(r0, SEG), cs]).astype(bf16)

    def step(s, mem_in):
        xpos = pl.multiple_of((PRE + TOK * s) // 2, 4)
        wr_pos = [pl.multiple_of(lax.rem(PRE + TOK * s + 8 * i, RQ) // 2, 4) for i in range(3)]
        rd = pl.multiple_of(lax.rem(SEG * s, RQ) // 2, 16)
        owr = pl.multiple_of(lax.rem(SEG * s, RO) // 2, 16)
        orow = pl.multiple_of(out_row(s), 8)
        ord_ = pl.multiple_of(lax.rem(orow, RO) // 2, 4)
        def with_mem(tok_u32, mem_rows):
            tok = _as_bf16(tok_u32)
            last = jnp.concatenate([tok[16:TOK].astype(f32), mem_rows], axis=0).astype(bf16)
            return jnp.concatenate([tok[0:16], last], axis=0)

        zero = zero_scr[0:TOK // 2, :]
        lhs = jnp.concatenate(
            [with_mem(xn_pk[k, pl.ds(xpos, TOK // 2), :] ^ zero, mem_in[:, 128 * k:128 * (k + 1)])
             for k in range(KT)], axis=1)

        mem_parts, probs = {}, {}

        def qkv(g, c):
            res = []
            for m in range(3):
                ms = []
                for hh in range(2):
                    y = _dot(lhs, _as_bf16(wqkv[_head(g, c, hh) * 3 + m]))
                    if m == 0:
                        y = y * SCALE
                    yp = _as_u32(y.astype(bf16))
                    for i in range(3):
                        qrings[g][(2 * c + hh) * 3 + m, pl.ds(wr_pos[i], 4), :] = yp[4 * i:4 * i + 4]
                    ms.append(y[TOK:])
                res.append(jnp.concatenate(ms, axis=0).astype(bf16))
            mem_parts[g, c] = res

        def pair_rows(g, c, m, mem_rows):
            t0 = _as_bf16(qrings[g][(2 * c) * 3 + m, pl.ds(rd, SEG // 2), :])
            t1 = _as_bf16(qrings[g][(2 * c + 1) * 3 + m, pl.ds(rd, SEG // 2), :])
            pad = [jnp.zeros((LK - L2, 128), bf16)] if (m > 0 and LK > L2) else []
            return jnp.concatenate([t0, t1, mem_rows] + pad, axis=0)

        def scores(g, c):
            qm, km, vm = mem_parts.pop((g, c))
            sc = lax.dot_general(pair_rows(g, c, 0, qm), pair_rows(g, c, 1, km),
                                 (((1,), (1,)), ((), ())), preferred_element_type=f32)
            fill = fill_scr[...]
            sc = jnp.where(fill == 0.0, sc, fill)
            e = jnp.exp2(sc - jnp.max(sc, axis=-1, keepdims=True))
            r = pl.reciprocal(jnp.sum(e, axis=-1, keepdims=True), approx=True)
            probs[g, c] = (e.astype(bf16), r, vm)

        def pv(g, c):
            e, r, vm = probs.pop((g, c))
            o = _dot(e, pair_rows(g, c, 2, vm)) * r
            for hh in range(2):
                h = 2 * c + hh
                orings[g][h, pl.ds(owr, SEG // 2), :] = _as_u32(o[SEG * hh:SEG * (hh + 1)].astype(bf16))
                om = o[2 * SEG + NMEM * hh:2 * SEG + NMEM * (hh + 1)]
                lhs_os[g][h] = _as_u32(with_mem(orings[g][h, pl.ds(ord_, TOK // 2), :], om))

        acc = [None] * KT

        def out_proj(gs, js):
            for j in js:
                l = jnp.concatenate([_as_bf16(lhs_os[g][k]) for g in gs for k in range(8)], axis=1)
                w = jnp.concatenate(
                    [_as_bf16(wo[j, 64 * _head(g, c, 0):64 * _head(g, c, 0) + 128, :])
                     for g in gs for c in range(4)], axis=0)
                a = _dot(l, w)
                if acc[j] is None:
                    cs = slice(128 * j, 128 * (j + 1))
                    acc[j] = a + jnp.concatenate([xpn_scr[pl.ds(orow, TOK), cs], jnp.zeros((NMEM, 128), f32)], axis=0)
                else:
                    acc[j] = acc[j] + a

        for item in "q0 q1 s0 q2 p0 s1 q3 p1 s2 w01a p2 s3 w012b L0 p3 w2a w3".split():
            g = int(item[1])
            if item[0] == "L":
                nxt = jnp.minimum(s + 1, NSEG - 1)
                ln_rows(pl.multiple_of(PRE + TOK * nxt, 8), TOK, 128, nxt)
            elif item[0] == "w":
                out_proj([int(ch) for ch in item[1:] if ch.isdigit()],
                         {"a": range(4), "b": range(4, 8)}.get(item[-1], range(8)))
            else:
                for c in {"a": range(2), "b": range(2, 4), "x": range(1), "y": range(1, 4), "u": range(3), "v": range(3, 4)}.get(item[-1], range(4)):
                    {"q": qkv, "s": scores, "p": pv}[item[0]](g, c)
        a = jnp.concatenate(acc, axis=1)
        out_stage[pl.ds(orow, TOK), :] = a[:TOK].astype(bf16)
        return _rnd(a[TOK:])

    def body(u, carry):
        mem = step(2 * u, mem_scr[...])
        filler(u)
        mem_scr[...] = step(2 * u + 1, mem)
        out_copy(pl.multiple_of(out_row(2 * u), 16), 2 * TOK, SEM_OUT).start()
        return carry
    lax.fori_loop(0, NSEG // 2, body, 0)

    wait_all(pool.at[pl.ds(0, FFN_ROWS)], SEM_FFN)
    for f in (3, 19, 35):
        out_copy(SEG * f, SEG, SEM_OUT).start()

    rv = racc[...]
    rrow = lax.broadcasted_iota(jnp.int32, rv.shape, 0)
    rlane = lax.broadcasted_iota(jnp.int32, rv.shape, 1)
    ridx = jnp.where(rrow < 128, rrow + 128 * rlane, PRE + (rrow - 128) + TOK * rlane).astype(f32)
    m0 = jnp.max(rv, keepdims=True)
    f0 = jnp.min(jnp.where(rv == m0, ridx, 1e9), keepdims=True)
    rv2 = jnp.where(ridx == f0, -jnp.inf, rv)
    m1 = jnp.max(rv2, keepdims=True)
    f1 = jnp.min(jnp.where(rv2 == m1, ridx, 1e9), keepdims=True)
    i0 = jnp.clip(f0[0, 0].astype(jnp.int32), 0, S - 1)
    i1 = jnp.clip(f1[0, 0].astype(jnp.int32), 0, S - 1)
    row16 = lax.broadcasted_iota(jnp.int32, (16, DM), 0)

    def xn_row(i):
        w = jnp.concatenate([xn_pk[k, pl.ds(i // 2, 1), :] for k in range(KT)], axis=1)
        return pltpu.bitcast(jnp.where(i % 2 == 0, w << 16, w & jnp.uint32(0xFFFF0000)), f32)
    xsel = jnp.where(row16 == 0, xn_row(i0), jnp.where(row16 == 1, xn_row(i1), 0.0)).astype(bf16)

    r51 = 51 * SEG
    for j in (6, 7):
        cs = slice(128 * j, 128 * (j + 1))
        a = _dot(o_rows((r51 % RO) // 2, SEG // 2), _as_bf16(wo[j]))
        out_stage[r51:r51 + SEG, cs] = (a + xpn_scr[r51:r51 + SEG, cs]).astype(bf16)
    out_copy(r51, SEG, SEM_OUT).start()

    e0 = r51 + SEG
    last = S - 128
    part = {}

    def add(key, v):
        part[key] = v if key not in part else v + part[key]

    def e_round(b, j, r):
        l = jnp.concatenate(
            [_as_bf16(orings[(h % 8) // 2][2 * (h // 8) + h % 2, 64 * b:64 * (b + 1), :])
             for h in range(4 * r, 4 * r + 4)], axis=1)
        add(("e", b, j), _dot(l, _as_bf16(wo[j, 256 * r:256 * (r + 1), :])))
        if r == 7:
            rows, cs = slice(e0 + 128 * b, e0 + 128 * (b + 1)), slice(128 * j, 128 * (j + 1))
            out_stage[rows, cs] = (part.pop(("e", b, j)) + xpn_scr[rows, cs]).astype(bf16)
            if j == KT - 1:
                out_copy(e0 + 128 * b, 128, SEM_OUT if b < 2 else SEM_OUT2).start()

    def up_round(w, name, j, r):
        add((name, j), _dot(xsel[:, 512 * r:512 * (r + 1)], _as_bf16(pool[pl.ds(w + 512 * j + 256 * r, 256), :])))
        if name == "u" and r == 1:
            gate = part.pop(("g", j))
            part["h", j] = (gate * jax.nn.sigmoid(gate) * part.pop(("u", j))).astype(bf16)

    def down_round(j, r):
        hid = jnp.concatenate([part["h", k] for k in range(4 * r, 4 * r + 4)], axis=1)
        add(("y", j), _dot(hid, _as_bf16(pool[pl.ds(D0 + FF // 2 * j + 256 * r, 256), :])))

    e_rounds = [(b, j, r) for b in range(3) for j in range(KT) for r in range(8)]
    m_rounds = [lambda j=j, r=r, w=w, n=n: up_round(w, n, j, r)
                for j in range(FT) for (w, n) in ((G0, "g"), (U0, "u")) for r in range(2)]
    m_rounds += [None] * 4
    m_rounds += [lambda j=j, r=r: down_round(j, r) for r in range(FT // 4) for j in range(KT)]
    m_rounds = [None] * 8 + m_rounds
    NM = 2
    for n, er in enumerate(e_rounds[:128]):
        e_round(*er)
        for mr in m_rounds[NM * n:NM * n + NM]:
            if mr is not None:
                mr()
    assert len(m_rounds) <= NM * 128
    rsel = jnp.where(lax.broadcasted_iota(jnp.int32, (16, 1), 0) == 0, m0, m1)
    y = jnp.concatenate([part.pop(("y", j)) for j in range(KT)], axis=1) * jax.nn.sigmoid(rsel)
    y0, y1 = y[0:1], y[1:2]
    xpn_scr[pl.ds(i0, 1), :] = xpn_scr[pl.ds(i0, 1), :] + jnp.where(i0 >= last, y0, 0.0)
    xpn_scr[pl.ds(i1, 1), :] = xpn_scr[pl.ds(i1, 1), :] + jnp.where(i1 >= last, y1, 0.0)
    for er in e_rounds[128:]:
        e_round(*er)

    out_copy(0, last, SEM_OUT).wait()
    g0 = pl.multiple_of((i0 // 16) * 16, 16)
    g1 = pl.multiple_of((i1 // 16) * 16, 16)
    redo0 = i0 < last
    redo1 = i1 < last
    send1 = jnp.logical_and(redo1, g1 != g0)

    def patch(i, gst, yy):
        blk = out_stage[pl.ds(gst, 16), :].astype(f32)
        out_stage[pl.ds(gst, 16), :] = (blk + jnp.where(row16 == i - gst, yy, 0.0)).astype(bf16)

    @pl.when(redo0)
    def _():
        patch(i0, g0, y0)

    @pl.when(redo1)
    def _():
        patch(i1, g1, y1)

    @pl.when(redo0)
    def _():
        out_copy(g0, 16, SEM_P0).start()

    @pl.when(send1)
    def _():
        out_copy(g1, 16, SEM_P1).start()

    out_copy(last, 128, SEM_OUT2).wait()

    @pl.when(redo0)
    def _():
        out_copy(g0, 16, SEM_P0).wait()

    @pl.when(send1)
    def _():
        out_copy(g1, 16, SEM_P1).wait()


@jax.jit
def pallas_parallel_sum__memory_aug_recurrent_mem_tr__moe_arch_mod__prompt_kernel(
    A_x: jax.Array,
    A_mem0: jax.Array,
    A_Wq: jax.Array,
    A_Wk: jax.Array,
    A_Wv: jax.Array,
    A_Wo: jax.Array,
    A_seg_len: jax.Array,
    B_x: jax.Array,
    B_w_r: jax.Array,
    B_w_gate: jax.Array,
    B_w_up: jax.Array,
    B_w_down: jax.Array,
):
    del A_seg_len, B_x
    assert A_x.shape == (1, S, DM) and A_mem0.shape == (1, NMEM, DM)
    assert A_Wq.shape == (DM, H, DH) and A_Wo.shape == (H, DH, DM) and B_w_gate.shape == (DM, FF)
    hbm = pl.BlockSpec(memory_space=pl.ANY)
    vmem = pl.BlockSpec(memory_space=pltpu.VMEM)
    scratch = [
        pltpu.VMEM((S, DM), bf16),
        pltpu.VMEM((S, DM), f32),
        pltpu.VMEM((KT, S // 2, 128), u32),
        pltpu.VMEM((16, DM), f32),
        pltpu.VMEM((48 * DM, 128), u32),
        pltpu.VMEM((3 * H, DM // 2, 128), u32),
        pltpu.VMEM((KT, H * DH // 2, 128), u32),
    ]
    scratch += [pltpu.VMEM((24, RQ // 2, 128), u32)] * NG
    scratch += [pltpu.VMEM((8, RO // 2, 128), u32)] * NG
    scratch += [pltpu.VMEM((8, 16, 128), u32)] * NG
    scratch += [
        pltpu.VMEM((NMEM, DM), f32),
        pltpu.VMEM((16, 128), u32),
        pltpu.VMEM((L2, LK), f32),
        pltpu.VMEM((128 + TOK, 128), f32),
        pltpu.VMEM((S, DM), bf16),
        pltpu.SemaphoreType.DMA((NSEM,)),
    ]
    return pl.pallas_call(
        _kernel,
        out_shape=jax.ShapeDtypeStruct((1, S, DM), bf16),
        in_specs=[hbm, vmem, hbm, hbm, hbm, hbm, vmem, hbm, hbm, hbm],
        out_specs=hbm,
        scratch_shapes=scratch,
        compiler_params=pltpu.CompilerParams(vmem_limit_bytes=124 * 1024 * 1024,
                                             disable_bounds_checks=True),
    )(A_x, A_mem0, A_Wq, A_Wk, A_Wv, A_Wo.reshape(H * DH, DM), B_w_r, B_w_gate, B_w_up, B_w_down)
```

```python
import jax
import jax.numpy as jnp
from jax import lax
import jax.experimental.pallas as pl
import jax.experimental.pallas.tpu as pltpu

bf16 = jnp.bfloat16
f32 = jnp.float32
u32 = jnp.uint32

S, DM, H, DH, NMEM, SEG, FF = 2048, 1024, 32, 128, 8, 32, 3584
NSEG = S // SEG
TOK = 24
PRE = S - NSEG * TOK
RQ = 544
RO = 832
NG = 4
KT = DM // 128
FT = FF // 128
L2 = 2 * (SEG + NMEM)
LOG2E = 1.4426950408889634
SCALE = DH ** -0.5 * LOG2E
EPS_BF16 = 1.0013580322265625e-05

SEM_W0 = 0
SEM_X0 = 9
SEM_XB, SEM_XC, SEM_WO, SEM_FFN, SEM_OUT, SEM_P0, SEM_P1, SEM_OUT2 = range(13, 21)
NSEM = 21
G0, U0, D0 = 0, FT * DM // 2, 2 * FT * DM // 2
FFN_ROWS = D0 + KT * FF // 2


def _as_bf16(x):
    return pltpu.bitcast(x, bf16)


def _as_u32(x):
    return pltpu.bitcast(x, u32)


def _rnd(x):
    return x.astype(bf16).astype(f32)


def _dot(a, b):
    return jnp.dot(a, b, preferred_element_type=f32)


def _head(g, c, hh):
    return 8 * c + 2 * g + hh


def _kernel(x_hbm, mem0_ref, wq_hbm, wk_hbm, wv_hbm, wo_hbm, wr_ref, wg_hbm, wu_hbm, wd_hbm,
            out_hbm,
            x_scr, xpn_scr, xn_pk, wr_scr, pool, wqkv, wo,
            qr0, qr1, qr2, qr3, or0, or1, or2, or3, lo0, lo1, lo2, lo3,
            mem_scr, zero_scr, fill_scr, racc, out_stage, sems):
    qrings = (qr0, qr1, qr2, qr3)
    orings = (or0, or1, or2, or3)
    lhs_os = (lo0, lo1, lo2, lo3)
    w32 = [w.bitcast(u32) for w in (wq_hbm, wk_hbm, wv_hbm)]
    wo32 = wo_hbm.bitcast(u32)
    wg32 = wg_hbm.bitcast(u32)
    wu32 = wu_hbm.bitcast(u32)
    wd32 = wd_hbm.bitcast(u32)

    def x_copy(r0, n, sem):
        return pltpu.make_async_copy(x_hbm.at[0, pl.ds(r0, n)], x_scr.at[pl.ds(r0, n)], sems.at[sem])

    def out_copy(r0, n, sem):
        return pltpu.make_async_copy(out_stage.at[pl.ds(r0, n)], out_hbm.at[0, pl.ds(r0, n)], sems.at[sem])

    def w_start(lo, hi, sem):
        for p in range(lo, hi):
            pltpu.make_async_copy(w32[p // 16].at[:, p % 16, :], pool.at[pl.ds(DM * p, DM)],
                                  sems.at[SEM_W0 + sem]).start()

    def w_wait(lo, n, sem):
        r0 = DM * lo if isinstance(lo, int) else pl.multiple_of(DM * lo, DM)
        wait_all(pool.at[pl.ds(r0, DM * n)], SEM_W0 + sem)

    def col_tiles_start(src, dst_of, sem, n):
        for j in range(n):
            pltpu.make_async_copy(src.at[:, pl.ds(128 * j, 128)], dst_of(j), sems.at[sem]).start()

    def wait_all(buf, sem):
        pltpu.make_async_copy(buf, buf, sems.at[sem]).wait()

    for c in range(4):
        x_copy(128 * c, 128, SEM_X0 + c).start()
    w_start(0, 1, 0)
    w_start(1, 2, 1)
    w_start(2, 4, 2)
    w_start(4, 8, 3)
    x_copy(PRE, SEG, SEM_XC).start()
    for i in range(5):
        w_start(8 + 8 * i, 16 + 8 * i, 4 + i)
    x_copy(PRE + SEG, S - PRE - SEG, SEM_XB).start()
    col_tiles_start(wo32, lambda j: wo.at[j], SEM_WO, KT)

    mem_scr[...] = mem0_ref[0].astype(f32)
    zero_scr[...] = jnp.zeros(zero_scr.shape, u32)
    wr_row = wr_ref[...].astype(f32).reshape(1, DM)
    wr_scr[0:8, :] = jnp.broadcast_to(wr_row, (8, DM))
    wr_scr[8:16, :] = jnp.broadcast_to(jnp.sum(wr_row, axis=-1, keepdims=True), (8, DM))
    racc[...] = jnp.full(racc.shape, -jnp.inf, f32)
    qi = lax.broadcasted_iota(jnp.int32, (L2, L2), 0)
    ki = lax.broadcasted_iota(jnp.int32, (L2, L2), 1)
    q_mem, k_mem = qi >= 2 * SEG, ki >= 2 * SEG
    q_head = jnp.where(q_mem, (qi - 2 * SEG) // NMEM, qi // SEG)
    k_head = jnp.where(k_mem, (ki - 2 * SEG) // NMEM, ki // SEG)
    visible = q_mem | k_mem | (qi >= ki)
    fill_scr[...] = jnp.where(q_head == k_head, jnp.where(visible, 0.0, -1e9 * LOG2E), -jnp.inf).astype(f32)

    def ln_rows(r0, n, racc_row, lane_id):
        lane = lax.broadcasted_iota(jnp.int32, (n, 128), 1)
        wr = jnp.concatenate([wr_scr[0:8, :]] * (n // 8), axis=0)
        wr_sum = jnp.concatenate([wr_scr[8:16, 0:1]] * (n // 8), axis=0)
        x = x_scr[pl.ds(r0, n), :].astype(f32)
        mean = jnp.sum(x, axis=-1, keepdims=True) * (1.0 / DM)
        msq = jnp.sum(x * x, axis=-1, keepdims=True) * (1.0 / DM)
        xw = jnp.sum(x * wr, axis=-1, keepdims=True)
        var = jnp.maximum(msq - mean * mean, 0.0)
        inv = 1.0 / _rnd(jnp.sqrt(_rnd(_rnd(var) + EPS_BF16)))
        mean = _rnd(mean)
        xnb = ((x - mean) * inv).astype(bf16)
        xpn_scr[pl.ds(r0, n), :] = x + xnb.astype(f32)
        xnp = _as_u32(xnb)
        p0 = r0 // 2 if isinstance(r0, int) else pl.multiple_of(r0 // 2, 4)
        for k in range(KT):
            xn_pk[k, pl.ds(p0, n // 2), :] = xnp[:, 128 * k:128 * (k + 1)]
        r = _rnd((xw - mean * wr_sum) * inv)
        racc[racc_row:racc_row + n, :] = jnp.where(lane == lane_id, r, racc[racc_row:racc_row + n, :])

    def ln_first(c, carry):
        x_copy(pl.multiple_of(128 * c, 128), 128, SEM_X0 + c).wait()
        for i in range(8):
            ln_rows(pl.multiple_of(c * 128 + 16 * i, 16), 16, 16 * i, c)
        return carry
    lax.fori_loop(0, PRE // 128, ln_first, 0)

    def pro_pairs(t, gs):
        m, c8 = t // 4, t % 4
        sc = (SCALE if m == 0 else None) if isinstance(t, int) else jnp.where(m == 0, SCALE, 1.0).astype(f32)
        for g in gs:
            p0 = DM * (4 * t + g)
            both = pool[pl.ds(p0 if isinstance(t, int) else pl.multiple_of(p0, DM), DM), :]
            pair = (pltpu.bitcast(both << 16, f32).astype(bf16),
                    pltpu.bitcast(both & jnp.uint32(0xFFFF0000), f32).astype(bf16))
            for hh in range(2):
                wqkv[_head(g, c8, hh) * 3 + m] = _as_u32(pair[hh])
                lhs = jnp.concatenate([_as_bf16(xn_pk[k, 0:PRE // 2, :]) for k in range(KT)], axis=1)
                y = _dot(lhs, pair[hh])
                if sc is not None:
                    y = y * sc
                qrings[g][(2 * c8 + hh) * 3 + m, 0:PRE // 2, :] = _as_u32(y.astype(bf16))

    w_wait(0, 1, 0)
    pro_pairs(0, (0,))
    w_wait(1, 1, 1)
    pro_pairs(0, (1,))
    w_wait(2, 2, 2)
    pro_pairs(0, (2, 3))
    w_wait(4, 4, 3)
    x_copy(PRE, SEG, SEM_XC).wait()
    pro_pairs(1, range(NG))
    ln_rows(PRE, TOK, 128, 0)
    for g in range(NG):
        orings[g][:, 48:64, :] = jnp.zeros((8, 16, 128), u32)

    def pro_body(i, carry):
        w_wait(8 + 8 * i, 8, 4 + i)
        pro_pairs(2 + 2 * i, range(NG))
        pro_pairs(3 + 2 * i, range(NG))
        return carry
    lax.fori_loop(0, 5, pro_body, 0)
    wait_all(wo, SEM_WO)
    x_copy(PRE + SEG, S - PRE - SEG, SEM_XB).wait()
    col_tiles_start(wg32, lambda j: pool.at[pl.ds(G0 + 512 * j, 512)], SEM_FFN, FT)
    col_tiles_start(wu32, lambda j: pool.at[pl.ds(U0 + 512 * j, 512)], SEM_FFN, FT)
    col_tiles_start(wd32, lambda j: pool.at[pl.ds(D0 + FF // 2 * j, FF // 2)], SEM_FFN, KT)

    def out_row(s):
        return TOK * s + SEG * ((s + 16) // 20)

    def o_rows(pos, n):
        return jnp.concatenate(
            [_as_bf16(orings[(h % 8) // 2][2 * (h // 8) + h % 2, pl.ds(pos, n), :]) for h in range(H)], axis=1)

    def filler(u):
        k = jnp.maximum(u - 2, 0)
        j = k % 8
        r0 = pl.multiple_of(SEG * (16 * (k // 8) + 3), SEG)
        pos = pl.multiple_of(lax.rem(r0, RO) // 2, 16)
        cs = pl.ds(pl.multiple_of(128 * j, 128), 128)
        a = _dot(o_rows(pos, SEG // 2), _as_bf16(wo[j]))
        out_stage[pl.ds(r0, SEG), cs] = (a + xpn_scr[pl.ds(r0, SEG), cs]).astype(bf16)

    def step(s, mem_in):
        xpos = pl.multiple_of((PRE + TOK * s) // 2, 4)
        wr_pos = [pl.multiple_of(lax.rem(PRE + TOK * s + 8 * i, RQ) // 2, 4) for i in range(3)]
        rd = pl.multiple_of(lax.rem(SEG * s, RQ) // 2, 16)
        owr = pl.multiple_of(lax.rem(SEG * s, RO) // 2, 16)
        orow = pl.multiple_of(out_row(s), 8)
        ord_ = pl.multiple_of(lax.rem(orow, RO) // 2, 4)

        def with_mem(tok_u32, mem_rows):
            tok = _as_bf16(tok_u32)
            last = jnp.concatenate([tok[16:TOK].astype(f32), mem_rows], axis=0).astype(bf16)
            return jnp.concatenate([tok[0:16], last], axis=0)

        zero = zero_scr[0:TOK // 2, :]
        lhs = jnp.concatenate(
            [with_mem(xn_pk[k, pl.ds(xpos, TOK // 2), :] ^ zero, mem_in[:, 128 * k:128 * (k + 1)])
             for k in range(KT)], axis=1)

        mem_parts, probs = {}, {}

        def qkv(g, c):
            res = {}
            for m in range(3):
                ms = []
                for hh in range(2):
                    y = _dot(lhs, _as_bf16(wqkv[_head(g, c, hh) * 3 + m]))
                    if m == 0:
                        y = y * SCALE
                    yp = _as_u32(y.astype(bf16))
                    for i in range(3):
                        qrings[g][(2 * c + hh) * 3 + m, pl.ds(wr_pos[i], 4), :] = yp[4 * i:4 * i + 4]
                    ms.append(y[TOK:])
                res[m] = jnp.concatenate(ms, axis=0).astype(bf16)
            mem_parts[g, c] = [res[m] for m in range(3)]

        def pair_rows(g, c, m, mem_rows):
            t0 = _as_bf16(qrings[g][(2 * c) * 3 + m, pl.ds(rd, SEG // 2), :])
            t1 = _as_bf16(qrings[g][(2 * c + 1) * 3 + m, pl.ds(rd, SEG // 2), :])
            return jnp.concatenate([t0, t1, mem_rows], axis=0)

        def scores(g, c):
            qm, km, vm = mem_parts.pop((g, c))
            sc = lax.dot_general(pair_rows(g, c, 0, qm), pair_rows(g, c, 1, km),
                                 (((1,), (1,)), ((), ())), preferred_element_type=f32)
            fill = fill_scr[...]
            sc = jnp.where(fill == 0.0, sc, fill)
            e = jnp.exp2(sc - jnp.max(sc, axis=-1, keepdims=True))
            r = pl.reciprocal(jnp.sum(e, axis=-1, keepdims=True), approx=True)
            probs[g, c] = (e.astype(bf16), r, vm)

        def pv(g, c):
            e, r, vm = probs.pop((g, c))
            o = _dot(e, pair_rows(g, c, 2, vm)) * r
            for hh in range(2):
                h = 2 * c + hh
                orings[g][h, pl.ds(owr, SEG // 2), :] = _as_u32(o[SEG * hh:SEG * (hh + 1)].astype(bf16))
                om = o[2 * SEG + NMEM * hh:2 * SEG + NMEM * (hh + 1)]
                lhs_os[g][h] = _as_u32(with_mem(orings[g][h, pl.ds(ord_, TOK // 2), :], om))

        acc = [None] * KT

        def out_proj(gs, js):
            for j in js:
                l = jnp.concatenate([_as_bf16(lhs_os[g][k]) for g in gs for k in range(8)], axis=1)
                w = jnp.concatenate(
                    [_as_bf16(wo[j, 64 * _head(g, c, 0):64 * _head(g, c, 0) + 128, :])
                     for g in gs for c in range(4)], axis=0)
                a = _dot(l, w)
                if acc[j] is None:
                    cs = slice(128 * j, 128 * (j + 1))
                    acc[j] = a + jnp.concatenate([xpn_scr[pl.ds(orow, TOK), cs], jnp.zeros((NMEM, 128), f32)], axis=0)
                else:
                    acc[j] = acc[j] + a

        for item in "q0 q1 s0 q2 p0 s1 q3 p1 s2 w01a p2 s3 w012b L0 p3 w2a w3".split():
            g = int(item[1])
            if item[0] == "L":
                nxt = jnp.minimum(s + 1, NSEG - 1)
                ln_rows(pl.multiple_of(PRE + TOK * nxt, 8), TOK, 128, nxt)
            elif item[0] == "w":
                out_proj([int(ch) for ch in item[1:] if ch.isdigit()],
                         {"a": range(4), "b": range(4, 8)}.get(item[-1], range(8)))
            else:
                for c in range(4):
                    {"q": qkv, "s": scores, "p": pv}[item[0]](g, c)
        a = jnp.concatenate(acc, axis=1)
        out_stage[pl.ds(orow, TOK), :] = a[:TOK].astype(bf16)
        return _rnd(a[TOK:])

    def body(u, carry):
        mem = step(2 * u, mem_scr[...])
        filler(u)
        mem_scr[...] = step(2 * u + 1, mem)
        out_copy(pl.multiple_of(out_row(2 * u), 16), 2 * TOK, SEM_OUT).start()
        return carry
    lax.fori_loop(0, NSEG // 2, body, 0)

    wait_all(pool.at[pl.ds(0, FFN_ROWS)], SEM_FFN)
    for f in (3, 19, 35):
        out_copy(SEG * f, SEG, SEM_OUT).start()

    rv = racc[...]
    rrow = lax.broadcasted_iota(jnp.int32, rv.shape, 0)
    rlane = lax.broadcasted_iota(jnp.int32, rv.shape, 1)
    ridx = jnp.where(rrow < 128, rrow + 128 * rlane, PRE + (rrow - 128) + TOK * rlane).astype(f32)
    m0 = jnp.max(rv, keepdims=True)
    f0 = jnp.min(jnp.where(rv == m0, ridx, 1e9), keepdims=True)
    rv2 = jnp.where(ridx == f0, -jnp.inf, rv)
    m1 = jnp.max(rv2, keepdims=True)
    f1 = jnp.min(jnp.where(rv2 == m1, ridx, 1e9), keepdims=True)
    i0 = jnp.clip(f0[0, 0].astype(jnp.int32), 0, S - 1)
    i1 = jnp.clip(f1[0, 0].astype(jnp.int32), 0, S - 1)
    row16 = lax.broadcasted_iota(jnp.int32, (16, DM), 0)

    def xn_row(i):
        w = jnp.concatenate([xn_pk[k, pl.ds(i // 2, 1), :] for k in range(KT)], axis=1)
        return pltpu.bitcast(jnp.where(i % 2 == 0, w << 16, w & jnp.uint32(0xFFFF0000)), f32)
    xsel = jnp.where(row16 == 0, xn_row(i0), jnp.where(row16 == 1, xn_row(i1), 0.0)).astype(bf16)

    r51 = 51 * SEG
    for j in (6, 7):
        cs = slice(128 * j, 128 * (j + 1))
        a = _dot(o_rows((r51 % RO) // 2, SEG // 2), _as_bf16(wo[j]))
        out_stage[r51:r51 + SEG, cs] = (a + xpn_scr[r51:r51 + SEG, cs]).astype(bf16)
    out_copy(r51, SEG, SEM_OUT).start()

    e0 = r51 + SEG
    last = S - 128
    part = {}

    def add(key, v):
        part[key] = v if key not in part else v + part[key]

    def e_round(b, j, r):
        l = jnp.concatenate(
            [_as_bf16(orings[(h % 8) // 2][2 * (h // 8) + h % 2, 64 * b:64 * (b + 1), :])
             for h in range(4 * r, 4 * r + 4)], axis=1)
        add(("e", b, j), _dot(l, _as_bf16(wo[j, 256 * r:256 * (r + 1), :])))
        if r == 7:
            rows, cs = slice(e0 + 128 * b, e0 + 128 * (b + 1)), slice(128 * j, 128 * (j + 1))
            out_stage[rows, cs] = (part.pop(("e", b, j)) + xpn_scr[rows, cs]).astype(bf16)
            if j == KT - 1:
                out_copy(e0 + 128 * b, 128, SEM_OUT if b < 2 else SEM_OUT2).start()

    def up_round(w, name, j, r):
        add((name, j), _dot(xsel[:, 512 * r:512 * (r + 1)], _as_bf16(pool[pl.ds(w + 512 * j + 256 * r, 256), :])))
        if name == "u" and r == 1:
            gate = part.pop(("g", j))
            part["h", j] = (gate * jax.nn.sigmoid(gate) * part.pop(("u", j))).astype(bf16)

    def down_round(j, r):
        hid = jnp.concatenate([part["h", k] for k in range(4 * r, 4 * r + 4)], axis=1)
        add(("y", j), _dot(hid, _as_bf16(pool[pl.ds(D0 + FF // 2 * j + 256 * r, 256), :])))

    e_rounds = [(b, j, r) for b in range(3) for j in range(KT) for r in range(8)]
    m_rounds = [lambda j=j, r=r, w=w, n=n: up_round(w, n, j, r)
                for j in range(FT) for (w, n) in ((G0, "g"), (U0, "u")) for r in range(2)]
    m_rounds += [None] * 4
    m_rounds += [lambda j=j, r=r: down_round(j, r) for r in range(FT // 4) for j in range(KT)]
    m_rounds = [None] * 8 + m_rounds
    NM = 2
    for n, er in enumerate(e_rounds[:128]):
        e_round(*er)
        for mr in m_rounds[NM * n:NM * n + NM]:
            if mr is not None:
                mr()
    assert len(m_rounds) <= NM * 128
    rsel = jnp.where(lax.broadcasted_iota(jnp.int32, (16, 1), 0) == 0, m0, m1)
    y = jnp.concatenate([part.pop(("y", j)) for j in range(KT)], axis=1) * jax.nn.sigmoid(rsel)
    y0, y1 = y[0:1], y[1:2]
    xpn_scr[pl.ds(i0, 1), :] = xpn_scr[pl.ds(i0, 1), :] + jnp.where(i0 >= last, y0, 0.0)
    xpn_scr[pl.ds(i1, 1), :] = xpn_scr[pl.ds(i1, 1), :] + jnp.where(i1 >= last, y1, 0.0)
    for er in e_rounds[128:]:
        e_round(*er)

    out_copy(0, last, SEM_OUT).wait()
    g0 = pl.multiple_of((i0 // 16) * 16, 16)
    g1 = pl.multiple_of((i1 // 16) * 16, 16)
    redo0 = i0 < last
    redo1 = i1 < last
    send1 = jnp.logical_and(redo1, g1 != g0)

    def patch(i, gst, yy):
        blk = out_stage[pl.ds(gst, 16), :].astype(f32)
        out_stage[pl.ds(gst, 16), :] = (blk + jnp.where(row16 == i - gst, yy, 0.0)).astype(bf16)

    @pl.when(redo0)
    def _():
        patch(i0, g0, y0)

    @pl.when(redo1)
    def _():
        patch(i1, g1, y1)

    @pl.when(redo0)
    def _():
        out_copy(g0, 16, SEM_P0).start()

    @pl.when(send1)
    def _():
        out_copy(g1, 16, SEM_P1).start()

    out_copy(last, 128, SEM_OUT2).wait()

    @pl.when(redo0)
    def _():
        out_copy(g0, 16, SEM_P0).wait()

    @pl.when(send1)
    def _():
        out_copy(g1, 16, SEM_P1).wait()


@jax.jit
def pallas_parallel_sum__memory_aug_recurrent_mem_tr__moe_arch_mod__prompt_kernel(
    A_x: jax.Array,
    A_mem0: jax.Array,
    A_Wq: jax.Array,
    A_Wk: jax.Array,
    A_Wv: jax.Array,
    A_Wo: jax.Array,
    A_seg_len: jax.Array,
    B_x: jax.Array,
    B_w_r: jax.Array,
    B_w_gate: jax.Array,
    B_w_up: jax.Array,
    B_w_down: jax.Array,
):
    del A_seg_len, B_x
    assert A_x.shape == (1, S, DM) and A_mem0.shape == (1, NMEM, DM)
    assert A_Wq.shape == (DM, H, DH) and A_Wo.shape == (H, DH, DM) and B_w_gate.shape == (DM, FF)
    hbm = pl.BlockSpec(memory_space=pl.ANY)
    vmem = pl.BlockSpec(memory_space=pltpu.VMEM)
    scratch = [
        pltpu.VMEM((S, DM), bf16),
        pltpu.VMEM((S, DM), f32),
        pltpu.VMEM((KT, S // 2, 128), u32),
        pltpu.VMEM((16, DM), f32),
        pltpu.VMEM((48 * DM, 128), u32),
        pltpu.VMEM((3 * H, DM // 2, 128), u32),
        pltpu.VMEM((KT, H * DH // 2, 128), u32),
    ]
    scratch += [pltpu.VMEM((24, RQ // 2, 128), u32)] * NG
    scratch += [pltpu.VMEM((8, RO // 2, 128), u32)] * NG
    scratch += [pltpu.VMEM((8, 16, 128), u32)] * NG
    scratch += [
        pltpu.VMEM((NMEM, DM), f32),
        pltpu.VMEM((16, 128), u32),
        pltpu.VMEM((L2, L2), f32),
        pltpu.VMEM((128 + TOK, 128), f32),
        pltpu.VMEM((S, DM), bf16),
        pltpu.SemaphoreType.DMA((NSEM,)),
    ]
    return pl.pallas_call(
        _kernel,
        out_shape=jax.ShapeDtypeStruct((1, S, DM), bf16),
        in_specs=[hbm, vmem, hbm, hbm, hbm, hbm, vmem, hbm, hbm, hbm],
        out_specs=hbm,
        scratch_shapes=scratch,
        compiler_params=pltpu.CompilerParams(vmem_limit_bytes=110 * 1024 * 1024,
                                             disable_bounds_checks=True),
    )(A_x, A_mem0, A_Wq, A_Wk, A_Wv, A_Wo.reshape(H * DH, DM), B_w_r, B_w_gate, B_w_up, B_w_down)
```

```python
import jax
import jax.numpy as jnp
from jax import lax
import jax.experimental.pallas as pl
import jax.experimental.pallas.tpu as pltpu

bf16 = jnp.bfloat16
f32 = jnp.float32
u32 = jnp.uint32

S, DM, H, DH, NMEM, SEG, FF = 2048, 1024, 32, 128, 8, 32, 3584
NSEG = S // SEG
TOK = 24
PRE = S - NSEG * TOK
RQ = 544
RO = 768
NG = 4
KT = DM // 128
FT = FF // 128
L2 = 2 * (SEG + NMEM)
LOG2E = 1.4426950408889634
SCALE = DH ** -0.5 * LOG2E
EPS_BF16 = 1.0013580322265625e-05

SEM_W0 = 0
SEM_X0 = 9
SEM_XB, SEM_XC, SEM_WO, SEM_FFN, SEM_OUT, SEM_P0, SEM_P1, SEM_OUT2 = range(13, 21)
NSEM = 21
G0, U0, D0 = 0, FT * DM // 2, 2 * FT * DM // 2
FFN_ROWS = D0 + KT * FF // 2


def _as_bf16(x):
    return pltpu.bitcast(x, bf16)


def _as_u32(x):
    return pltpu.bitcast(x, u32)


def _rnd(x):
    return x.astype(bf16).astype(f32)


def _dot(a, b):
    return jnp.dot(a, b, preferred_element_type=f32)


def _head(g, c, hh):
    return 8 * c + 2 * g + hh


def _kernel(x_hbm, mem0_ref, wq_hbm, wk_hbm, wv_hbm, wo_hbm, wr_ref, wg_hbm, wu_hbm, wd_hbm,
            out_hbm,
            x_scr, xpn_scr, xn_pk, wr_scr, pool, wqkv, wo,
            qr0, qr1, qr2, qr3, or0, or1, or2, or3, lo0, lo1, lo2, lo3,
            mem_scr, zero_scr, fill_scr, racc, out_stage, sems):
    qrings = (qr0, qr1, qr2, qr3)
    orings = (or0, or1, or2, or3)
    lhs_os = (lo0, lo1, lo2, lo3)
    w32 = [w.bitcast(u32) for w in (wq_hbm, wk_hbm, wv_hbm)]
    wo32 = wo_hbm.bitcast(u32)
    wg32 = wg_hbm.bitcast(u32)
    wu32 = wu_hbm.bitcast(u32)
    wd32 = wd_hbm.bitcast(u32)

    def x_copy(r0, n, sem):
        return pltpu.make_async_copy(x_hbm.at[0, pl.ds(r0, n)], x_scr.at[pl.ds(r0, n)], sems.at[sem])

    def out_copy(r0, n, sem):
        return pltpu.make_async_copy(out_stage.at[pl.ds(r0, n)], out_hbm.at[0, pl.ds(r0, n)], sems.at[sem])

    def w_start(lo, hi, sem):
        for p in range(lo, hi):
            pltpu.make_async_copy(w32[p // 16].at[:, p % 16, :], pool.at[pl.ds(DM * p, DM)],
                                  sems.at[SEM_W0 + sem]).start()

    def w_wait(lo, n, sem):
        r0 = DM * lo if isinstance(lo, int) else pl.multiple_of(DM * lo, DM)
        wait_all(pool.at[pl.ds(r0, DM * n)], SEM_W0 + sem)

    def col_tiles_start(src, dst_of, sem, n):
        for j in range(n):
            pltpu.make_async_copy(src.at[:, pl.ds(128 * j, 128)], dst_of(j), sems.at[sem]).start()

    def wait_all(buf, sem):
        pltpu.make_async_copy(buf, buf, sems.at[sem]).wait()

    for c in range(4):
        x_copy(128 * c, 128, SEM_X0 + c).start()
    w_start(0, 1, 0)
    w_start(1, 2, 1)
    w_start(2, 4, 2)
    w_start(4, 8, 3)
    x_copy(PRE, SEG, SEM_XC).start()
    for i in range(5):
        w_start(8 + 8 * i, 16 + 8 * i, 4 + i)
    x_copy(PRE + SEG, S - PRE - SEG, SEM_XB).start()
    col_tiles_start(wo32, lambda j: wo.at[j], SEM_WO, KT)

    mem_scr[...] = mem0_ref[0].astype(f32)
    zero_scr[...] = jnp.zeros(zero_scr.shape, u32)
    wr_row = wr_ref[...].astype(f32).reshape(1, DM)
    wr_scr[0:8, :] = jnp.broadcast_to(wr_row, (8, DM))
    wr_scr[8:16, :] = jnp.broadcast_to(jnp.sum(wr_row, axis=-1, keepdims=True), (8, DM))
    racc[...] = jnp.full(racc.shape, -jnp.inf, f32)
    qi = lax.broadcasted_iota(jnp.int32, (L2, L2), 0)
    ki = lax.broadcasted_iota(jnp.int32, (L2, L2), 1)
    q_mem, k_mem = qi >= 2 * SEG, ki >= 2 * SEG
    q_head = jnp.where(q_mem, (qi - 2 * SEG) // NMEM, qi // SEG)
    k_head = jnp.where(k_mem, (ki - 2 * SEG) // NMEM, ki // SEG)
    visible = q_mem | k_mem | (qi >= ki)
    fill_scr[...] = jnp.where(q_head == k_head, jnp.where(visible, 0.0, -1e9 * LOG2E), -jnp.inf).astype(f32)

    def ln_rows(r0, n, racc_row, lane_id):
        lane = lax.broadcasted_iota(jnp.int32, (n, 128), 1)
        wr = jnp.concatenate([wr_scr[0:8, :]] * (n // 8), axis=0)
        wr_sum = jnp.concatenate([wr_scr[8:16, 0:1]] * (n // 8), axis=0)
        x = x_scr[pl.ds(r0, n), :].astype(f32)
        mean = jnp.sum(x, axis=-1, keepdims=True) * (1.0 / DM)
        msq = jnp.sum(x * x, axis=-1, keepdims=True) * (1.0 / DM)
        xw = jnp.sum(x * wr, axis=-1, keepdims=True)
        var = jnp.maximum(msq - mean * mean, 0.0)
        inv = 1.0 / _rnd(jnp.sqrt(_rnd(_rnd(var) + EPS_BF16)))
        mean = _rnd(mean)
        xnb = ((x - mean) * inv).astype(bf16)
        xpn_scr[pl.ds(r0, n), :] = x + xnb.astype(f32)
        xnp = _as_u32(xnb)
        p0 = r0 // 2 if isinstance(r0, int) else pl.multiple_of(r0 // 2, 4)
        for k in range(KT):
            xn_pk[k, pl.ds(p0, n // 2), :] = xnp[:, 128 * k:128 * (k + 1)]
        r = _rnd((xw - mean * wr_sum) * inv)
        racc[racc_row:racc_row + n, :] = jnp.where(lane == lane_id, r, racc[racc_row:racc_row + n, :])

    def ln_first(c, carry):
        x_copy(pl.multiple_of(128 * c, 128), 128, SEM_X0 + c).wait()
        for i in range(8):
            ln_rows(pl.multiple_of(c * 128 + 16 * i, 16), 16, 16 * i, c)
        return carry
    lax.fori_loop(0, PRE // 128, ln_first, 0)

    def pro_pairs(t, gs):
        m, c8 = t // 4, t % 4
        sc = (SCALE if m == 0 else None) if isinstance(t, int) else jnp.where(m == 0, SCALE, 1.0).astype(f32)
        for g in gs:
            p0 = DM * (4 * t + g)
            both = pool[pl.ds(p0 if isinstance(t, int) else pl.multiple_of(p0, DM), DM), :]
            pair = (pltpu.bitcast(both << 16, f32).astype(bf16),
                    pltpu.bitcast(both & jnp.uint32(0xFFFF0000), f32).astype(bf16))
            for hh in range(2):
                wqkv[_head(g, c8, hh) * 3 + m] = _as_u32(pair[hh])
                lhs = jnp.concatenate([_as_bf16(xn_pk[k, 0:PRE // 2, :]) for k in range(KT)], axis=1)
                y = _dot(lhs, pair[hh])
                if sc is not None:
                    y = y * sc
                qrings[g][(2 * c8 + hh) * 3 + m, 0:PRE // 2, :] = _as_u32(y.astype(bf16))

    w_wait(0, 1, 0)
    pro_pairs(0, (0,))
    w_wait(1, 1, 1)
    pro_pairs(0, (1,))
    w_wait(2, 2, 2)
    pro_pairs(0, (2, 3))
    w_wait(4, 4, 3)
    x_copy(PRE, SEG, SEM_XC).wait()
    pro_pairs(1, range(NG))
    ln_rows(PRE, TOK, 128, 0)

    def pro_body(i, carry):
        w_wait(8 + 8 * i, 8, 4 + i)
        pro_pairs(2 + 2 * i, range(NG))
        pro_pairs(3 + 2 * i, range(NG))
        return carry
    lax.fori_loop(0, 5, pro_body, 0)
    wait_all(wo, SEM_WO)
    x_copy(PRE + SEG, S - PRE - SEG, SEM_XB).wait()
    col_tiles_start(wg32, lambda j: pool.at[pl.ds(G0 + 512 * j, 512)], SEM_FFN, FT)
    col_tiles_start(wu32, lambda j: pool.at[pl.ds(U0 + 512 * j, 512)], SEM_FFN, FT)
    col_tiles_start(wd32, lambda j: pool.at[pl.ds(D0 + FF // 2 * j, FF // 2)], SEM_FFN, KT)

    def step(s, mem_in, do_ln=True):
        xpos = pl.multiple_of((PRE + TOK * s) // 2, 4)
        wr_pos = [pl.multiple_of(lax.rem(PRE + TOK * s + 8 * i, RQ) // 2, 4) for i in range(3)]
        rd = pl.multiple_of(lax.rem(SEG * s, RQ) // 2, 16)
        owr = pl.multiple_of(lax.rem(SEG * s, RO) // 2, 16)
        orow = pl.multiple_of(TOK * s, 8)
        ord_ = pl.multiple_of(lax.rem(orow, RO) // 2, 4)

        def with_mem(tok_u32, mem_rows):
            tok = _as_bf16(tok_u32)
            last = jnp.concatenate([tok[16:TOK].astype(f32), mem_rows], axis=0).astype(bf16)
            return jnp.concatenate([tok[0:16], last], axis=0)

        zero = zero_scr[0:TOK // 2, :]
        lhs = jnp.concatenate(
            [with_mem(xn_pk[k, pl.ds(xpos, TOK // 2), :] ^ zero, mem_in[:, 128 * k:128 * (k + 1)])
             for k in range(KT)], axis=1)

        mem_parts, probs = {}, {}
        NS = 6
        first = [(c, m, hh) for c in range(4) for m in range(3) for hh in range(2)][:NS]
        lo = {key: _dot(lhs[:, :512], _as_bf16(wqkv[_head(0, key[0], key[2]) * 3 + key[1], 0:256, :])) for key in first}

        def qkv(g, c):
            res = {}
            for m in range(3):
                ms = []
                for hh in range(2):
                    if g == 0 and (c, m, hh) in lo:
                        y = _dot(lhs[:, 512:], _as_bf16(wqkv[_head(g, c, hh) * 3 + m, 256:512, :])) + lo[c, m, hh]
                    else:
                        y = _dot(lhs, _as_bf16(wqkv[_head(g, c, hh) * 3 + m]))
                    if m == 0:
                        y = y * SCALE
                    yp = _as_u32(y.astype(bf16))
                    for i in range(3):
                        qrings[g][(2 * c + hh) * 3 + m, pl.ds(wr_pos[i], 4), :] = yp[4 * i:4 * i + 4]
                    ms.append(y[TOK:])
                res[m] = jnp.concatenate(ms, axis=0).astype(bf16)
            mem_parts[g, c] = [res[m] for m in range(3)]

        def pair_rows(g, c, m, mem_rows):
            t0 = _as_bf16(qrings[g][(2 * c) * 3 + m, pl.ds(rd, SEG // 2), :])
            t1 = _as_bf16(qrings[g][(2 * c + 1) * 3 + m, pl.ds(rd, SEG // 2), :])
            return jnp.concatenate([t0, t1, mem_rows], axis=0)

        def scores(g, c):
            qm, km, vm = mem_parts.pop((g, c))
            sc = lax.dot_general(pair_rows(g, c, 0, qm), pair_rows(g, c, 1, km),
                                 (((1,), (1,)), ((), ())), preferred_element_type=f32)
            fill = fill_scr[...]
            sc = jnp.where(fill == 0.0, sc, fill)
            e = jnp.exp2(sc - jnp.max(sc, axis=-1, keepdims=True))
            r = pl.reciprocal(jnp.sum(e, axis=-1, keepdims=True), approx=True)
            probs[g, c] = (e.astype(bf16), r, vm)

        def pv(g, c):
            e, r, vm = probs.pop((g, c))
            o = _dot(e, pair_rows(g, c, 2, vm)) * r
            for hh in range(2):
                h = 2 * c + hh
                orings[g][h, pl.ds(owr, SEG // 2), :] = _as_u32(o[SEG * hh:SEG * (hh + 1)].astype(bf16))
                om = o[2 * SEG + NMEM * hh:2 * SEG + NMEM * (hh + 1)]
                lhs_os[g][h] = _as_u32(with_mem(orings[g][h, pl.ds(ord_, TOK // 2), :], om))

        acc = [None] * KT

        def out_proj(gs, js):
            for j in js:
                l = jnp.concatenate([_as_bf16(lhs_os[g][k]) for g in gs for k in range(8)], axis=1)
                w = jnp.concatenate(
                    [_as_bf16(wo[j, 64 * _head(g, c, 0):64 * _head(g, c, 0) + 128, :])
                     for g in gs for c in range(4)], axis=0)
                a = _dot(l, w)
                if acc[j] is None:
                    cs = slice(128 * j, 128 * (j + 1))
                    acc[j] = a + jnp.concatenate([xpn_scr[pl.ds(orow, TOK), cs], jnp.zeros((NMEM, 128), f32)], axis=0)
                else:
                    acc[j] = acc[j] + a

        for item in "q0 q1 s0 q2 p0 s1 q3 p1 s2 w01a p2 s3 w012b L0 p3 w2a w3".split():
            g = int(item[1])
            if item[0] == "L":
                if do_ln:
                    nxt = jnp.minimum(s + 1, NSEG - 1)
                    ln_rows(pl.multiple_of(PRE + TOK * nxt, 8), TOK, 128, nxt)
            elif item[0] == "w":
                out_proj([int(ch) for ch in item[1:] if ch.isdigit()],
                         {"a": range(4), "b": range(4, 8)}.get(item[-1], range(8)))
            else:
                for c in range(4):
                    {"q": qkv, "s": scores, "p": pv}[item[0]](g, c)
        a = jnp.concatenate(acc, axis=1)
        out_stage[pl.ds(orow, TOK), :] = a[:TOK].astype(bf16)
        return _rnd(a[TOK:])

    UNR = 3
    PEEL = 1

    def body(u, carry):
        mem = mem_scr[...]
        for i in range(UNR):
            mem = step(UNR * u + i, mem)
        mem_scr[...] = mem
        out_copy(pl.multiple_of(TOK * UNR * u, 8), UNR * TOK, SEM_OUT).start()
        return carry
    lax.fori_loop(0, (NSEG - PEEL) // UNR, body, 0)

    wait_all(pool.at[pl.ds(0, FFN_ROWS)], SEM_FFN)

    mem = mem_scr[...]
    for s in range(NSEG - PEEL, NSEG):
        mem = step(jnp.int32(s), mem, do_ln=s < NSEG - 1)
    if PEEL:
        out_copy(TOK * (NSEG - PEEL), PEEL * TOK, SEM_OUT).start()

    rv = racc[...]
    rrow = lax.broadcasted_iota(jnp.int32, rv.shape, 0)
    rlane = lax.broadcasted_iota(jnp.int32, rv.shape, 1)
    ridx = jnp.where(rrow < 128, rrow + 128 * rlane, PRE + (rrow - 128) + TOK * rlane).astype(f32)
    m0 = jnp.max(rv, keepdims=True)
    f0 = jnp.min(jnp.where(rv == m0, ridx, 1e9), keepdims=True)
    rv2 = jnp.where(ridx == f0, -jnp.inf, rv)
    m1 = jnp.max(rv2, keepdims=True)
    f1 = jnp.min(jnp.where(rv2 == m1, ridx, 1e9), keepdims=True)
    i0 = jnp.clip(f0[0, 0].astype(jnp.int32), 0, S - 1)
    i1 = jnp.clip(f1[0, 0].astype(jnp.int32), 0, S - 1)
    row16 = lax.broadcasted_iota(jnp.int32, (16, DM), 0)

    def xn_row(i):
        w = jnp.concatenate([xn_pk[k, pl.ds(i // 2, 1), :] for k in range(KT)], axis=1)
        return pltpu.bitcast(jnp.where(i % 2 == 0, w << 16, w & jnp.uint32(0xFFFF0000)), f32)
    xsel = jnp.where(row16 == 0, xn_row(i0), jnp.where(row16 == 1, xn_row(i1), 0.0)).astype(bf16)

    e0 = NSEG * TOK
    last = S - 128
    part = {}

    def add(key, v):
        part[key] = v if key not in part else v + part[key]

    def e_round(b, j, r):
        l = jnp.concatenate(
            [_as_bf16(orings[(h % 8) // 2][2 * (h // 8) + h % 2, 64 * b:64 * (b + 1), :])
             for h in range(4 * r, 4 * r + 4)], axis=1)
        add(("e", b, j), _dot(l, _as_bf16(wo[j, 256 * r:256 * (r + 1), :])))
        if r == 7:
            rows, cs = slice(e0 + 128 * b, e0 + 128 * (b + 1)), slice(128 * j, 128 * (j + 1))
            out_stage[rows, cs] = (part.pop(("e", b, j)) + xpn_scr[rows, cs]).astype(bf16)
            if j == KT - 1:
                out_copy(e0 + 128 * b, 128, SEM_OUT if b < 3 else SEM_OUT2).start()

    def up_round(w, name, j, r):
        add((name, j), _dot(xsel[:, 512 * r:512 * (r + 1)], _as_bf16(pool[pl.ds(w + 512 * j + 256 * r, 256), :])))
        if name == "u" and r == 1:
            gate = part.pop(("g", j))
            part["h", j] = (gate * jax.nn.sigmoid(gate) * part.pop(("u", j))).astype(bf16)

    def down_round(j, r):
        hid = jnp.concatenate([part["h", k] for k in range(4 * r, 4 * r + 4)], axis=1)
        add(("y", j), _dot(hid, _as_bf16(pool[pl.ds(D0 + FF // 2 * j + 256 * r, 256), :])))

    e_rounds = [(b, j, r) for b in range(4) for j in range(KT) for r in range(8)]
    m_rounds = [lambda j=j, r=r, w=w, n=n: up_round(w, n, j, r)
                for j in range(FT) for (w, n) in ((G0, "g"), (U0, "u")) for r in range(2)]
    m_rounds += [None] * 4
    m_rounds += [lambda j=j, r=r: down_round(j, r) for r in range(FT // 4) for j in range(KT)]
    m_rounds = [None] * 2 + m_rounds
    NM = 2
    for n, er in enumerate(e_rounds[:128]):
        e_round(*er)
        for mr in m_rounds[NM * n:NM * n + NM]:
            if mr is not None:
                mr()
    assert len(m_rounds) <= NM * 128
    rsel = jnp.where(lax.broadcasted_iota(jnp.int32, (16, 1), 0) == 0, m0, m1)
    y = jnp.concatenate([part.pop(("y", j)) for j in range(KT)], axis=1) * jax.nn.sigmoid(rsel)
    y0, y1 = y[0:1], y[1:2]
    xpn_scr[pl.ds(i0, 1), :] = xpn_scr[pl.ds(i0, 1), :] + jnp.where(i0 >= last, y0, 0.0)
    xpn_scr[pl.ds(i1, 1), :] = xpn_scr[pl.ds(i1, 1), :] + jnp.where(i1 >= last, y1, 0.0)
    for er in e_rounds[128:]:
        e_round(*er)

    out_copy(0, last, SEM_OUT).wait()
    g0 = pl.multiple_of((i0 // 16) * 16, 16)
    g1 = pl.multiple_of((i1 // 16) * 16, 16)
    redo0 = i0 < last
    redo1 = i1 < last
    send1 = jnp.logical_and(redo1, g1 != g0)

    def patch(i, gst, yy):
        blk = out_stage[pl.ds(gst, 16), :].astype(f32)
        out_stage[pl.ds(gst, 16), :] = (blk + jnp.where(row16 == i - gst, yy, 0.0)).astype(bf16)

    @pl.when(redo0)
    def _():
        patch(i0, g0, y0)

    @pl.when(redo1)
    def _():
        patch(i1, g1, y1)

    @pl.when(redo0)
    def _():
        out_copy(g0, 16, SEM_P0).start()

    @pl.when(send1)
    def _():
        out_copy(g1, 16, SEM_P1).start()

    out_copy(last, 128, SEM_OUT2).wait()

    @pl.when(redo0)
    def _():
        out_copy(g0, 16, SEM_P0).wait()

    @pl.when(send1)
    def _():
        out_copy(g1, 16, SEM_P1).wait()


@jax.jit
def pallas_parallel_sum__memory_aug_recurrent_mem_tr__moe_arch_mod__prompt_kernel(
    A_x: jax.Array,
    A_mem0: jax.Array,
    A_Wq: jax.Array,
    A_Wk: jax.Array,
    A_Wv: jax.Array,
    A_Wo: jax.Array,
    A_seg_len: jax.Array,
    B_x: jax.Array,
    B_w_r: jax.Array,
    B_w_gate: jax.Array,
    B_w_up: jax.Array,
    B_w_down: jax.Array,
):
    del A_seg_len, B_x
    assert A_x.shape == (1, S, DM) and A_mem0.shape == (1, NMEM, DM)
    assert A_Wq.shape == (DM, H, DH) and A_Wo.shape == (H, DH, DM) and B_w_gate.shape == (DM, FF)
    hbm = pl.BlockSpec(memory_space=pl.ANY)
    vmem = pl.BlockSpec(memory_space=pltpu.VMEM)
    scratch = [
        pltpu.VMEM((S, DM), bf16),
        pltpu.VMEM((S, DM), f32),
        pltpu.VMEM((KT, S // 2, 128), u32),
        pltpu.VMEM((16, DM), f32),
        pltpu.VMEM((48 * DM, 128), u32),
        pltpu.VMEM((3 * H, DM // 2, 128), u32),
        pltpu.VMEM((KT, H * DH // 2, 128), u32),
    ]
    scratch += [pltpu.VMEM((24, RQ // 2, 128), u32)] * NG
    scratch += [pltpu.VMEM((8, RO // 2, 128), u32)] * NG
    scratch += [pltpu.VMEM((8, 16, 128), u32)] * NG
    scratch += [
        pltpu.VMEM((NMEM, DM), f32),
        pltpu.VMEM((16, 128), u32),
        pltpu.VMEM((L2, L2), f32),
        pltpu.VMEM((128 + TOK, 128), f32),
        pltpu.VMEM((S, DM), bf16),
        pltpu.SemaphoreType.DMA((NSEM,)),
    ]
    return pl.pallas_call(
        _kernel,
        out_shape=jax.ShapeDtypeStruct((1, S, DM), bf16),
        in_specs=[hbm, vmem, hbm, hbm, hbm, hbm, vmem, hbm, hbm, hbm],
        out_specs=hbm,
        scratch_shapes=scratch,
        compiler_params=pltpu.CompilerParams(vmem_limit_bytes=110 * 1024 * 1024,
                                             disable_bounds_checks=True),
    )(A_x, A_mem0, A_Wq, A_Wk, A_Wv, A_Wo.reshape(H * DH, DM), B_w_r, B_w_gate, B_w_up, B_w_down)
```

```python
import jax
import jax.numpy as jnp
from jax import lax
import jax.experimental.pallas as pl
import jax.experimental.pallas.tpu as pltpu

bf16 = jnp.bfloat16
f32 = jnp.float32
u32 = jnp.uint32

S, DM, H, DH, NMEM, SEG, FF = 2048, 1024, 32, 128, 8, 32, 3584
NSEG = S // SEG
TOK = 24
PRE = S - NSEG * TOK
RQ = 544
RO = 768
NG = 4
KT = DM // 128
FT = FF // 128
L2 = 2 * (SEG + NMEM)
LOG2E = 1.4426950408889634
SCALE = DH ** -0.5 * LOG2E
EPS_BF16 = 1.0013580322265625e-05

SEM_W0 = 0
SEM_X0 = 9
SEM_XB, SEM_XC, SEM_WO, SEM_FFN, SEM_OUT, SEM_P0, SEM_P1, SEM_OUT2 = range(13, 21)
NSEM = 21
G0, U0, D0 = 0, FT * DM // 2, 2 * FT * DM // 2
FFN_ROWS = D0 + KT * FF // 2


def _as_bf16(x):
    return pltpu.bitcast(x, bf16)


def _as_u32(x):
    return pltpu.bitcast(x, u32)


def _rnd(x):
    return x.astype(bf16).astype(f32)


def _dot(a, b):
    return jnp.dot(a, b, preferred_element_type=f32)


def _head(g, c, hh):
    return 8 * c + 2 * g + hh


def _kernel(x_hbm, mem0_ref, wq_hbm, wk_hbm, wv_hbm, wo_hbm, wr_ref, wg_hbm, wu_hbm, wd_hbm,
            out_hbm,
            x_scr, xpn_scr, xn_pk, wr_scr, pool, wqkv, wo,
            qr0, qr1, qr2, qr3, or0, or1, or2, or3, lo0, lo1, lo2, lo3,
            mem_scr, zero_scr, fill_scr, racc, out_stage, sems):
    qrings = (qr0, qr1, qr2, qr3)
    orings = (or0, or1, or2, or3)
    lhs_os = (lo0, lo1, lo2, lo3)
    w32 = [w.bitcast(u32) for w in (wq_hbm, wk_hbm, wv_hbm)]
    wo32 = wo_hbm.bitcast(u32)
    wg32 = wg_hbm.bitcast(u32)
    wu32 = wu_hbm.bitcast(u32)
    wd32 = wd_hbm.bitcast(u32)

    def x_copy(r0, n, sem):
        return pltpu.make_async_copy(x_hbm.at[0, pl.ds(r0, n)], x_scr.at[pl.ds(r0, n)], sems.at[sem])

    def out_copy(r0, n, sem):
        return pltpu.make_async_copy(out_stage.at[pl.ds(r0, n)], out_hbm.at[0, pl.ds(r0, n)], sems.at[sem])

    def w_start(lo, hi, sem):
        for p in range(lo, hi):
            pltpu.make_async_copy(w32[p // 16].at[:, p % 16, :], pool.at[pl.ds(DM * p, DM)],
                                  sems.at[SEM_W0 + sem]).start()

    def w_wait(lo, n, sem):
        r0 = DM * lo if isinstance(lo, int) else pl.multiple_of(DM * lo, DM)
        wait_all(pool.at[pl.ds(r0, DM * n)], SEM_W0 + sem)

    def col_tiles_start(src, dst_of, sem, n):
        for j in range(n):
            pltpu.make_async_copy(src.at[:, pl.ds(128 * j, 128)], dst_of(j), sems.at[sem]).start()

    def wait_all(buf, sem):
        pltpu.make_async_copy(buf, buf, sems.at[sem]).wait()

    for c in range(4):
        x_copy(128 * c, 128, SEM_X0 + c).start()
    w_start(0, 1, 0)
    w_start(1, 2, 1)
    w_start(2, 4, 2)
    w_start(4, 8, 3)
    x_copy(PRE, SEG, SEM_XC).start()
    for i in range(5):
        w_start(8 + 8 * i, 16 + 8 * i, 4 + i)
    x_copy(PRE + SEG, S - PRE - SEG, SEM_XB).start()
    col_tiles_start(wo32, lambda j: wo.at[j], SEM_WO, KT)

    mem_scr[...] = mem0_ref[0].astype(f32)
    zero_scr[...] = jnp.zeros(zero_scr.shape, u32)
    wr_row = wr_ref[...].astype(f32).reshape(1, DM)
    wr_scr[0:8, :] = jnp.broadcast_to(wr_row, (8, DM))
    wr_scr[8:16, :] = jnp.broadcast_to(jnp.sum(wr_row, axis=-1, keepdims=True), (8, DM))
    racc[...] = jnp.full(racc.shape, -jnp.inf, f32)
    qi = lax.broadcasted_iota(jnp.int32, (L2, L2), 0)
    ki = lax.broadcasted_iota(jnp.int32, (L2, L2), 1)
    q_mem, k_mem = qi >= 2 * SEG, ki >= 2 * SEG
    q_head = jnp.where(q_mem, (qi - 2 * SEG) // NMEM, qi // SEG)
    k_head = jnp.where(k_mem, (ki - 2 * SEG) // NMEM, ki // SEG)
    visible = q_mem | k_mem | (qi >= ki)
    fill_scr[...] = jnp.where(q_head == k_head, jnp.where(visible, 0.0, -1e9 * LOG2E), -jnp.inf).astype(f32)

    def ln_rows(r0, n, racc_row, lane_id):
        lane = lax.broadcasted_iota(jnp.int32, (n, 128), 1)
        wr = jnp.concatenate([wr_scr[0:8, :]] * (n // 8), axis=0)
        wr_sum = jnp.concatenate([wr_scr[8:16, 0:1]] * (n // 8), axis=0)
        x = x_scr[pl.ds(r0, n), :].astype(f32)
        mean = jnp.sum(x, axis=-1, keepdims=True) * (1.0 / DM)
        msq = jnp.sum(x * x, axis=-1, keepdims=True) * (1.0 / DM)
        xw = jnp.sum(x * wr, axis=-1, keepdims=True)
        var = jnp.maximum(msq - mean * mean, 0.0)
        inv = 1.0 / _rnd(jnp.sqrt(_rnd(_rnd(var) + EPS_BF16)))
        mean = _rnd(mean)
        xnb = ((x - mean) * inv).astype(bf16)
        xpn_scr[pl.ds(r0, n), :] = x + xnb.astype(f32)
        xnp = _as_u32(xnb)
        p0 = r0 // 2 if isinstance(r0, int) else pl.multiple_of(r0 // 2, 4)
        for k in range(KT):
            xn_pk[k, pl.ds(p0, n // 2), :] = xnp[:, 128 * k:128 * (k + 1)]
        r = _rnd((xw - mean * wr_sum) * inv)
        racc[racc_row:racc_row + n, :] = jnp.where(lane == lane_id, r, racc[racc_row:racc_row + n, :])

    def ln_first(c, carry):
        x_copy(pl.multiple_of(128 * c, 128), 128, SEM_X0 + c).wait()
        for i in range(8):
            ln_rows(pl.multiple_of(c * 128 + 16 * i, 16), 16, 16 * i, c)
        return carry
    lax.fori_loop(0, PRE // 128, ln_first, 0)

    def pro_pairs(t, gs):
        m, c8 = t // 4, t % 4
        sc = (SCALE if m == 0 else None) if isinstance(t, int) else jnp.where(m == 0, SCALE, 1.0).astype(f32)
        for g in gs:
            p0 = DM * (4 * t + g)
            both = pool[pl.ds(p0 if isinstance(t, int) else pl.multiple_of(p0, DM), DM), :]
            pair = (pltpu.bitcast(both << 16, f32).astype(bf16),
                    pltpu.bitcast(both & jnp.uint32(0xFFFF0000), f32).astype(bf16))
            for hh in range(2):
                wqkv[_head(g, c8, hh) * 3 + m] = _as_u32(pair[hh])
                lhs = jnp.concatenate([_as_bf16(xn_pk[k, 0:PRE // 2, :]) for k in range(KT)], axis=1)
                y = _dot(lhs, pair[hh])
                if sc is not None:
                    y = y * sc
                qrings[g][(2 * c8 + hh) * 3 + m, 0:PRE // 2, :] = _as_u32(y.astype(bf16))

    w_wait(0, 1, 0)
    pro_pairs(0, (0,))
    w_wait(1, 1, 1)
    pro_pairs(0, (1,))
    w_wait(2, 2, 2)
    pro_pairs(0, (2, 3))
    w_wait(4, 4, 3)
    x_copy(PRE, SEG, SEM_XC).wait()
    pro_pairs(1, range(NG))
    ln_rows(PRE, TOK, 128, 0)

    def pro_body(i, carry):
        w_wait(8 + 8 * i, 8, 4 + i)
        pro_pairs(2 + 2 * i, range(NG))
        pro_pairs(3 + 2 * i, range(NG))
        return carry
    lax.fori_loop(0, 5, pro_body, 0)
    wait_all(wo, SEM_WO)
    x_copy(PRE + SEG, S - PRE - SEG, SEM_XB).wait()
    col_tiles_start(wg32, lambda j: pool.at[pl.ds(G0 + 512 * j, 512)], SEM_FFN, FT)
    col_tiles_start(wu32, lambda j: pool.at[pl.ds(U0 + 512 * j, 512)], SEM_FFN, FT)
    col_tiles_start(wd32, lambda j: pool.at[pl.ds(D0 + FF // 2 * j, FF // 2)], SEM_FFN, KT)

    def step(s, mem_in, do_ln=True):
        xpos = pl.multiple_of((PRE + TOK * s) // 2, 4)
        wr_pos = [pl.multiple_of(lax.rem(PRE + TOK * s + 8 * i, RQ) // 2, 4) for i in range(3)]
        rd = pl.multiple_of(lax.rem(SEG * s, RQ) // 2, 16)
        owr = pl.multiple_of(lax.rem(SEG * s, RO) // 2, 16)
        orow = pl.multiple_of(TOK * s, 8)
        ord_ = pl.multiple_of(lax.rem(orow, RO) // 2, 4)

        def with_mem(tok_u32, mem_rows):
            tok = _as_bf16(tok_u32)
            last = jnp.concatenate([tok[16:TOK].astype(f32), mem_rows], axis=0).astype(bf16)
            return jnp.concatenate([tok[0:16], last], axis=0)

        zero = zero_scr[0:TOK // 2, :]
        lhs = jnp.concatenate(
            [with_mem(xn_pk[k, pl.ds(xpos, TOK // 2), :] ^ zero, mem_in[:, 128 * k:128 * (k + 1)])
             for k in range(KT)], axis=1)

        mem_parts, probs = {}, {}
        NS = 6
        first = [(c, m, hh) for c in range(4) for m in range(3) for hh in range(2)][:NS]
        lo = {key: _dot(lhs[:, :512], _as_bf16(wqkv[_head(0, key[0], key[2]) * 3 + key[1], 0:256, :])) for key in first}

        def qkv(g, c):
            res = {}
            for m in range(3):
                ms = []
                for hh in range(2):
                    if g == 0 and (c, m, hh) in lo:
                        y = _dot(lhs[:, 512:], _as_bf16(wqkv[_head(g, c, hh) * 3 + m, 256:512, :])) + lo[c, m, hh]
                    else:
                        y = _dot(lhs, _as_bf16(wqkv[_head(g, c, hh) * 3 + m]))
                    if m == 0:
                        y = y * SCALE
                    yp = _as_u32(y.astype(bf16))
                    for i in range(3):
                        qrings[g][(2 * c + hh) * 3 + m, pl.ds(wr_pos[i], 4), :] = yp[4 * i:4 * i + 4]
                    ms.append(y[TOK:])
                res[m] = jnp.concatenate(ms, axis=0).astype(bf16)
            mem_parts[g, c] = [res[m] for m in range(3)]

        def pair_rows(g, c, m, mem_rows):
            t0 = _as_bf16(qrings[g][(2 * c) * 3 + m, pl.ds(rd, SEG // 2), :])
            t1 = _as_bf16(qrings[g][(2 * c + 1) * 3 + m, pl.ds(rd, SEG // 2), :])
            return jnp.concatenate([t0, t1, mem_rows], axis=0)

        def scores(g, c):
            qm, km, vm = mem_parts.pop((g, c))
            sc = lax.dot_general(pair_rows(g, c, 0, qm), pair_rows(g, c, 1, km),
                                 (((1,), (1,)), ((), ())), preferred_element_type=f32)
            fill = fill_scr[...]
            sc = jnp.where(fill == 0.0, sc, fill)
            e = jnp.exp2(sc - jnp.max(sc, axis=-1, keepdims=True))
            r = pl.reciprocal(jnp.sum(e, axis=-1, keepdims=True), approx=True)
            probs[g, c] = (e.astype(bf16), r, vm)

        def pv(g, c):
            e, r, vm = probs.pop((g, c))
            o = _dot(e, pair_rows(g, c, 2, vm)) * r
            for hh in range(2):
                h = 2 * c + hh
                orings[g][h, pl.ds(owr, SEG // 2), :] = _as_u32(o[SEG * hh:SEG * (hh + 1)].astype(bf16))
                om = o[2 * SEG + NMEM * hh:2 * SEG + NMEM * (hh + 1)]
                lhs_os[g][h] = _as_u32(with_mem(orings[g][h, pl.ds(ord_, TOK // 2), :], om))

        acc = [None] * KT

        def out_proj(gs, js):
            for j in js:
                l = jnp.concatenate([_as_bf16(lhs_os[g][k]) for g in gs for k in range(8)], axis=1)
                w = jnp.concatenate(
                    [_as_bf16(wo[j, 64 * _head(g, c, 0):64 * _head(g, c, 0) + 128, :])
                     for g in gs for c in range(4)], axis=0)
                a = _dot(l, w)
                if acc[j] is None:
                    cs = slice(128 * j, 128 * (j + 1))
                    acc[j] = a + jnp.concatenate([xpn_scr[pl.ds(orow, TOK), cs], jnp.zeros((NMEM, 128), f32)], axis=0)
                else:
                    acc[j] = acc[j] + a

        for item in "q0 q1 s0 q2 p0 s1 q3 p1 s2 w01a p2 s3 w012b L0 p3 w2a w3".split():
            g = int(item[1])
            if item[0] == "L":
                if do_ln:
                    nxt = jnp.minimum(s + 1, NSEG - 1)
                    ln_rows(pl.multiple_of(PRE + TOK * nxt, 8), TOK, 128, nxt)
            elif item[0] == "w":
                out_proj([int(ch) for ch in item[1:] if ch.isdigit()],
                         {"a": range(4), "b": range(4, 8)}.get(item[-1], range(8)))
            else:
                for c in range(4):
                    {"q": qkv, "s": scores, "p": pv}[item[0]](g, c)
        a = jnp.concatenate(acc, axis=1)
        out_stage[pl.ds(orow, TOK), :] = a[:TOK].astype(bf16)
        return _rnd(a[TOK:])

    UNR = 3
    PEEL = 1

    def body(u, carry):
        mem = mem_scr[...]
        for i in range(UNR):
            mem = step(UNR * u + i, mem)
        mem_scr[...] = mem
        out_copy(pl.multiple_of(TOK * UNR * u, 8), UNR * TOK, SEM_OUT).start()
        return carry
    lax.fori_loop(0, (NSEG - PEEL) // UNR, body, 0)

    wait_all(pool.at[pl.ds(0, FFN_ROWS)], SEM_FFN)

    mem = mem_scr[...]
    for s in range(NSEG - PEEL, NSEG):
        mem = step(jnp.int32(s), mem, do_ln=s < NSEG - 1)
    if PEEL:
        out_copy(TOK * (NSEG - PEEL), PEEL * TOK, SEM_OUT).start()

    rv = racc[...]
    rrow = lax.broadcasted_iota(jnp.int32, rv.shape, 0)
    rlane = lax.broadcasted_iota(jnp.int32, rv.shape, 1)
    ridx = jnp.where(rrow < 128, rrow + 128 * rlane, PRE + (rrow - 128) + TOK * rlane).astype(f32)
    m0 = jnp.max(rv, keepdims=True)
    f0 = jnp.min(jnp.where(rv == m0, ridx, 1e9), keepdims=True)
    rv2 = jnp.where(ridx == f0, -jnp.inf, rv)
    m1 = jnp.max(rv2, keepdims=True)
    f1 = jnp.min(jnp.where(rv2 == m1, ridx, 1e9), keepdims=True)
    i0 = jnp.clip(f0[0, 0].astype(jnp.int32), 0, S - 1)
    i1 = jnp.clip(f1[0, 0].astype(jnp.int32), 0, S - 1)
    row16 = lax.broadcasted_iota(jnp.int32, (16, DM), 0)

    def xn_row(i):
        w = jnp.concatenate([xn_pk[k, pl.ds(i // 2, 1), :] for k in range(KT)], axis=1)
        return pltpu.bitcast(jnp.where(i % 2 == 0, w << 16, w & jnp.uint32(0xFFFF0000)), f32)
    row8 = lax.broadcasted_iota(jnp.int32, (8, DM), 0)
    xsel = jnp.where(row8 == 0, xn_row(i0), jnp.where(row8 == 1, xn_row(i1), 0.0))

    e0 = NSEG * TOK
    last = S - 128
    part = {}

    def add(key, v):
        part[key] = v if key not in part else v + part[key]

    def e_round(b, j, r):
        l = jnp.concatenate(
            [_as_bf16(orings[(h % 8) // 2][2 * (h // 8) + h % 2, 64 * b:64 * (b + 1), :])
             for h in range(4 * r, 4 * r + 4)], axis=1)
        add(("e", b, j), _dot(l, _as_bf16(wo[j, 256 * r:256 * (r + 1), :])))
        if r == 7:
            rows, cs = slice(e0 + 128 * b, e0 + 128 * (b + 1)), slice(128 * j, 128 * (j + 1))
            out_stage[rows, cs] = (part.pop(("e", b, j)) + xpn_scr[rows, cs]).astype(bf16)
            if j == KT - 1:
                out_copy(e0 + 128 * b, 128, SEM_OUT if b < 3 else SEM_OUT2).start()

    def up_round(w, name, j, r):
        wt = _as_bf16(pool[pl.ds(w + 512 * j + 256 * r, 256), :]).astype(f32)
        add((name, j), _dot(xsel[:, 512 * r:512 * (r + 1)], wt))
        if name == "u" and r == 1:
            gate = part.pop(("g", j))
            part["h", j] = _rnd(gate * jax.nn.sigmoid(gate) * part.pop(("u", j)))

    def down_round(j, r):
        hid = jnp.concatenate([part["h", k] for k in range(4 * r, 4 * r + 4)], axis=1)
        add(("y", j), _dot(hid, _as_bf16(pool[pl.ds(D0 + FF // 2 * j + 256 * r, 256), :]).astype(f32)))

    e_rounds = [(b, j, r) for b in range(4) for j in range(KT) for r in range(8)]
    m_rounds = [lambda j=j, r=r, w=w, n=n: up_round(w, n, j, r)
                for j in range(FT) for (w, n) in ((G0, "g"), (U0, "u")) for r in range(2)]
    m_rounds += [None] * 2
    m_rounds += [lambda j=j, r=r: down_round(j, r) for r in range(FT // 4) for j in range(KT)]
    m_rounds = [None] * 1 + m_rounds
    NM = 1
    for n, er in enumerate(e_rounds[:192]):
        e_round(*er)
        for mr in m_rounds[NM * n:NM * n + NM]:
            if mr is not None:
                mr()
    assert len(m_rounds) <= NM * 192
    rsel = jnp.where(lax.broadcasted_iota(jnp.int32, (8, 1), 0) == 0, m0, m1)
    y = jnp.concatenate([part.pop(("y", j)) for j in range(KT)], axis=1) * jax.nn.sigmoid(rsel)
    y0, y1 = y[0:1], y[1:2]
    xpn_scr[pl.ds(i0, 1), :] = xpn_scr[pl.ds(i0, 1), :] + jnp.where(i0 >= last, y0, 0.0)
    xpn_scr[pl.ds(i1, 1), :] = xpn_scr[pl.ds(i1, 1), :] + jnp.where(i1 >= last, y1, 0.0)
    for er in e_rounds[192:]:
        e_round(*er)

    out_copy(0, last, SEM_OUT).wait()
    g0 = pl.multiple_of((i0 // 16) * 16, 16)
    g1 = pl.multiple_of((i1 // 16) * 16, 16)
    redo0 = i0 < last
    redo1 = i1 < last
    send1 = jnp.logical_and(redo1, g1 != g0)

    def patch(i, gst, yy):
        blk = out_stage[pl.ds(gst, 16), :].astype(f32)
        out_stage[pl.ds(gst, 16), :] = (blk + jnp.where(row16 == i - gst, yy, 0.0)).astype(bf16)

    @pl.when(redo0)
    def _():
        patch(i0, g0, y0)

    @pl.when(redo1)
    def _():
        patch(i1, g1, y1)

    @pl.when(redo0)
    def _():
        out_copy(g0, 16, SEM_P0).start()

    @pl.when(send1)
    def _():
        out_copy(g1, 16, SEM_P1).start()

    out_copy(last, 128, SEM_OUT2).wait()

    @pl.when(redo0)
    def _():
        out_copy(g0, 16, SEM_P0).wait()

    @pl.when(send1)
    def _():
        out_copy(g1, 16, SEM_P1).wait()


@jax.jit
def pallas_parallel_sum__memory_aug_recurrent_mem_tr__moe_arch_mod__prompt_kernel(
    A_x: jax.Array,
    A_mem0: jax.Array,
    A_Wq: jax.Array,
    A_Wk: jax.Array,
    A_Wv: jax.Array,
    A_Wo: jax.Array,
    A_seg_len: jax.Array,
    B_x: jax.Array,
    B_w_r: jax.Array,
    B_w_gate: jax.Array,
    B_w_up: jax.Array,
    B_w_down: jax.Array,
):
    del A_seg_len, B_x
    assert A_x.shape == (1, S, DM) and A_mem0.shape == (1, NMEM, DM)
    assert A_Wq.shape == (DM, H, DH) and A_Wo.shape == (H, DH, DM) and B_w_gate.shape == (DM, FF)
    hbm = pl.BlockSpec(memory_space=pl.ANY)
    vmem = pl.BlockSpec(memory_space=pltpu.VMEM)
    scratch = [
        pltpu.VMEM((S, DM), bf16),
        pltpu.VMEM((S, DM), f32),
        pltpu.VMEM((KT, S // 2, 128), u32),
        pltpu.VMEM((16, DM), f32),
        pltpu.VMEM((48 * DM, 128), u32),
        pltpu.VMEM((3 * H, DM // 2, 128), u32),
        pltpu.VMEM((KT, H * DH // 2, 128), u32),
    ]
    scratch += [pltpu.VMEM((24, RQ // 2, 128), u32)] * NG
    scratch += [pltpu.VMEM((8, RO // 2, 128), u32)] * NG
    scratch += [pltpu.VMEM((8, 16, 128), u32)] * NG
    scratch += [
        pltpu.VMEM((NMEM, DM), f32),
        pltpu.VMEM((16, 128), u32),
        pltpu.VMEM((L2, L2), f32),
        pltpu.VMEM((128 + TOK, 128), f32),
        pltpu.VMEM((S, DM), bf16),
        pltpu.SemaphoreType.DMA((NSEM,)),
    ]
    return pl.pallas_call(
        _kernel,
        out_shape=jax.ShapeDtypeStruct((1, S, DM), bf16),
        in_specs=[hbm, vmem, hbm, hbm, hbm, hbm, vmem, hbm, hbm, hbm],
        out_specs=hbm,
        scratch_shapes=scratch,
        compiler_params=pltpu.CompilerParams(vmem_limit_bytes=110 * 1024 * 1024,
                                             disable_bounds_checks=True),
    )(A_x, A_mem0, A_Wq, A_Wk, A_Wv, A_Wo.reshape(H * DH, DM), B_w_r, B_w_gate, B_w_up, B_w_down)
```

```python
import jax
import jax.numpy as jnp
from jax import lax
import jax.experimental.pallas as pl
import jax.experimental.pallas.tpu as pltpu

bf16 = jnp.bfloat16
f32 = jnp.float32
u32 = jnp.uint32

S, DM, H, DH, NMEM, SEG, FF = 2048, 1024, 32, 128, 8, 32, 3584
NSEG = S // SEG
TOK = 24
PRE = S - NSEG * TOK
RQ = 544
RO = 768
NG = 4
KT = DM // 128
FT = FF // 128
L2 = 2 * (SEG + NMEM)
LOG2E = 1.4426950408889634
SCALE = DH ** -0.5 * LOG2E
EPS_BF16 = 1.0013580322265625e-05

SEM_W0 = 0
SEM_X0 = 9
SEM_XB, SEM_XC, SEM_WO, SEM_FFN, SEM_OUT, SEM_P0, SEM_P1, SEM_OUT2 = range(13, 21)
NSEM = 21
G0, U0, D0 = 0, FT * DM // 2, 2 * FT * DM // 2
FFN_ROWS = D0 + KT * FF // 2


def _as_bf16(x):
    return pltpu.bitcast(x, bf16)


def _as_u32(x):
    return pltpu.bitcast(x, u32)


def _rnd(x):
    return x.astype(bf16).astype(f32)


def _dot(a, b):
    return jnp.dot(a, b, preferred_element_type=f32)


def _head(g, c, hh):
    return 8 * c + 2 * g + hh


def _kernel(x_hbm, mem0_ref, wq_hbm, wk_hbm, wv_hbm, wo_hbm, wr_ref, wg_hbm, wu_hbm, wd_hbm,
            out_hbm,
            x_scr, xpn_scr, xn_pk, wr_scr, pool, wqkv, wo,
            qr0, qr1, qr2, qr3, or0, or1, or2, or3, lo0, lo1, lo2, lo3,
            mem_scr, zero_scr, fill_scr, racc, out_stage, sems):
    qrings = (qr0, qr1, qr2, qr3)
    orings = (or0, or1, or2, or3)
    lhs_os = (lo0, lo1, lo2, lo3)
    w32 = [w.bitcast(u32) for w in (wq_hbm, wk_hbm, wv_hbm)]
    wo32 = wo_hbm.bitcast(u32)
    wg32 = wg_hbm.bitcast(u32)
    wu32 = wu_hbm.bitcast(u32)
    wd32 = wd_hbm.bitcast(u32)

    def x_copy(r0, n, sem):
        return pltpu.make_async_copy(x_hbm.at[0, pl.ds(r0, n)], x_scr.at[pl.ds(r0, n)], sems.at[sem])

    def out_copy(r0, n, sem):
        return pltpu.make_async_copy(out_stage.at[pl.ds(r0, n)], out_hbm.at[0, pl.ds(r0, n)], sems.at[sem])

    def w_start(lo, hi, sem):
        for p in range(lo, hi):
            pltpu.make_async_copy(w32[p // 16].at[:, p % 16, :], pool.at[pl.ds(DM * p, DM)],
                                  sems.at[SEM_W0 + sem]).start()

    def w_wait(lo, n, sem):
        r0 = DM * lo if isinstance(lo, int) else pl.multiple_of(DM * lo, DM)
        wait_all(pool.at[pl.ds(r0, DM * n)], SEM_W0 + sem)

    def col_tiles_start(src, dst_of, sem, n):
        for j in range(n):
            pltpu.make_async_copy(src.at[:, pl.ds(128 * j, 128)], dst_of(j), sems.at[sem]).start()

    def wait_all(buf, sem):
        pltpu.make_async_copy(buf, buf, sems.at[sem]).wait()

    for c in range(4):
        x_copy(128 * c, 128, SEM_X0 + c).start()
    w_start(0, 1, 0)
    w_start(1, 2, 1)
    w_start(2, 4, 2)
    w_start(4, 8, 3)
    x_copy(PRE, SEG, SEM_XC).start()
    for i in range(5):
        w_start(8 + 8 * i, 16 + 8 * i, 4 + i)
    x_copy(PRE + SEG, S - PRE - SEG, SEM_XB).start()
    col_tiles_start(wo32, lambda j: wo.at[j], SEM_WO, KT)

    mem_scr[...] = mem0_ref[0].astype(f32)
    zero_scr[...] = jnp.zeros(zero_scr.shape, u32)
    wr_row = wr_ref[...].astype(f32).reshape(1, DM)
    wr_scr[0:8, :] = jnp.broadcast_to(wr_row, (8, DM))
    wr_scr[8:16, :] = jnp.broadcast_to(jnp.sum(wr_row, axis=-1, keepdims=True), (8, DM))
    racc[...] = jnp.full(racc.shape, -jnp.inf, f32)
    qi = lax.broadcasted_iota(jnp.int32, (L2, L2), 0)
    ki = lax.broadcasted_iota(jnp.int32, (L2, L2), 1)
    q_mem, k_mem = qi >= 2 * SEG, ki >= 2 * SEG
    q_head = jnp.where(q_mem, (qi - 2 * SEG) // NMEM, qi // SEG)
    k_head = jnp.where(k_mem, (ki - 2 * SEG) // NMEM, ki // SEG)
    visible = q_mem | k_mem | (qi >= ki)
    fill_scr[...] = jnp.where(q_head == k_head, jnp.where(visible, 0.0, -1e9 * LOG2E), -jnp.inf).astype(f32)

    def ln_rows(r0, n, racc_row, lane_id):
        lane = lax.broadcasted_iota(jnp.int32, (n, 128), 1)
        wr = jnp.concatenate([wr_scr[0:8, :]] * (n // 8), axis=0)
        wr_sum = jnp.concatenate([wr_scr[8:16, 0:1]] * (n // 8), axis=0)
        x = x_scr[pl.ds(r0, n), :].astype(f32)
        mean = jnp.sum(x, axis=-1, keepdims=True) * (1.0 / DM)
        msq = jnp.sum(x * x, axis=-1, keepdims=True) * (1.0 / DM)
        xw = jnp.sum(x * wr, axis=-1, keepdims=True)
        var = jnp.maximum(msq - mean * mean, 0.0)
        inv = 1.0 / _rnd(jnp.sqrt(_rnd(_rnd(var) + EPS_BF16)))
        mean = _rnd(mean)
        xnb = ((x - mean) * inv).astype(bf16)
        xpn_scr[pl.ds(r0, n), :] = x + xnb.astype(f32)
        xnp = _as_u32(xnb)
        p0 = r0 // 2 if isinstance(r0, int) else pl.multiple_of(r0 // 2, 4)
        for k in range(KT):
            xn_pk[k, pl.ds(p0, n // 2), :] = xnp[:, 128 * k:128 * (k + 1)]
        r = _rnd((xw - mean * wr_sum) * inv)
        racc[racc_row:racc_row + n, :] = jnp.where(lane == lane_id, r, racc[racc_row:racc_row + n, :])

    def ln_first(c, carry):
        x_copy(pl.multiple_of(128 * c, 128), 128, SEM_X0 + c).wait()
        for i in range(8):
            ln_rows(pl.multiple_of(c * 128 + 16 * i, 16), 16, 16 * i, c)
        return carry
    lax.fori_loop(0, PRE // 128, ln_first, 0)

    def pro_pairs(t, gs):
        m, c8 = t // 4, t % 4
        sc = (SCALE if m == 0 else None) if isinstance(t, int) else jnp.where(m == 0, SCALE, 1.0).astype(f32)
        for g in gs:
            p0 = DM * (4 * t + g)
            both = pool[pl.ds(p0 if isinstance(t, int) else pl.multiple_of(p0, DM), DM), :]
            pair = (pltpu.bitcast(both << 16, f32).astype(bf16),
                    pltpu.bitcast(both & jnp.uint32(0xFFFF0000), f32).astype(bf16))
            for hh in range(2):
                wqkv[_head(g, c8, hh) * 3 + m] = _as_u32(pair[hh])
                lhs = jnp.concatenate([_as_bf16(xn_pk[k, 0:PRE // 2, :]) for k in range(KT)], axis=1)
                y = _dot(lhs, pair[hh])
                if sc is not None:
                    y = y * sc
                qrings[g][(2 * c8 + hh) * 3 + m, 0:PRE // 2, :] = _as_u32(y.astype(bf16))

    w_wait(0, 1, 0)
    pro_pairs(0, (0,))
    w_wait(1, 1, 1)
    pro_pairs(0, (1,))
    w_wait(2, 2, 2)
    pro_pairs(0, (2, 3))
    w_wait(4, 4, 3)
    x_copy(PRE, SEG, SEM_XC).wait()
    pro_pairs(1, range(NG))
    ln_rows(PRE, TOK, 128, 0)

    def pro_body(i, carry):
        w_wait(8 + 8 * i, 8, 4 + i)
        pro_pairs(2 + 2 * i, range(NG))
        pro_pairs(3 + 2 * i, range(NG))
        return carry
    lax.fori_loop(0, 5, pro_body, 0)
    wait_all(wo, SEM_WO)
    x_copy(PRE + SEG, S - PRE - SEG, SEM_XB).wait()
    col_tiles_start(wg32, lambda j: pool.at[pl.ds(G0 + 512 * j, 512)], SEM_FFN, FT)
    col_tiles_start(wu32, lambda j: pool.at[pl.ds(U0 + 512 * j, 512)], SEM_FFN, FT)
    col_tiles_start(wd32, lambda j: pool.at[pl.ds(D0 + FF // 2 * j, FF // 2)], SEM_FFN, KT)

    def step(s, mem_in, do_ln=True):
        xpos = pl.multiple_of((PRE + TOK * s) // 2, 4)
        wr_pos = [pl.multiple_of(lax.rem(PRE + TOK * s + 8 * i, RQ) // 2, 4) for i in range(3)]
        rd = pl.multiple_of(lax.rem(SEG * s, RQ) // 2, 16)
        owr = pl.multiple_of(lax.rem(SEG * s, RO) // 2, 16)
        orow = pl.multiple_of(TOK * s, 8)
        ord_ = pl.multiple_of(lax.rem(orow, RO) // 2, 4)

        def with_mem(tok_u32, mem_rows):
            tok = _as_bf16(tok_u32)
            last = jnp.concatenate([tok[16:TOK].astype(f32), mem_rows], axis=0).astype(bf16)
            return jnp.concatenate([tok[0:16], last], axis=0)

        zero = zero_scr[0:TOK // 2, :]
        lhs = jnp.concatenate(
            [with_mem(xn_pk[k, pl.ds(xpos, TOK // 2), :] ^ zero, mem_in[:, 128 * k:128 * (k + 1)])
             for k in range(KT)], axis=1)

        mem_parts, probs = {}, {}
        NS = 6
        first = [(c, m, hh) for c in range(4) for m in range(3) for hh in range(2)][:NS]
        lo = {key: _dot(lhs[:, :512], _as_bf16(wqkv[_head(0, key[0], key[2]) * 3 + key[1], 0:256, :])) for key in first}

        def qkv(g, c):
            res = {}
            for m in range(3):
                ms = []
                for hh in range(2):
                    if g == 0 and (c, m, hh) in lo:
                        y = _dot(lhs[:, 512:], _as_bf16(wqkv[_head(g, c, hh) * 3 + m, 256:512, :])) + lo[c, m, hh]
                    else:
                        y = _dot(lhs, _as_bf16(wqkv[_head(g, c, hh) * 3 + m]))
                    if m == 0:
                        y = y * SCALE
                    yp = _as_u32(y.astype(bf16))
                    for i in range(3):
                        qrings[g][(2 * c + hh) * 3 + m, pl.ds(wr_pos[i], 4), :] = yp[4 * i:4 * i + 4]
                    ms.append(y[TOK:])
                res[m] = jnp.concatenate(ms, axis=0).astype(bf16)
            mem_parts[g, c] = [res[m] for m in range(3)]

        def pair_rows(g, c, m, mem_rows):
            t0 = _as_bf16(qrings[g][(2 * c) * 3 + m, pl.ds(rd, SEG // 2), :])
            t1 = _as_bf16(qrings[g][(2 * c + 1) * 3 + m, pl.ds(rd, SEG // 2), :])
            return jnp.concatenate([t0, t1, mem_rows], axis=0)

        def scores(g, c):
            qm, km, vm = mem_parts.pop((g, c))
            sc = lax.dot_general(pair_rows(g, c, 0, qm), pair_rows(g, c, 1, km),
                                 (((1,), (1,)), ((), ())), preferred_element_type=f32)
            fill = fill_scr[...]
            sc = jnp.where(fill == 0.0, sc, fill)
            e = jnp.exp2(sc - jnp.max(sc, axis=-1, keepdims=True))
            r = pl.reciprocal(jnp.sum(e, axis=-1, keepdims=True), approx=True)
            probs[g, c] = (e.astype(bf16), r, vm)

        def pv(g, c):
            e, r, vm = probs.pop((g, c))
            o = _dot(e, pair_rows(g, c, 2, vm)) * r
            for hh in range(2):
                h = 2 * c + hh
                orings[g][h, pl.ds(owr, SEG // 2), :] = _as_u32(o[SEG * hh:SEG * (hh + 1)].astype(bf16))
                om = o[2 * SEG + NMEM * hh:2 * SEG + NMEM * (hh + 1)]
                lhs_os[g][h] = _as_u32(with_mem(orings[g][h, pl.ds(ord_, TOK // 2), :], om))

        acc = [None] * KT

        def out_proj(gs, js):
            for j in js:
                l = jnp.concatenate([_as_bf16(lhs_os[g][k]) for g in gs for k in range(8)], axis=1)
                w = jnp.concatenate(
                    [_as_bf16(wo[j, 64 * _head(g, c, 0):64 * _head(g, c, 0) + 128, :])
                     for g in gs for c in range(4)], axis=0)
                a = _dot(l, w)
                if acc[j] is None:
                    cs = slice(128 * j, 128 * (j + 1))
                    acc[j] = a + jnp.concatenate([xpn_scr[pl.ds(orow, TOK), cs], jnp.zeros((NMEM, 128), f32)], axis=0)
                else:
                    acc[j] = acc[j] + a

        for item in "q0 q1 s0 q2 p0 s1 q3 p1 s2 w01a p2 s3 w012b L0 p3 w2a w3".split():
            g = int(item[1])
            if item[0] == "L":
                if do_ln:
                    nxt = jnp.minimum(s + 1, NSEG - 1)
                    ln_rows(pl.multiple_of(PRE + TOK * nxt, 8), TOK, 128, nxt)
            elif item[0] == "w":
                out_proj([int(ch) for ch in item[1:] if ch.isdigit()],
                         {"a": range(4), "b": range(4, 8)}.get(item[-1], range(8)))
            else:
                for c in range(4):
                    {"q": qkv, "s": scores, "p": pv}[item[0]](g, c)
        a = jnp.concatenate(acc, axis=1)
        out_stage[pl.ds(orow, TOK), :] = a[:TOK].astype(bf16)
        return _rnd(a[TOK:])

    UNR = 3
    PEEL = 1

    def body(u, carry):
        mem = mem_scr[...]
        for i in range(UNR):
            mem = step(UNR * u + i, mem)
        mem_scr[...] = mem
        out_copy(pl.multiple_of(TOK * UNR * u, 8), UNR * TOK, SEM_OUT).start()
        return carry
    lax.fori_loop(0, (NSEG - PEEL) // UNR, body, 0)

    wait_all(pool.at[pl.ds(0, FFN_ROWS)], SEM_FFN)

    mem = mem_scr[...]
    for s in range(NSEG - PEEL, NSEG):
        mem = step(jnp.int32(s), mem, do_ln=s < NSEG - 1)
    if PEEL:
        out_copy(TOK * (NSEG - PEEL), PEEL * TOK, SEM_OUT).start()

    rv = racc[...]
    rrow = lax.broadcasted_iota(jnp.int32, rv.shape, 0)
    rlane = lax.broadcasted_iota(jnp.int32, rv.shape, 1)
    ridx = jnp.where(rrow < 128, rrow + 128 * rlane, PRE + (rrow - 128) + TOK * rlane).astype(f32)
    m0 = jnp.max(rv, keepdims=True)
    f0 = jnp.min(jnp.where(rv == m0, ridx, 1e9), keepdims=True)
    rv2 = jnp.where(ridx == f0, -jnp.inf, rv)
    m1 = jnp.max(rv2, keepdims=True)
    f1 = jnp.min(jnp.where(rv2 == m1, ridx, 1e9), keepdims=True)
    i0 = jnp.clip(f0[0, 0].astype(jnp.int32), 0, S - 1)
    i1 = jnp.clip(f1[0, 0].astype(jnp.int32), 0, S - 1)
    row16 = lax.broadcasted_iota(jnp.int32, (16, DM), 0)

    def xn_row(i):
        w = jnp.concatenate([xn_pk[k, pl.ds(i // 2, 1), :] for k in range(KT)], axis=1)
        return pltpu.bitcast(jnp.where(i % 2 == 0, w << 16, w & jnp.uint32(0xFFFF0000)), f32)
    row8 = lax.broadcasted_iota(jnp.int32, (8, DM), 0)
    xsel = jnp.where(row8 == 0, xn_row(i0), jnp.where(row8 == 1, xn_row(i1), 0.0))

    e0 = NSEG * TOK
    e_rows = ((0, 128), (128, 128), (256, 128), (384, 96), (480, 32))
    last = S - 128
    part = {}

    def add(key, v):
        part[key] = v if key not in part else v + part[key]

    def e_round(b, j, r):
        r0, n = e_rows[b]
        l = jnp.concatenate(
            [_as_bf16(orings[(h % 8) // 2][2 * (h // 8) + h % 2, r0 // 2:(r0 + n) // 2, :])
             for h in range(4 * r, 4 * r + 4)], axis=1)
        add(("e", b, j), _dot(l, _as_bf16(wo[j, 256 * r:256 * (r + 1), :])))
        if r == 7:
            rows, cs = slice(e0 + r0, e0 + r0 + n), slice(128 * j, 128 * (j + 1))
            out_stage[rows, cs] = (part.pop(("e", b, j)) + xpn_scr[rows, cs]).astype(bf16)
            if j == KT - 1:
                out_copy(e0 + r0, n, SEM_OUT if b < 3 else SEM_OUT2).start()

    def up_round(w, name, j, r):
        wt = _as_bf16(pool[pl.ds(w + 512 * j + 256 * r, 256), :]).astype(f32)
        add((name, j), _dot(xsel[:, 512 * r:512 * (r + 1)], wt))
        if name == "u" and r == 1:
            gate = part.pop(("g", j))
            part["h", j] = _rnd(gate * jax.nn.sigmoid(gate) * part.pop(("u", j)))

    def down_round(j, r):
        hid = jnp.concatenate([part["h", k] for k in range(4 * r, 4 * r + 4)], axis=1)
        add(("y", j), _dot(hid, _as_bf16(pool[pl.ds(D0 + FF // 2 * j + 256 * r, 256), :]).astype(f32)))

    e_rounds = [(b, j, r) for b in range(5) for j in range(KT) for r in range(8)]
    m_rounds = [lambda j=j, r=r, w=w, n=n: up_round(w, n, j, r)
                for j in range(FT) for (w, n) in ((G0, "g"), (U0, "u")) for r in range(2)]
    m_rounds += [None] * 2
    m_rounds += [lambda j=j, r=r: down_round(j, r) for r in range(FT // 4) for j in range(KT)]
    m_rounds = [None] * 1 + m_rounds
    NM = 1
    for n, er in enumerate(e_rounds[:192]):
        e_round(*er)
        for mr in m_rounds[NM * n:NM * n + NM]:
            if mr is not None:
                mr()
    assert len(m_rounds) <= NM * 192
    rsel = jnp.where(lax.broadcasted_iota(jnp.int32, (8, 1), 0) == 0, m0, m1)
    y = jnp.concatenate([part.pop(("y", j)) for j in range(KT)], axis=1) * jax.nn.sigmoid(rsel)
    y0, y1 = y[0:1], y[1:2]
    xpn_scr[pl.ds(i0, 1), :] = xpn_scr[pl.ds(i0, 1), :] + jnp.where(i0 >= last, y0, 0.0)
    xpn_scr[pl.ds(i1, 1), :] = xpn_scr[pl.ds(i1, 1), :] + jnp.where(i1 >= last, y1, 0.0)
    for er in e_rounds[192:]:
        e_round(*er)

    out_copy(0, last, SEM_OUT).wait()
    g0 = pl.multiple_of((i0 // 16) * 16, 16)
    g1 = pl.multiple_of((i1 // 16) * 16, 16)
    redo0 = i0 < last
    redo1 = i1 < last
    send1 = jnp.logical_and(redo1, g1 != g0)

    def patch(i, gst, yy):
        blk = out_stage[pl.ds(gst, 16), :].astype(f32)
        out_stage[pl.ds(gst, 16), :] = (blk + jnp.where(row16 == i - gst, yy, 0.0)).astype(bf16)

    @pl.when(redo0)
    def _():
        patch(i0, g0, y0)

    @pl.when(redo1)
    def _():
        patch(i1, g1, y1)

    @pl.when(redo0)
    def _():
        out_copy(g0, 16, SEM_P0).start()

    @pl.when(send1)
    def _():
        out_copy(g1, 16, SEM_P1).start()

    out_copy(last, 128, SEM_OUT2).wait()

    @pl.when(redo0)
    def _():
        out_copy(g0, 16, SEM_P0).wait()

    @pl.when(send1)
    def _():
        out_copy(g1, 16, SEM_P1).wait()


@jax.jit
def pallas_parallel_sum__memory_aug_recurrent_mem_tr__moe_arch_mod__prompt_kernel(
    A_x: jax.Array,
    A_mem0: jax.Array,
    A_Wq: jax.Array,
    A_Wk: jax.Array,
    A_Wv: jax.Array,
    A_Wo: jax.Array,
    A_seg_len: jax.Array,
    B_x: jax.Array,
    B_w_r: jax.Array,
    B_w_gate: jax.Array,
    B_w_up: jax.Array,
    B_w_down: jax.Array,
):
    del A_seg_len, B_x
    assert A_x.shape == (1, S, DM) and A_mem0.shape == (1, NMEM, DM)
    assert A_Wq.shape == (DM, H, DH) and A_Wo.shape == (H, DH, DM) and B_w_gate.shape == (DM, FF)
    hbm = pl.BlockSpec(memory_space=pl.ANY)
    vmem = pl.BlockSpec(memory_space=pltpu.VMEM)
    scratch = [
        pltpu.VMEM((S, DM), bf16),
        pltpu.VMEM((S, DM), f32),
        pltpu.VMEM((KT, S // 2, 128), u32),
        pltpu.VMEM((16, DM), f32),
        pltpu.VMEM((48 * DM, 128), u32),
        pltpu.VMEM((3 * H, DM // 2, 128), u32),
        pltpu.VMEM((KT, H * DH // 2, 128), u32),
    ]
    scratch += [pltpu.VMEM((24, RQ // 2, 128), u32)] * NG
    scratch += [pltpu.VMEM((8, RO // 2, 128), u32)] * NG
    scratch += [pltpu.VMEM((8, 16, 128), u32)] * NG
    scratch += [
        pltpu.VMEM((NMEM, DM), f32),
        pltpu.VMEM((16, 128), u32),
        pltpu.VMEM((L2, L2), f32),
        pltpu.VMEM((128 + TOK, 128), f32),
        pltpu.VMEM((S, DM), bf16),
        pltpu.SemaphoreType.DMA((NSEM,)),
    ]
    return pl.pallas_call(
        _kernel,
        out_shape=jax.ShapeDtypeStruct((1, S, DM), bf16),
        in_specs=[hbm, vmem, hbm, hbm, hbm, hbm, vmem, hbm, hbm, hbm],
        out_specs=hbm,
        scratch_shapes=scratch,
        compiler_params=pltpu.CompilerParams(vmem_limit_bytes=110 * 1024 * 1024,
                                             disable_bounds_checks=True),
    )(A_x, A_mem0, A_Wq, A_Wk, A_Wv, A_Wo.reshape(H * DH, DM), B_w_r, B_w_gate, B_w_up, B_w_down)
```

```python
import jax
import jax.numpy as jnp
from jax import lax
import jax.experimental.pallas as pl
import jax.experimental.pallas.tpu as pltpu

bf16 = jnp.bfloat16
f32 = jnp.float32
u32 = jnp.uint32

S, DM, H, DH, NMEM, SEG, FF = 2048, 1024, 32, 128, 8, 32, 3584
NSEG = S // SEG
TOK = 24
PRE = S - NSEG * TOK
RQ = 544
RO = 768
NG = 4
KT = DM // 128
FT = FF // 128
L2 = 2 * (SEG + NMEM)
LOG2E = 1.4426950408889634
SCALE = DH ** -0.5 * LOG2E
EPS_BF16 = 1.0013580322265625e-05

SEM_W0 = 0
SEM_X0 = 9
SEM_XB, SEM_XC, SEM_WO, SEM_FFN, SEM_OUT, SEM_P0, SEM_P1, SEM_OUT2 = range(13, 21)
NSEM = 21
G0, U0, D0 = 0, FT * DM // 2, 2 * FT * DM // 2
FFN_ROWS = D0 + KT * FF // 2


def _as_bf16(x):
    return pltpu.bitcast(x, bf16)


def _as_u32(x):
    return pltpu.bitcast(x, u32)


def _rnd(x):
    return x.astype(bf16).astype(f32)


def _dot(a, b):
    return jnp.dot(a, b, preferred_element_type=f32)


def _head(g, c, hh):
    return 8 * c + 2 * g + hh


def _kernel(x_hbm, mem0_ref, wq_hbm, wk_hbm, wv_hbm, wo_hbm, wr_ref, wg_hbm, wu_hbm, wd_hbm,
            out_hbm,
            x_scr, xpn_scr, xn_pk, wr_scr, pool, wqkv, wo,
            qr0, qr1, qr2, qr3, or0, or1, or2, or3, lo0, lo1, lo2, lo3,
            mem_scr, zero_scr, fill_scr, racc, out_stage, sems):
    qrings = (qr0, qr1, qr2, qr3)
    orings = (or0, or1, or2, or3)
    lhs_os = (lo0, lo1, lo2, lo3)
    w32 = [w.bitcast(u32) for w in (wq_hbm, wk_hbm, wv_hbm)]
    wo32 = wo_hbm.bitcast(u32)
    wg32 = wg_hbm.bitcast(u32)
    wu32 = wu_hbm.bitcast(u32)
    wd32 = wd_hbm.bitcast(u32)

    def x_copy(r0, n, sem):
        return pltpu.make_async_copy(x_hbm.at[0, pl.ds(r0, n)], x_scr.at[pl.ds(r0, n)], sems.at[sem])

    def out_copy(r0, n, sem):
        return pltpu.make_async_copy(out_stage.at[pl.ds(r0, n)], out_hbm.at[0, pl.ds(r0, n)], sems.at[sem])

    def w_start(lo, hi, sem):
        for p in range(lo, hi):
            pltpu.make_async_copy(w32[p // 16].at[:, p % 16, :], pool.at[pl.ds(DM * p, DM)],
                                  sems.at[SEM_W0 + sem]).start()

    def w_wait(lo, n, sem):
        r0 = DM * lo if isinstance(lo, int) else pl.multiple_of(DM * lo, DM)
        wait_all(pool.at[pl.ds(r0, DM * n)], SEM_W0 + sem)

    def col_tiles_start(src, dst_of, sem, n):
        for j in range(n):
            pltpu.make_async_copy(src.at[:, pl.ds(128 * j, 128)], dst_of(j), sems.at[sem]).start()

    def wait_all(buf, sem):
        pltpu.make_async_copy(buf, buf, sems.at[sem]).wait()

    for c in range(4):
        x_copy(128 * c, 128, SEM_X0 + c).start()
    w_start(0, 1, 0)
    w_start(1, 2, 1)
    w_start(2, 4, 2)
    w_start(4, 8, 3)
    x_copy(PRE, SEG, SEM_XC).start()
    for i in range(5):
        w_start(8 + 8 * i, 16 + 8 * i, 4 + i)
    x_copy(PRE + SEG, S - PRE - SEG, SEM_XB).start()
    col_tiles_start(wo32, lambda j: wo.at[j], SEM_WO, KT)

    mem_scr[...] = mem0_ref[0].astype(f32)
    zero_scr[...] = jnp.zeros(zero_scr.shape, u32)
    wr_row = wr_ref[...].astype(f32).reshape(1, DM)
    wr_scr[0:8, :] = jnp.broadcast_to(wr_row, (8, DM))
    wr_scr[8:16, :] = jnp.broadcast_to(jnp.sum(wr_row, axis=-1, keepdims=True), (8, DM))
    racc[...] = jnp.full(racc.shape, -jnp.inf, f32)
    qi = lax.broadcasted_iota(jnp.int32, (L2, L2), 0)
    ki = lax.broadcasted_iota(jnp.int32, (L2, L2), 1)
    q_mem, k_mem = qi >= 2 * SEG, ki >= 2 * SEG
    q_head = jnp.where(q_mem, (qi - 2 * SEG) // NMEM, qi // SEG)
    k_head = jnp.where(k_mem, (ki - 2 * SEG) // NMEM, ki // SEG)
    visible = q_mem | k_mem | (qi >= ki)
    fill_scr[...] = jnp.where(q_head == k_head, jnp.where(visible, 0.0, -1e9 * LOG2E), -jnp.inf).astype(f32)

    def ln_rows(r0, n, racc_row, lane_id):
        lane = lax.broadcasted_iota(jnp.int32, (n, 128), 1)
        wr = jnp.concatenate([wr_scr[0:8, :]] * (n // 8), axis=0)
        wr_sum = jnp.concatenate([wr_scr[8:16, 0:1]] * (n // 8), axis=0)
        x = x_scr[pl.ds(r0, n), :].astype(f32)
        mean = jnp.sum(x, axis=-1, keepdims=True) * (1.0 / DM)
        msq = jnp.sum(x * x, axis=-1, keepdims=True) * (1.0 / DM)
        xw = jnp.sum(x * wr, axis=-1, keepdims=True)
        var = jnp.maximum(msq - mean * mean, 0.0)
        inv = 1.0 / _rnd(jnp.sqrt(_rnd(_rnd(var) + EPS_BF16)))
        mean = _rnd(mean)
        xnb = ((x - mean) * inv).astype(bf16)
        xpn_scr[pl.ds(r0, n), :] = x + xnb.astype(f32)
        xnp = _as_u32(xnb)
        p0 = r0 // 2 if isinstance(r0, int) else pl.multiple_of(r0 // 2, 4)
        for k in range(KT):
            xn_pk[k, pl.ds(p0, n // 2), :] = xnp[:, 128 * k:128 * (k + 1)]
        r = _rnd((xw - mean * wr_sum) * inv)
        racc[racc_row:racc_row + n, :] = jnp.where(lane == lane_id, r, racc[racc_row:racc_row + n, :])

    def ln_first(c, carry):
        x_copy(pl.multiple_of(128 * c, 128), 128, SEM_X0 + c).wait()
        for i in range(8):
            ln_rows(pl.multiple_of(c * 128 + 16 * i, 16), 16, 16 * i, c)
        return carry
    lax.fori_loop(0, PRE // 128, ln_first, 0)

    def pro_pairs(t, gs):
        m, c8 = t // 4, t % 4
        sc = (SCALE if m == 0 else None) if isinstance(t, int) else jnp.where(m == 0, SCALE, 1.0).astype(f32)
        for g in gs:
            p0 = DM * (4 * t + g)
            both = pool[pl.ds(p0 if isinstance(t, int) else pl.multiple_of(p0, DM), DM), :]
            pair = (pltpu.bitcast(both << 16, f32).astype(bf16),
                    pltpu.bitcast(both & jnp.uint32(0xFFFF0000), f32).astype(bf16))
            for hh in range(2):
                wqkv[_head(g, c8, hh) * 3 + m] = _as_u32(pair[hh])
                lhs = jnp.concatenate([_as_bf16(xn_pk[k, 0:PRE // 2, :]) for k in range(KT)], axis=1)
                y = _dot(lhs, pair[hh])
                if sc is not None:
                    y = y * sc
                qrings[g][(2 * c8 + hh) * 3 + m, 0:PRE // 2, :] = _as_u32(y.astype(bf16))

    w_wait(0, 1, 0)
    pro_pairs(0, (0,))
    w_wait(1, 1, 1)
    pro_pairs(0, (1,))
    w_wait(2, 2, 2)
    pro_pairs(0, (2, 3))
    w_wait(4, 4, 3)
    x_copy(PRE, SEG, SEM_XC).wait()
    pro_pairs(1, range(NG))
    ln_rows(PRE, TOK, 128, 0)

    def pro_body(i, carry):
        w_wait(8 + 8 * i, 8, 4 + i)
        pro_pairs(2 + 2 * i, range(NG))
        pro_pairs(3 + 2 * i, range(NG))
        return carry
    lax.fori_loop(0, 5, pro_body, 0)
    wait_all(wo, SEM_WO)
    x_copy(PRE + SEG, S - PRE - SEG, SEM_XB).wait()
    col_tiles_start(wg32, lambda j: pool.at[pl.ds(G0 + 512 * j, 512)], SEM_FFN, FT)
    col_tiles_start(wu32, lambda j: pool.at[pl.ds(U0 + 512 * j, 512)], SEM_FFN, FT)
    col_tiles_start(wd32, lambda j: pool.at[pl.ds(D0 + FF // 2 * j, FF // 2)], SEM_FFN, KT)

    def step(s, mem_in, do_ln=True):
        xpos = pl.multiple_of((PRE + TOK * s) // 2, 4)
        wr_pos = [pl.multiple_of(lax.rem(PRE + TOK * s + 8 * i, RQ) // 2, 4) for i in range(3)]
        rd = pl.multiple_of(lax.rem(SEG * s, RQ) // 2, 16)
        owr = pl.multiple_of(lax.rem(SEG * s, RO) // 2, 16)
        orow = pl.multiple_of(TOK * s, 8)
        ord_ = pl.multiple_of(lax.rem(orow, RO) // 2, 4)

        def with_mem(tok_u32, mem_rows):
            tok = _as_bf16(tok_u32)
            last = jnp.concatenate([tok[16:TOK].astype(f32), mem_rows], axis=0).astype(bf16)
            return jnp.concatenate([tok[0:16], last], axis=0)

        zero = zero_scr[0:TOK // 2, :]
        lhs = jnp.concatenate(
            [with_mem(xn_pk[k, pl.ds(xpos, TOK // 2), :] ^ zero, mem_in[:, 128 * k:128 * (k + 1)])
             for k in range(KT)], axis=1)

        mem_parts, probs = {}, {}
        NS = 6
        first = [(c, m, hh) for c in range(4) for m in range(3) for hh in range(2)][:NS]
        lo = {key: _dot(lhs[:, :512], _as_bf16(wqkv[_head(0, key[0], key[2]) * 3 + key[1], 0:256, :])) for key in first}

        def qkv(g, c):
            res = {}
            for m in range(3):
                ms = []
                for hh in range(2):
                    if g == 0 and (c, m, hh) in lo:
                        y = _dot(lhs[:, 512:], _as_bf16(wqkv[_head(g, c, hh) * 3 + m, 256:512, :])) + lo[c, m, hh]
                    else:
                        y = _dot(lhs, _as_bf16(wqkv[_head(g, c, hh) * 3 + m]))
                    if m == 0:
                        y = y * SCALE
                    yp = _as_u32(y.astype(bf16))
                    for i in range(3):
                        qrings[g][(2 * c + hh) * 3 + m, pl.ds(wr_pos[i], 4), :] = yp[4 * i:4 * i + 4]
                    ms.append(y[TOK:])
                res[m] = jnp.concatenate(ms, axis=0).astype(bf16)
            mem_parts[g, c] = [res[m] for m in range(3)]

        def pair_rows(g, c, m, mem_rows):
            t0 = _as_bf16(qrings[g][(2 * c) * 3 + m, pl.ds(rd, SEG // 2), :])
            t1 = _as_bf16(qrings[g][(2 * c + 1) * 3 + m, pl.ds(rd, SEG // 2), :])
            return jnp.concatenate([t0, t1, mem_rows], axis=0)

        def scores(g, c):
            qm, km, vm = mem_parts.pop((g, c))
            sc = lax.dot_general(pair_rows(g, c, 0, qm), pair_rows(g, c, 1, km),
                                 (((1,), (1,)), ((), ())), preferred_element_type=f32)
            fill = fill_scr[...]
            sc = jnp.where(fill == 0.0, sc, fill)
            e = jnp.exp2(sc - jnp.max(sc, axis=-1, keepdims=True))
            r = pl.reciprocal(jnp.sum(e, axis=-1, keepdims=True), approx=True)
            probs[g, c] = (e.astype(bf16), r, vm)

        def pv(g, c):
            e, r, vm = probs.pop((g, c))
            o = _dot(e, pair_rows(g, c, 2, vm)) * r
            for hh in range(2):
                h = 2 * c + hh
                orings[g][h, pl.ds(owr, SEG // 2), :] = _as_u32(o[SEG * hh:SEG * (hh + 1)].astype(bf16))
                om = o[2 * SEG + NMEM * hh:2 * SEG + NMEM * (hh + 1)]
                lhs_os[g][h] = _as_u32(with_mem(orings[g][h, pl.ds(ord_, TOK // 2), :], om))

        acc = [None] * KT

        def out_proj(gs, js):
            for j in js:
                l = jnp.concatenate([_as_bf16(lhs_os[g][k]) for g in gs for k in range(8)], axis=1)
                w = jnp.concatenate(
                    [_as_bf16(wo[j, 64 * _head(g, c, 0):64 * _head(g, c, 0) + 128, :])
                     for g in gs for c in range(4)], axis=0)
                a = _dot(l, w)
                if acc[j] is None:
                    cs = slice(128 * j, 128 * (j + 1))
                    acc[j] = a + jnp.concatenate([xpn_scr[pl.ds(orow, TOK), cs], jnp.zeros((NMEM, 128), f32)], axis=0)
                else:
                    acc[j] = acc[j] + a

        for item in "q0 q1 s0 q2 p0 s1 q3 p1 s2 w01a p2 s3 w012b L0 p3 w2a w3".split():
            g = int(item[1])
            if item[0] == "L":
                if do_ln:
                    nxt = jnp.minimum(s + 1, NSEG - 1)
                    ln_rows(pl.multiple_of(PRE + TOK * nxt, 8), TOK, 128, nxt)
            elif item[0] == "w":
                if ":" in item:
                    gs, js = item[1:].split(":")
                    out_proj([int(ch) for ch in gs], [int(ch) for ch in js])
                    continue
                out_proj([int(ch) for ch in item[1:] if ch.isdigit()],
                         {"a": range(4), "b": range(4, 8)}.get(item[-1], range(8)))
            else:
                for c in range(4):
                    {"q": qkv, "s": scores, "p": pv}[item[0]](g, c)
        a = jnp.concatenate(acc, axis=1)
        out_stage[pl.ds(orow, TOK), :] = a[:TOK].astype(bf16)
        return _rnd(a[TOK:])

    UNR = 3
    PEEL = 1

    def body(u, carry):
        mem = mem_scr[...]
        for i in range(UNR):
            mem = step(UNR * u + i, mem)
        mem_scr[...] = mem
        out_copy(pl.multiple_of(TOK * UNR * u, 8), UNR * TOK, SEM_OUT).start()
        return carry
    lax.fori_loop(0, (NSEG - PEEL) // UNR, body, 0)

    wait_all(pool.at[pl.ds(0, FFN_ROWS)], SEM_FFN)

    mem = mem_scr[...]
    for s in range(NSEG - PEEL, NSEG):
        mem = step(jnp.int32(s), mem, do_ln=s < NSEG - 1)
    if PEEL:
        out_copy(TOK * (NSEG - PEEL), PEEL * TOK, SEM_OUT).start()

    rv = racc[...]
    rrow = lax.broadcasted_iota(jnp.int32, rv.shape, 0)
    rlane = lax.broadcasted_iota(jnp.int32, rv.shape, 1)
    ridx = jnp.where(rrow < 128, rrow + 128 * rlane, PRE + (rrow - 128) + TOK * rlane).astype(f32)
    m0 = jnp.max(rv, keepdims=True)
    f0 = jnp.min(jnp.where(rv == m0, ridx, 1e9), keepdims=True)
    rv2 = jnp.where(ridx == f0, -jnp.inf, rv)
    m1 = jnp.max(rv2, keepdims=True)
    f1 = jnp.min(jnp.where(rv2 == m1, ridx, 1e9), keepdims=True)
    i0 = jnp.clip(f0[0, 0].astype(jnp.int32), 0, S - 1)
    i1 = jnp.clip(f1[0, 0].astype(jnp.int32), 0, S - 1)
    row16 = lax.broadcasted_iota(jnp.int32, (16, DM), 0)

    def xn_row(i):
        w = jnp.concatenate([xn_pk[k, pl.ds(i // 2, 1), :] for k in range(KT)], axis=1)
        return pltpu.bitcast(jnp.where(i % 2 == 0, w << 16, w & jnp.uint32(0xFFFF0000)), f32)
    row8 = lax.broadcasted_iota(jnp.int32, (8, DM), 0)
    xsel = jnp.where(row8 == 0, xn_row(i0), jnp.where(row8 == 1, xn_row(i1), 0.0))

    e0 = NSEG * TOK
    e_rows = ((0, 128), (128, 128), (256, 128), (384, 96), (480, 32))
    last = S - 128
    part = {}

    def add(key, v):
        part[key] = v if key not in part else v + part[key]

    def e_round(b, j, r):
        r0, n = e_rows[b]
        l = jnp.concatenate(
            [_as_bf16(orings[(h % 8) // 2][2 * (h // 8) + h % 2, r0 // 2:(r0 + n) // 2, :])
             for h in range(4 * r, 4 * r + 4)], axis=1)
        add(("e", b, j), _dot(l, _as_bf16(wo[j, 256 * r:256 * (r + 1), :])))
        if r == 7:
            rows, cs = slice(e0 + r0, e0 + r0 + n), slice(128 * j, 128 * (j + 1))
            out_stage[rows, cs] = (part.pop(("e", b, j)) + xpn_scr[rows, cs]).astype(bf16)
            if j == KT - 1:
                out_copy(e0 + r0, n, SEM_OUT if b < 3 else SEM_OUT2).start()

    def up_round(w, name, j, r):
        wt = _as_bf16(pool[pl.ds(w + 512 * j + 256 * r, 256), :]).astype(f32)
        add((name, j), _dot(xsel[:, 512 * r:512 * (r + 1)], wt))
        if name == "u" and r == 1:
            gate = part.pop(("g", j))
            part["h", j] = _rnd(gate * jax.nn.sigmoid(gate) * part.pop(("u", j)))

    def down_round(j, r):
        hid = jnp.concatenate([part["h", k] for k in range(4 * r, 4 * r + 4)], axis=1)
        add(("y", j), _dot(hid, _as_bf16(pool[pl.ds(D0 + FF // 2 * j + 256 * r, 256), :]).astype(f32)))

    e_rounds = [(b, j, r) for b in range(5) for j in range(KT) for r in range(8)]
    m_rounds = [lambda j=j, r=r, w=w, n=n: up_round(w, n, j, r)
                for j in range(FT) for (w, n) in ((G0, "g"), (U0, "u")) for r in range(2)]
    m_rounds += [None] * 2
    m_rounds += [lambda j=j, r=r: down_round(j, r) for r in range(FT // 4) for j in range(KT)]
    m_rounds = [None] * 1 + m_rounds
    NM = 1
    for n, er in enumerate(e_rounds[:192]):
        e_round(*er)
        for mr in m_rounds[NM * n:NM * n + NM]:
            if mr is not None:
                mr()
    assert len(m_rounds) <= NM * 192
    rsel = jnp.where(lax.broadcasted_iota(jnp.int32, (8, 1), 0) == 0, m0, m1)
    y = jnp.concatenate([part.pop(("y", j)) for j in range(KT)], axis=1) * jax.nn.sigmoid(rsel)
    y0, y1 = y[0:1], y[1:2]
    xpn_scr[pl.ds(i0, 1), :] = xpn_scr[pl.ds(i0, 1), :] + jnp.where(i0 >= last, y0, 0.0)
    xpn_scr[pl.ds(i1, 1), :] = xpn_scr[pl.ds(i1, 1), :] + jnp.where(i1 >= last, y1, 0.0)
    for er in e_rounds[192:]:
        e_round(*er)

    out_copy(0, last, SEM_OUT).wait()
    g0 = pl.multiple_of((i0 // 16) * 16, 16)
    g1 = pl.multiple_of((i1 // 16) * 16, 16)
    redo0 = i0 < last
    redo1 = i1 < last
    send1 = jnp.logical_and(redo1, g1 != g0)

    def patch(i, gst, yy):
        blk = out_stage[pl.ds(gst, 16), :].astype(f32)
        out_stage[pl.ds(gst, 16), :] = (blk + jnp.where(row16 == i - gst, yy, 0.0)).astype(bf16)

    @pl.when(redo0)
    def _():
        patch(i0, g0, y0)

    @pl.when(redo1)
    def _():
        patch(i1, g1, y1)

    @pl.when(redo0)
    def _():
        out_copy(g0, 16, SEM_P0).start()

    @pl.when(send1)
    def _():
        out_copy(g1, 16, SEM_P1).start()

    out_copy(last, 128, SEM_OUT2).wait()

    @pl.when(redo0)
    def _():
        out_copy(g0, 16, SEM_P0).wait()

    @pl.when(send1)
    def _():
        out_copy(g1, 16, SEM_P1).wait()


@jax.jit
def pallas_parallel_sum__memory_aug_recurrent_mem_tr__moe_arch_mod__prompt_kernel(
    A_x: jax.Array,
    A_mem0: jax.Array,
    A_Wq: jax.Array,
    A_Wk: jax.Array,
    A_Wv: jax.Array,
    A_Wo: jax.Array,
    A_seg_len: jax.Array,
    B_x: jax.Array,
    B_w_r: jax.Array,
    B_w_gate: jax.Array,
    B_w_up: jax.Array,
    B_w_down: jax.Array,
):
    del A_seg_len, B_x
    assert A_x.shape == (1, S, DM) and A_mem0.shape == (1, NMEM, DM)
    assert A_Wq.shape == (DM, H, DH) and A_Wo.shape == (H, DH, DM) and B_w_gate.shape == (DM, FF)
    hbm = pl.BlockSpec(memory_space=pl.ANY)
    vmem = pl.BlockSpec(memory_space=pltpu.VMEM)
    scratch = [
        pltpu.VMEM((S, DM), bf16),
        pltpu.VMEM((S, DM), f32),
        pltpu.VMEM((KT, S // 2, 128), u32),
        pltpu.VMEM((16, DM), f32),
        pltpu.VMEM((48 * DM, 128), u32),
        pltpu.VMEM((3 * H, DM // 2, 128), u32),
        pltpu.VMEM((KT, H * DH // 2, 128), u32),
    ]
    scratch += [pltpu.VMEM((24, RQ // 2, 128), u32)] * NG
    scratch += [pltpu.VMEM((8, RO // 2, 128), u32)] * NG
    scratch += [pltpu.VMEM((8, 16, 128), u32)] * NG
    scratch += [
        pltpu.VMEM((NMEM, DM), f32),
        pltpu.VMEM((16, 128), u32),
        pltpu.VMEM((L2, L2), f32),
        pltpu.VMEM((128 + TOK, 128), f32),
        pltpu.VMEM((S, DM), bf16),
        pltpu.SemaphoreType.DMA((NSEM,)),
    ]
    return pl.pallas_call(
        _kernel,
        out_shape=jax.ShapeDtypeStruct((1, S, DM), bf16),
        in_specs=[hbm, vmem, hbm, hbm, hbm, hbm, vmem, hbm, hbm, hbm],
        out_specs=hbm,
        scratch_shapes=scratch,
        compiler_params=pltpu.CompilerParams(vmem_limit_bytes=110 * 1024 * 1024,
                                             disable_bounds_checks=True),
    )(A_x, A_mem0, A_Wq, A_Wk, A_Wv, A_Wo.reshape(H * DH, DM), B_w_r, B_w_gate, B_w_up, B_w_down)
```

```python
import jax
import jax.numpy as jnp
from jax import lax
import jax.experimental.pallas as pl
import jax.experimental.pallas.tpu as pltpu

bf16 = jnp.bfloat16
f32 = jnp.float32
u32 = jnp.uint32

S, DM, H, DH, NMEM, SEG, FF = 2048, 1024, 32, 128, 8, 32, 3584
NSEG = S // SEG
TOK = 24
PRE = S - NSEG * TOK
RQ = 544
RO = 768
UNR = 3
NG = 4
KT = DM // 128
FT = FF // 128
L2 = 2 * (SEG + NMEM)
LOG2E = 1.4426950408889634
SCALE = DH ** -0.5 * LOG2E
EPS_BF16 = 1.0013580322265625e-05

SEM_W0 = 0
SEM_X0 = 9
SEM_XB, SEM_XC, SEM_WO, SEM_FFN, SEM_OUT, SEM_P0, SEM_P1, SEM_OUT2 = range(13, 21)
NSEM = 21
G0, U0, D0 = 0, FT * DM // 2, 2 * FT * DM // 2
FFN_ROWS = D0 + KT * FF // 2


def _as_bf16(x):
    return pltpu.bitcast(x, bf16)


def _as_u32(x):
    return pltpu.bitcast(x, u32)


def _rnd(x):
    return x.astype(bf16).astype(f32)


def _dot(a, b):
    return jnp.dot(a, b, preferred_element_type=f32)


def _head(g, c, hh):
    return 8 * c + 2 * g + hh


def _kernel(x_hbm, mem0_ref, wq_hbm, wk_hbm, wv_hbm, wo_hbm, wr_ref, wg_hbm, wu_hbm, wd_hbm,
            out_hbm,
            x_scr, xpn_scr, xn_pk, wr_scr, pool, wqkv, wo,
            qr0, qr1, qr2, qr3, or0, or1, or2, or3, lo0, lo1, lo2, lo3,
            mem_scr, zero_scr, fill_scr, racc, out_stage, sems):
    qrings = (qr0, qr1, qr2, qr3)
    orings = (or0, or1, or2, or3)
    lhs_os = (lo0, lo1, lo2, lo3)
    w32 = [w.bitcast(u32) for w in (wq_hbm, wk_hbm, wv_hbm)]
    wo32 = wo_hbm.bitcast(u32)
    wg32 = wg_hbm.bitcast(u32)
    wu32 = wu_hbm.bitcast(u32)
    wd32 = wd_hbm.bitcast(u32)

    def x_copy(r0, n, sem):
        return pltpu.make_async_copy(x_hbm.at[0, pl.ds(r0, n)], x_scr.at[pl.ds(r0, n)], sems.at[sem])

    def out_copy(r0, n, sem):
        return pltpu.make_async_copy(out_stage.at[pl.ds(r0, n)], out_hbm.at[0, pl.ds(r0, n)], sems.at[sem])

    def w_start(lo, hi, sem):
        for p in range(lo, hi):
            pltpu.make_async_copy(w32[p // 16].at[:, p % 16, :], pool.at[pl.ds(DM * p, DM)],
                                  sems.at[SEM_W0 + sem]).start()

    def w_wait(lo, n, sem):
        r0 = DM * lo if isinstance(lo, int) else pl.multiple_of(DM * lo, DM)
        wait_all(pool.at[pl.ds(r0, DM * n)], SEM_W0 + sem)

    def col_tiles_start(src, dst_of, sem, n):
        for j in range(n):
            pltpu.make_async_copy(src.at[:, pl.ds(128 * j, 128)], dst_of(j), sems.at[sem]).start()

    def wait_all(buf, sem):
        pltpu.make_async_copy(buf, buf, sems.at[sem]).wait()

    for c in range(4):
        x_copy(128 * c, 128, SEM_X0 + c).start()
    w_start(0, 1, 0)
    w_start(1, 2, 1)
    w_start(2, 4, 2)
    w_start(4, 8, 3)
    x_copy(PRE, SEG, SEM_XC).start()
    for i in range(5):
        w_start(8 + 8 * i, 16 + 8 * i, 4 + i)
    x_copy(PRE + SEG, S - PRE - SEG, SEM_XB).start()
    col_tiles_start(wo32, lambda j: wo.at[j], SEM_WO, KT)

    mem_scr[...] = mem0_ref[0].astype(f32)
    zero_scr[...] = jnp.zeros(zero_scr.shape, u32)
    wr_row = wr_ref[...].astype(f32).reshape(1, DM)
    wr_scr[0:8, :] = jnp.broadcast_to(wr_row, (8, DM))
    wr_scr[8:16, :] = jnp.broadcast_to(jnp.sum(wr_row, axis=-1, keepdims=True), (8, DM))
    racc[...] = jnp.full(racc.shape, -jnp.inf, f32)
    qi = lax.broadcasted_iota(jnp.int32, (L2, L2), 0)
    ki = lax.broadcasted_iota(jnp.int32, (L2, L2), 1)
    q_mem, k_mem = qi >= 2 * SEG, ki >= 2 * SEG
    q_head = jnp.where(q_mem, (qi - 2 * SEG) // NMEM, qi // SEG)
    k_head = jnp.where(k_mem, (ki - 2 * SEG) // NMEM, ki // SEG)
    visible = q_mem | k_mem | (qi >= ki)
    fill_scr[...] = jnp.where(q_head == k_head, jnp.where(visible, 0.0, -1e9 * LOG2E), -jnp.inf).astype(f32)

    def ln_rows(r0, n, racc_row, lane_id):
        lane = lax.broadcasted_iota(jnp.int32, (n, 128), 1)
        wr = jnp.concatenate([wr_scr[0:8, :]] * (n // 8), axis=0)
        wr_sum = jnp.concatenate([wr_scr[8:16, 0:1]] * (n // 8), axis=0)
        x = x_scr[pl.ds(r0, n), :].astype(f32)
        mean = jnp.sum(x, axis=-1, keepdims=True) * (1.0 / DM)
        msq = jnp.sum(x * x, axis=-1, keepdims=True) * (1.0 / DM)
        xw = jnp.sum(x * wr, axis=-1, keepdims=True)
        var = jnp.maximum(msq - mean * mean, 0.0)
        inv = 1.0 / _rnd(jnp.sqrt(_rnd(_rnd(var) + EPS_BF16)))
        mean = _rnd(mean)
        xnb = ((x - mean) * inv).astype(bf16)
        xpn_scr[pl.ds(r0, n), :] = x + xnb.astype(f32)
        xnp = _as_u32(xnb)
        p0 = r0 // 2 if isinstance(r0, int) else pl.multiple_of(r0 // 2, 4)
        for k in range(KT):
            xn_pk[k, pl.ds(p0, n // 2), :] = xnp[:, 128 * k:128 * (k + 1)]
        r = _rnd((xw - mean * wr_sum) * inv)
        racc[racc_row:racc_row + n, :] = jnp.where(lane == lane_id, r, racc[racc_row:racc_row + n, :])

    def ln_first(c, carry):
        x_copy(pl.multiple_of(128 * c, 128), 128, SEM_X0 + c).wait()
        for i in range(8):
            ln_rows(pl.multiple_of(c * 128 + 16 * i, 16), 16, 16 * i, c)
        return carry
    lax.fori_loop(0, PRE // 128, ln_first, 0)

    def pro_pairs(t, gs):
        m, c8 = t // 4, t % 4
        sc = (SCALE if m == 0 else None) if isinstance(t, int) else jnp.where(m == 0, SCALE, 1.0).astype(f32)
        for g in gs:
            p0 = DM * (4 * t + g)
            both = pool[pl.ds(p0 if isinstance(t, int) else pl.multiple_of(p0, DM), DM), :]
            pair = (pltpu.bitcast(both << 16, f32).astype(bf16),
                    pltpu.bitcast(both & jnp.uint32(0xFFFF0000), f32).astype(bf16))
            for hh in range(2):
                wqkv[_head(g, c8, hh) * 3 + m] = _as_u32(pair[hh])
                lhs = jnp.concatenate([_as_bf16(xn_pk[k, 0:PRE // 2, :]) for k in range(KT)], axis=1)
                y = _dot(lhs, pair[hh])
                if sc is not None:
                    y = y * sc
                qrings[g][(2 * c8 + hh) * 3 + m, 0:PRE // 2, :] = _as_u32(y.astype(bf16))

    w_wait(0, 1, 0)
    pro_pairs(0, (0,))
    w_wait(1, 1, 1)
    pro_pairs(0, (1,))
    w_wait(2, 2, 2)
    pro_pairs(0, (2, 3))
    w_wait(4, 4, 3)
    x_copy(PRE, SEG, SEM_XC).wait()
    pro_pairs(1, range(NG))
    ln_rows(PRE, TOK, 128, 0)

    def pro_body(i, carry):
        w_wait(8 + 8 * i, 8, 4 + i)
        pro_pairs(2 + 2 * i, range(NG))
        pro_pairs(3 + 2 * i, range(NG))
        return carry
    lax.fori_loop(0, 5, pro_body, 0)
    wait_all(wo, SEM_WO)
    x_copy(PRE + SEG, S - PRE - SEG, SEM_XB).wait()
    col_tiles_start(wg32, lambda j: pool.at[pl.ds(G0 + 512 * j, 512)], SEM_FFN, FT)
    col_tiles_start(wu32, lambda j: pool.at[pl.ds(U0 + 512 * j, 512)], SEM_FFN, FT)
    col_tiles_start(wd32, lambda j: pool.at[pl.ds(D0 + FF // 2 * j, FF // 2)], SEM_FFN, KT)

    def step(s, mem_in, do_ln=True):
        xpos = pl.multiple_of((PRE + TOK * s) // 2, 4)
        wr_pos = [pl.multiple_of(lax.rem(PRE + TOK * s + 8 * i, RQ) // 2, 4) for i in range(3)]
        rd = pl.multiple_of(lax.rem(SEG * s, RQ) // 2, 16)
        owr = pl.multiple_of(lax.rem(SEG * s, RO) // 2, 16)
        orow = pl.multiple_of(TOK * s, 8)
        ord_ = pl.multiple_of(lax.rem(orow, RO) // 2, 4)

        def with_mem(tok_u32, mem_rows):
            tok = _as_bf16(tok_u32)
            last = jnp.concatenate([tok[16:TOK].astype(f32), mem_rows], axis=0).astype(bf16)
            return jnp.concatenate([tok[0:16], last], axis=0)

        zero = zero_scr[0:TOK // 2, :]
        lhs = jnp.concatenate(
            [with_mem(xn_pk[k, pl.ds(xpos, TOK // 2), :] ^ zero, mem_in[:, 128 * k:128 * (k + 1)])
             for k in range(KT)], axis=1)

        mem_parts, probs = {}, {}
        lo = {(0, m, hh): _dot(lhs[:, :512], _as_bf16(wqkv[_head(0, 0, hh) * 3 + m, 0:256, :]))
              for m in range(3) for hh in range(2)}

        def qkv(g, c):
            res = []
            for m in range(3):
                ms = []
                for hh in range(2):
                    if g == 0 and (c, m, hh) in lo:
                        y = _dot(lhs[:, 512:], _as_bf16(wqkv[_head(g, c, hh) * 3 + m, 256:512, :])) + lo[c, m, hh]
                    else:
                        y = _dot(lhs, _as_bf16(wqkv[_head(g, c, hh) * 3 + m]))
                    if m == 0:
                        y = y * SCALE
                    yp = _as_u32(y.astype(bf16))
                    for i in range(3):
                        qrings[g][(2 * c + hh) * 3 + m, pl.ds(wr_pos[i], 4), :] = yp[4 * i:4 * i + 4]
                    ms.append(y[TOK:])
                res.append(jnp.concatenate(ms, axis=0).astype(bf16))
            mem_parts[g, c] = res

        def pair_rows(g, c, m, mem_rows):
            t0 = _as_bf16(qrings[g][(2 * c) * 3 + m, pl.ds(rd, SEG // 2), :])
            t1 = _as_bf16(qrings[g][(2 * c + 1) * 3 + m, pl.ds(rd, SEG // 2), :])
            return jnp.concatenate([t0, t1, mem_rows], axis=0)

        def scores(g, c):
            qm, km, vm = mem_parts.pop((g, c))
            sc = lax.dot_general(pair_rows(g, c, 0, qm), pair_rows(g, c, 1, km),
                                 (((1,), (1,)), ((), ())), preferred_element_type=f32)
            fill = fill_scr[...]
            sc = jnp.where(fill == 0.0, sc, fill)
            e = jnp.exp2(sc - jnp.max(sc, axis=-1, keepdims=True))
            r = pl.reciprocal(jnp.sum(e, axis=-1, keepdims=True), approx=True)
            probs[g, c] = (e.astype(bf16), r, vm)

        def pv(g, c):
            e, r, vm = probs.pop((g, c))
            o = _dot(e, pair_rows(g, c, 2, vm)) * r
            for hh in range(2):
                h = 2 * c + hh
                orings[g][h, pl.ds(owr, SEG // 2), :] = _as_u32(o[SEG * hh:SEG * (hh + 1)].astype(bf16))
                om = o[2 * SEG + NMEM * hh:2 * SEG + NMEM * (hh + 1)]
                lhs_os[g][h] = _as_u32(with_mem(orings[g][h, pl.ds(ord_, TOK // 2), :], om))

        acc = [None] * KT

        def out_proj(gs, js):
            for j in js:
                l = jnp.concatenate([_as_bf16(lhs_os[g][k]) for g in gs for k in range(8)], axis=1)
                w = jnp.concatenate(
                    [_as_bf16(wo[j, 64 * _head(g, c, 0):64 * _head(g, c, 0) + 128, :])
                     for g in gs for c in range(4)], axis=0)
                a = _dot(l, w)
                if acc[j] is None:
                    cs = slice(128 * j, 128 * (j + 1))
                    acc[j] = a + jnp.concatenate([xpn_scr[pl.ds(orow, TOK), cs], jnp.zeros((NMEM, 128), f32)], axis=0)
                else:
                    acc[j] = acc[j] + a

        def group(fn, g):
            for c in range(4):
                fn(g, c)

        group(qkv, 0)
        group(qkv, 1)
        group(scores, 0)
        group(qkv, 2)
        group(pv, 0)
        group(scores, 1)
        group(qkv, 3)
        group(pv, 1)
        group(scores, 2)
        out_proj((0, 1), range(4))
        group(pv, 2)
        group(scores, 3)
        out_proj((0, 1, 2), range(4, 8))
        if do_ln:
            nxt = jnp.minimum(s + 1, NSEG - 1)
            ln_rows(pl.multiple_of(PRE + TOK * nxt, 8), TOK, 128, nxt)
        group(pv, 3)
        out_proj((2,), range(4))
        out_proj((3,), range(8))
        a = jnp.concatenate(acc, axis=1)
        out_stage[pl.ds(orow, TOK), :] = a[:TOK].astype(bf16)
        return _rnd(a[TOK:])

    def body(u, carry):
        mem = mem_scr[...]
        for i in range(UNR):
            mem = step(UNR * u + i, mem)
        mem_scr[...] = mem
        out_copy(pl.multiple_of(TOK * UNR * u, 8), UNR * TOK, SEM_OUT).start()
        return carry
    lax.fori_loop(0, (NSEG - 1) // UNR, body, 0)

    wait_all(pool.at[pl.ds(0, FFN_ROWS)], SEM_FFN)

    step(jnp.int32(NSEG - 1), mem_scr[...], do_ln=False)
    out_copy(TOK * (NSEG - 1), TOK, SEM_OUT).start()

    rv = racc[...]
    rrow = lax.broadcasted_iota(jnp.int32, rv.shape, 0)
    rlane = lax.broadcasted_iota(jnp.int32, rv.shape, 1)
    ridx = jnp.where(rrow < 128, rrow + 128 * rlane, PRE + (rrow - 128) + TOK * rlane).astype(f32)
    m0 = jnp.max(rv, keepdims=True)
    f0 = jnp.min(jnp.where(rv == m0, ridx, 1e9), keepdims=True)
    rv2 = jnp.where(ridx == f0, -jnp.inf, rv)
    m1 = jnp.max(rv2, keepdims=True)
    f1 = jnp.min(jnp.where(rv2 == m1, ridx, 1e9), keepdims=True)
    i0 = jnp.clip(f0[0, 0].astype(jnp.int32), 0, S - 1)
    i1 = jnp.clip(f1[0, 0].astype(jnp.int32), 0, S - 1)
    row16 = lax.broadcasted_iota(jnp.int32, (16, DM), 0)

    def xn_row(i):
        w = jnp.concatenate([xn_pk[k, pl.ds(i // 2, 1), :] for k in range(KT)], axis=1)
        return pltpu.bitcast(jnp.where(i % 2 == 0, w << 16, w & jnp.uint32(0xFFFF0000)), f32)
    row8 = lax.broadcasted_iota(jnp.int32, (8, DM), 0)
    xsel = jnp.where(row8 == 0, xn_row(i0), jnp.where(row8 == 1, xn_row(i1), 0.0))

    e0 = NSEG * TOK
    e_rows = ((0, 128), (128, 128), (256, 128), (384, 96), (480, 32))
    last = S - 128
    part = {}

    def add(key, v):
        part[key] = v if key not in part else v + part[key]

    def e_round(b, j, r):
        r0, n = e_rows[b]
        l = jnp.concatenate(
            [_as_bf16(orings[(h % 8) // 2][2 * (h // 8) + h % 2, r0 // 2:(r0 + n) // 2, :])
             for h in range(4 * r, 4 * r + 4)], axis=1)
        add(("e", b, j), _dot(l, _as_bf16(wo[j, 256 * r:256 * (r + 1), :])))
        if r == 7:
            rows, cs = slice(e0 + r0, e0 + r0 + n), slice(128 * j, 128 * (j + 1))
            out_stage[rows, cs] = (part.pop(("e", b, j)) + xpn_scr[rows, cs]).astype(bf16)
            if j == KT - 1:
                out_copy(e0 + r0, n, SEM_OUT if b < 3 else SEM_OUT2).start()

    def up_round(w, name, j, r):
        wt = _as_bf16(pool[pl.ds(w + 512 * j + 256 * r, 256), :]).astype(f32)
        add((name, j), _dot(xsel[:, 512 * r:512 * (r + 1)], wt))
        if name == "u" and r == 1:
            gate = part.pop(("g", j))
            part["h", j] = _rnd(gate * jax.nn.sigmoid(gate) * part.pop(("u", j)))

    def down_round(j, r):
        hid = jnp.concatenate([part["h", k] for k in range(4 * r, 4 * r + 4)], axis=1)
        add(("y", j), _dot(hid, _as_bf16(pool[pl.ds(D0 + FF // 2 * j + 256 * r, 256), :]).astype(f32)))

    e_rounds = [(b, j, r) for b in range(5) for j in range(KT) for r in range(8)]
    m_rounds = [lambda j=j, r=r, w=w, n=n: up_round(w, n, j, r)
                for j in range(FT) for (w, n) in ((G0, "g"), (U0, "u")) for r in range(2)]
    m_rounds += [None] * 2
    m_rounds += [lambda j=j, r=r: down_round(j, r) for r in range(FT // 4) for j in range(KT)]
    m_rounds = [None] + m_rounds
    assert len(m_rounds) <= 192
    for n, er in enumerate(e_rounds[:192]):
        e_round(*er)
        if n < len(m_rounds) and m_rounds[n] is not None:
            m_rounds[n]()
    rsel = jnp.where(lax.broadcasted_iota(jnp.int32, (8, 1), 0) == 0, m0, m1)
    y = jnp.concatenate([part.pop(("y", j)) for j in range(KT)], axis=1) * jax.nn.sigmoid(rsel)
    y0, y1 = y[0:1], y[1:2]
    xpn_scr[pl.ds(i0, 1), :] = xpn_scr[pl.ds(i0, 1), :] + jnp.where(i0 >= last, y0, 0.0)
    xpn_scr[pl.ds(i1, 1), :] = xpn_scr[pl.ds(i1, 1), :] + jnp.where(i1 >= last, y1, 0.0)
    for er in e_rounds[192:]:
        e_round(*er)

    out_copy(0, last, SEM_OUT).wait()
    g0 = pl.multiple_of((i0 // 16) * 16, 16)
    g1 = pl.multiple_of((i1 // 16) * 16, 16)
    redo0 = i0 < last
    redo1 = i1 < last
    send1 = jnp.logical_and(redo1, g1 != g0)

    def patch(i, gst, yy):
        blk = out_stage[pl.ds(gst, 16), :].astype(f32)
        out_stage[pl.ds(gst, 16), :] = (blk + jnp.where(row16 == i - gst, yy, 0.0)).astype(bf16)

    @pl.when(redo0)
    def _():
        patch(i0, g0, y0)

    @pl.when(redo1)
    def _():
        patch(i1, g1, y1)

    @pl.when(redo0)
    def _():
        out_copy(g0, 16, SEM_P0).start()

    @pl.when(send1)
    def _():
        out_copy(g1, 16, SEM_P1).start()

    out_copy(last, 128, SEM_OUT2).wait()

    @pl.when(redo0)
    def _():
        out_copy(g0, 16, SEM_P0).wait()

    @pl.when(send1)
    def _():
        out_copy(g1, 16, SEM_P1).wait()


@jax.jit
def pallas_parallel_sum__memory_aug_recurrent_mem_tr__moe_arch_mod__prompt_kernel(
    A_x: jax.Array,
    A_mem0: jax.Array,
    A_Wq: jax.Array,
    A_Wk: jax.Array,
    A_Wv: jax.Array,
    A_Wo: jax.Array,
    A_seg_len: jax.Array,
    B_x: jax.Array,
    B_w_r: jax.Array,
    B_w_gate: jax.Array,
    B_w_up: jax.Array,
    B_w_down: jax.Array,
):
    del A_seg_len, B_x
    assert A_x.shape == (1, S, DM) and A_mem0.shape == (1, NMEM, DM)
    assert A_Wq.shape == (DM, H, DH) and A_Wo.shape == (H, DH, DM) and B_w_gate.shape == (DM, FF)
    hbm = pl.BlockSpec(memory_space=pl.ANY)
    vmem = pl.BlockSpec(memory_space=pltpu.VMEM)
    scratch = [
        pltpu.VMEM((S, DM), bf16),
        pltpu.VMEM((S, DM), f32),
        pltpu.VMEM((KT, S // 2, 128), u32),
        pltpu.VMEM((16, DM), f32),
        pltpu.VMEM((48 * DM, 128), u32),
        pltpu.VMEM((3 * H, DM // 2, 128), u32),
        pltpu.VMEM((KT, H * DH // 2, 128), u32),
    ]
    scratch += [pltpu.VMEM((24, RQ // 2, 128), u32)] * NG
    scratch += [pltpu.VMEM((8, RO // 2, 128), u32)] * NG
    scratch += [pltpu.VMEM((8, 16, 128), u32)] * NG
    scratch += [
        pltpu.VMEM((NMEM, DM), f32),
        pltpu.VMEM((16, 128), u32),
        pltpu.VMEM((L2, L2), f32),
        pltpu.VMEM((128 + TOK, 128), f32),
        pltpu.VMEM((S, DM), bf16),
        pltpu.SemaphoreType.DMA((NSEM,)),
    ]
    return pl.pallas_call(
        _kernel,
        out_shape=jax.ShapeDtypeStruct((1, S, DM), bf16),
        in_specs=[hbm, vmem, hbm, hbm, hbm, hbm, vmem, hbm, hbm, hbm],
        out_specs=hbm,
        scratch_shapes=scratch,
        compiler_params=pltpu.CompilerParams(vmem_limit_bytes=110 * 1024 * 1024,
                                             disable_bounds_checks=True),
    )(A_x, A_mem0, A_Wq, A_Wk, A_Wv, A_Wo.reshape(H * DH, DM), B_w_r, B_w_gate, B_w_up, B_w_down)
```

```python
import jax
import jax.numpy as jnp
from jax import lax
import jax.experimental.pallas as pl
import jax.experimental.pallas.tpu as pltpu

bf16 = jnp.bfloat16
f32 = jnp.float32
u32 = jnp.uint32

S, DM, H, DH, NMEM, SEG, FF = 2048, 1024, 32, 128, 8, 32, 3584
NSEG = S // SEG
TOK = 24
PRE = S - NSEG * TOK
RQ = 544
RO = 768
UNR = 3
NG = 4
KT = DM // 128
FT = FF // 128
L2 = 2 * (SEG + NMEM)
LOG2E = 1.4426950408889634
SCALE = DH ** -0.5 * LOG2E
EPS_BF16 = 1.0013580322265625e-05

SEM_W0 = 0
SEM_X0 = 9
SEM_XB, SEM_XC, SEM_WO, SEM_FFN, SEM_OUT, SEM_P0, SEM_P1, SEM_OUT2 = range(13, 21)
NSEM = 21
G0, U0, D0 = 0, FT * DM // 2, 2 * FT * DM // 2
FFN_ROWS = D0 + KT * FF // 2


def _as_bf16(x):
    return pltpu.bitcast(x, bf16)


def _as_u32(x):
    return pltpu.bitcast(x, u32)


def _rnd(x):
    return x.astype(bf16).astype(f32)


def _dot(a, b):
    return jnp.dot(a, b, preferred_element_type=f32)


def _head(g, c, hh):
    return 8 * c + 2 * g + hh


def _kernel(x_hbm, mem0_ref, wq_hbm, wk_hbm, wv_hbm, wo_hbm, wr_ref, wg_hbm, wu_hbm, wd_hbm,
            out_hbm,
            x_scr, xpn_scr, xn_pk, wr_scr, pool, wqkv, wo,
            qr0, qr1, qr2, qr3, or0, or1, or2, or3, lo0, lo1, lo2, lo3,
            mem_scr, zero_scr, fill_scr, racc, out_stage, sems):
    qrings = (qr0, qr1, qr2, qr3)
    orings = (or0, or1, or2, or3)
    lhs_os = (lo0, lo1, lo2, lo3)
    w32 = [w.bitcast(u32) for w in (wq_hbm, wk_hbm, wv_hbm)]
    wo32 = wo_hbm.bitcast(u32)
    wg32 = wg_hbm.bitcast(u32)
    wu32 = wu_hbm.bitcast(u32)
    wd32 = wd_hbm.bitcast(u32)

    def x_copy(r0, n, sem):
        return pltpu.make_async_copy(x_hbm.at[0, pl.ds(r0, n)], x_scr.at[pl.ds(r0, n)], sems.at[sem])

    def out_copy(r0, n, sem):
        return pltpu.make_async_copy(out_stage.at[pl.ds(r0, n)], out_hbm.at[0, pl.ds(r0, n)], sems.at[sem])

    def w_start(lo, hi, sem):
        for p in range(lo, hi):
            pltpu.make_async_copy(w32[p // 16].at[:, p % 16, :], pool.at[pl.ds(DM * p, DM)],
                                  sems.at[SEM_W0 + sem]).start()

    def w_wait(lo, n, sem):
        r0 = DM * lo if isinstance(lo, int) else pl.multiple_of(DM * lo, DM)
        wait_all(pool.at[pl.ds(r0, DM * n)], SEM_W0 + sem)

    def col_tiles_start(src, dst_of, sem, n):
        for j in range(n):
            pltpu.make_async_copy(src.at[:, pl.ds(128 * j, 128)], dst_of(j), sems.at[sem]).start()

    def wait_all(buf, sem):
        pltpu.make_async_copy(buf, buf, sems.at[sem]).wait()

    for c in range(4):
        x_copy(128 * c, 128, SEM_X0 + c).start()
    w_start(0, 1, 0)
    w_start(1, 2, 1)
    w_start(2, 4, 2)
    w_start(4, 8, 3)
    x_copy(PRE, SEG, SEM_XC).start()
    for i in range(5):
        w_start(8 + 8 * i, 16 + 8 * i, 4 + i)
    x_copy(PRE + SEG, S - PRE - SEG, SEM_XB).start()
    col_tiles_start(wo32, lambda j: wo.at[j], SEM_WO, KT)

    mem_scr[...] = mem0_ref[0].astype(f32)
    zero_scr[...] = jnp.zeros(zero_scr.shape, u32)
    wr_row = wr_ref[...].astype(f32).reshape(1, DM)
    wr_scr[0:8, :] = jnp.broadcast_to(wr_row, (8, DM))
    wr_scr[8:16, :] = jnp.broadcast_to(jnp.sum(wr_row, axis=-1, keepdims=True), (8, DM))
    racc[...] = jnp.full(racc.shape, -jnp.inf, f32)
    qi = lax.broadcasted_iota(jnp.int32, (L2, L2), 0)
    ki = lax.broadcasted_iota(jnp.int32, (L2, L2), 1)
    q_mem, k_mem = qi >= 2 * SEG, ki >= 2 * SEG
    q_head = jnp.where(q_mem, (qi - 2 * SEG) // NMEM, qi // SEG)
    k_head = jnp.where(k_mem, (ki - 2 * SEG) // NMEM, ki // SEG)
    visible = q_mem | k_mem | (qi >= ki)
    fill_scr[...] = jnp.where(q_head == k_head, jnp.where(visible, 0.0, -1e9 * LOG2E), -jnp.inf).astype(f32)

    def ln_rows(r0, n, racc_row, lane_id):
        lane = lax.broadcasted_iota(jnp.int32, (n, 128), 1)
        wr = jnp.concatenate([wr_scr[0:8, :]] * (n // 8), axis=0)
        wr_sum = jnp.concatenate([wr_scr[8:16, 0:1]] * (n // 8), axis=0)
        x = x_scr[pl.ds(r0, n), :].astype(f32)
        mean = jnp.sum(x, axis=-1, keepdims=True) * (1.0 / DM)
        msq = jnp.sum(x * x, axis=-1, keepdims=True) * (1.0 / DM)
        xw = jnp.sum(x * wr, axis=-1, keepdims=True)
        var = jnp.maximum(msq - mean * mean, 0.0)
        inv = 1.0 / _rnd(jnp.sqrt(_rnd(_rnd(var) + EPS_BF16)))
        mean = _rnd(mean)
        xnb = ((x - mean) * inv).astype(bf16)
        xpn_scr[pl.ds(r0, n), :] = x + xnb.astype(f32)
        xnp = _as_u32(xnb)
        p0 = r0 // 2 if isinstance(r0, int) else pl.multiple_of(r0 // 2, 4)
        for k in range(KT):
            xn_pk[k, pl.ds(p0, n // 2), :] = xnp[:, 128 * k:128 * (k + 1)]
        r = _rnd((xw - mean * wr_sum) * inv)
        racc[racc_row:racc_row + n, :] = jnp.where(lane == lane_id, r, racc[racc_row:racc_row + n, :])

    def ln_first(c, carry):
        x_copy(pl.multiple_of(128 * c, 128), 128, SEM_X0 + c).wait()
        for i in range(8):
            ln_rows(pl.multiple_of(c * 128 + 16 * i, 16), 16, 16 * i, c)
        return carry
    lax.fori_loop(0, PRE // 128, ln_first, 0)

    def pro_pairs(t, gs):
        m, c8 = t // 4, t % 4
        sc = (SCALE if m == 0 else None) if isinstance(t, int) else jnp.where(m == 0, SCALE, 1.0).astype(f32)
        for g in gs:
            p0 = DM * (4 * t + g)
            both = pool[pl.ds(p0 if isinstance(t, int) else pl.multiple_of(p0, DM), DM), :]
            pair = (pltpu.bitcast(both << 16, f32).astype(bf16),
                    pltpu.bitcast(both & jnp.uint32(0xFFFF0000), f32).astype(bf16))
            for hh in range(2):
                wqkv[_head(g, c8, hh) * 3 + m] = _as_u32(pair[hh])
                lhs = jnp.concatenate([_as_bf16(xn_pk[k, 0:PRE // 2, :]) for k in range(KT)], axis=1)
                y = _dot(lhs, pair[hh])
                if sc is not None:
                    y = y * sc
                qrings[g][(2 * c8 + hh) * 3 + m, 0:PRE // 2, :] = _as_u32(y.astype(bf16))

    w_wait(0, 1, 0)
    pro_pairs(0, (0,))
    w_wait(1, 1, 1)
    pro_pairs(0, (1,))
    w_wait(2, 2, 2)
    pro_pairs(0, (2, 3))
    w_wait(4, 4, 3)
    x_copy(PRE, SEG, SEM_XC).wait()
    pro_pairs(1, range(NG))
    ln_rows(PRE, TOK, 128, 0)

    def pro_body(i, carry):
        w_wait(8 + 8 * i, 8, 4 + i)
        pro_pairs(2 + 2 * i, range(NG))
        pro_pairs(3 + 2 * i, range(NG))
        return carry
    lax.fori_loop(0, 5, pro_body, 0)
    wait_all(wo, SEM_WO)
    x_copy(PRE + SEG, S - PRE - SEG, SEM_XB).wait()
    col_tiles_start(wg32, lambda j: pool.at[pl.ds(G0 + 512 * j, 512)], SEM_FFN, FT)
    col_tiles_start(wu32, lambda j: pool.at[pl.ds(U0 + 512 * j, 512)], SEM_FFN, FT)
    col_tiles_start(wd32, lambda j: pool.at[pl.ds(D0 + FF // 2 * j, FF // 2)], SEM_FFN, KT)

    def step(s, mem_in):
        final = isinstance(s, int)
        nq = 2 * SEG if final else L2

        def packed(row, ring, mult):
            return (row % ring) // 2 if final else pl.multiple_of(lax.rem(row, ring) // 2, mult)

        xpos = (PRE + TOK * s) // 2 if final else pl.multiple_of((PRE + TOK * s) // 2, 4)
        orow = TOK * s if final else pl.multiple_of(TOK * s, 8)
        wr_pos = [packed(PRE + TOK * s + 8 * i, RQ, 4) for i in range(3)]
        rd = packed(SEG * s, RQ, 16)
        owr = packed(SEG * s, RO, 16)
        ord_ = packed(orow, RO, 4)

        def with_mem(tok_u32, mem_rows):
            tok = _as_bf16(tok_u32)
            last = jnp.concatenate([tok[16:TOK].astype(f32), mem_rows], axis=0).astype(bf16)
            return jnp.concatenate([tok[0:16], last], axis=0)

        zero = zero_scr[0:TOK // 2, :]
        lhs = jnp.concatenate(
            [with_mem(xn_pk[k, pl.ds(xpos, TOK // 2), :] ^ zero, mem_in[:, 128 * k:128 * (k + 1)])
             for k in range(KT)], axis=1)

        mem_parts, probs = {}, {}
        lo = {(0, m, hh): _dot(lhs[:, :512], _as_bf16(wqkv[_head(0, 0, hh) * 3 + m, 0:256, :]))
              for m in range(3) for hh in range(2)}

        def qkv(g, c):
            res = []
            for m in range(3):
                ms = []
                for hh in range(2):
                    if g == 0 and (c, m, hh) in lo:
                        y = _dot(lhs[:, 512:], _as_bf16(wqkv[_head(g, c, hh) * 3 + m, 256:512, :])) + lo[c, m, hh]
                    else:
                        y = _dot(lhs, _as_bf16(wqkv[_head(g, c, hh) * 3 + m]))
                    if m == 0:
                        y = y * SCALE
                    yp = _as_u32(y.astype(bf16))
                    for i in range(3):
                        qrings[g][(2 * c + hh) * 3 + m, pl.ds(wr_pos[i], 4), :] = yp[4 * i:4 * i + 4]
                    ms.append(y[TOK:])
                res.append(jnp.concatenate(ms, axis=0).astype(bf16))
            mem_parts[g, c] = res

        def pair_rows(g, c, m, mem_rows):
            t0 = _as_bf16(qrings[g][(2 * c) * 3 + m, pl.ds(rd, SEG // 2), :])
            t1 = _as_bf16(qrings[g][(2 * c + 1) * 3 + m, pl.ds(rd, SEG // 2), :])
            return jnp.concatenate([t0, t1, mem_rows], axis=0)

        def scores(g, c):
            qm, km, vm = mem_parts.pop((g, c))
            sc = lax.dot_general(pair_rows(g, c, 0, qm)[0:nq], pair_rows(g, c, 1, km),
                                 (((1,), (1,)), ((), ())), preferred_element_type=f32)
            fill = fill_scr[0:nq, :]
            sc = jnp.where(fill == 0.0, sc, fill)
            e = jnp.exp2(sc - jnp.max(sc, axis=-1, keepdims=True))
            r = pl.reciprocal(jnp.sum(e, axis=-1, keepdims=True), approx=True)
            probs[g, c] = (e.astype(bf16), r, vm)

        def pv(g, c):
            e, r, vm = probs.pop((g, c))
            o = _dot(e, pair_rows(g, c, 2, vm)) * r
            for hh in range(2):
                h = 2 * c + hh
                orings[g][h, pl.ds(owr, SEG // 2), :] = _as_u32(o[SEG * hh:SEG * (hh + 1)].astype(bf16))
                om = jnp.zeros((NMEM, 128), f32) if final else o[2 * SEG + NMEM * hh:2 * SEG + NMEM * (hh + 1)]
                lhs_os[g][h] = _as_u32(with_mem(orings[g][h, pl.ds(ord_, TOK // 2), :], om))

        acc = [None] * KT

        def out_proj(gs, js):
            for j in js:
                l = jnp.concatenate([_as_bf16(lhs_os[g][k]) for g in gs for k in range(8)], axis=1)
                w = jnp.concatenate(
                    [_as_bf16(wo[j, 64 * _head(g, c, 0):64 * _head(g, c, 0) + 128, :])
                     for g in gs for c in range(4)], axis=0)
                a = _dot(l, w)
                if acc[j] is None:
                    cs = slice(128 * j, 128 * (j + 1))
                    acc[j] = a + jnp.concatenate([xpn_scr[pl.ds(orow, TOK), cs], jnp.zeros((NMEM, 128), f32)], axis=0)
                else:
                    acc[j] = acc[j] + a

        def group(fn, g):
            for c in range(4):
                fn(g, c)

        group(qkv, 0)
        group(qkv, 1)
        group(scores, 0)
        group(qkv, 2)
        group(pv, 0)
        group(scores, 1)
        group(qkv, 3)
        group(pv, 1)
        group(scores, 2)
        out_proj((0, 1), range(4))
        group(pv, 2)
        group(scores, 3)
        out_proj((0, 1, 2), range(4, 8))
        if not final:
            ln_rows(pl.multiple_of(PRE + TOK * (s + 1), 8), TOK, 128, s + 1)
        group(pv, 3)
        out_proj((2,), range(4))
        out_proj((3,), range(8))
        a = jnp.concatenate(acc, axis=1)
        out_stage[pl.ds(orow, TOK), :] = a[:TOK].astype(bf16)
        return _rnd(a[TOK:])

    def body(u, carry):
        mem = mem_scr[...]
        for i in range(UNR):
            mem = step(UNR * u + i, mem)
        mem_scr[...] = mem
        out_copy(pl.multiple_of(TOK * UNR * u, 8), UNR * TOK, SEM_OUT).start()
        return carry
    lax.fori_loop(0, (NSEG - 1) // UNR, body, 0)

    wait_all(pool.at[pl.ds(0, FFN_ROWS)], SEM_FFN)

    step(NSEG - 1, mem_scr[...])
    out_copy(TOK * (NSEG - 1), TOK, SEM_OUT).start()

    rv = racc[...]
    rrow = lax.broadcasted_iota(jnp.int32, rv.shape, 0)
    rlane = lax.broadcasted_iota(jnp.int32, rv.shape, 1)
    ridx = jnp.where(rrow < 128, rrow + 128 * rlane, PRE + (rrow - 128) + TOK * rlane).astype(f32)
    m0 = jnp.max(rv, keepdims=True)
    f0 = jnp.min(jnp.where(rv == m0, ridx, 1e9), keepdims=True)
    rv2 = jnp.where(ridx == f0, -jnp.inf, rv)
    m1 = jnp.max(rv2, keepdims=True)
    f1 = jnp.min(jnp.where(rv2 == m1, ridx, 1e9), keepdims=True)
    i0 = jnp.clip(f0[0, 0].astype(jnp.int32), 0, S - 1)
    i1 = jnp.clip(f1[0, 0].astype(jnp.int32), 0, S - 1)
    row16 = lax.broadcasted_iota(jnp.int32, (16, DM), 0)

    def xn_row(i):
        w = jnp.concatenate([xn_pk[k, pl.ds(i // 2, 1), :] for k in range(KT)], axis=1)
        return pltpu.bitcast(jnp.where(i % 2 == 0, w << 16, w & jnp.uint32(0xFFFF0000)), f32)
    row8 = lax.broadcasted_iota(jnp.int32, (8, DM), 0)
    xsel = jnp.where(row8 == 0, xn_row(i0), jnp.where(row8 == 1, xn_row(i1), 0.0))

    e0 = NSEG * TOK
    e_rows = ((0, 128), (128, 128), (256, 128), (384, 96), (480, 32))
    last = S - 128
    part = {}

    def add(key, v):
        part[key] = v if key not in part else v + part[key]

    def e_round(b, j, r):
        r0, n = e_rows[b]
        l = jnp.concatenate(
            [_as_bf16(orings[(h % 8) // 2][2 * (h // 8) + h % 2, r0 // 2:(r0 + n) // 2, :])
             for h in range(4 * r, 4 * r + 4)], axis=1)
        add(("e", b, j), _dot(l, _as_bf16(wo[j, 256 * r:256 * (r + 1), :])))
        if r == 7:
            rows, cs = slice(e0 + r0, e0 + r0 + n), slice(128 * j, 128 * (j + 1))
            out_stage[rows, cs] = (part.pop(("e", b, j)) + xpn_scr[rows, cs]).astype(bf16)
            if j == KT - 1:
                out_copy(e0 + r0, n, SEM_OUT if b < 3 else SEM_OUT2).start()

    def up_round(w, name, j, r):
        wt = _as_bf16(pool[pl.ds(w + 512 * j + 256 * r, 256), :]).astype(f32)
        add((name, j), _dot(xsel[:, 512 * r:512 * (r + 1)], wt))
        if name == "u" and r == 1:
            gate = part.pop(("g", j))
            part["h", j] = _rnd(gate * jax.nn.sigmoid(gate) * part.pop(("u", j)))

    def down_round(j, r):
        hid = jnp.concatenate([part["h", k] for k in range(4 * r, 4 * r + 4)], axis=1)
        add(("y", j), _dot(hid, _as_bf16(pool[pl.ds(D0 + FF // 2 * j + 256 * r, 256), :]).astype(f32)))

    e_rounds = [(b, j, r) for b in range(5) for j in range(KT) for r in range(8)]
    m_rounds = [lambda j=j, r=r, w=w, n=n: up_round(w, n, j, r)
                for j in range(FT) for (w, n) in ((G0, "g"), (U0, "u")) for r in range(2)]
    m_rounds += [None] * 2
    m_rounds += [lambda j=j, r=r: down_round(j, r) for r in range(FT // 4) for j in range(KT)]
    m_rounds = [None] + m_rounds
    assert len(m_rounds) <= 192
    for n, er in enumerate(e_rounds[:192]):
        e_round(*er)
        if n < len(m_rounds) and m_rounds[n] is not None:
            m_rounds[n]()
    rsel = jnp.where(lax.broadcasted_iota(jnp.int32, (8, 1), 0) == 0, m0, m1)
    y = jnp.concatenate([part.pop(("y", j)) for j in range(KT)], axis=1) * jax.nn.sigmoid(rsel)
    y0, y1 = y[0:1], y[1:2]
    xpn_scr[pl.ds(i0, 1), :] = xpn_scr[pl.ds(i0, 1), :] + jnp.where(i0 >= last, y0, 0.0)
    xpn_scr[pl.ds(i1, 1), :] = xpn_scr[pl.ds(i1, 1), :] + jnp.where(i1 >= last, y1, 0.0)
    for er in e_rounds[192:]:
        e_round(*er)

    out_copy(0, last, SEM_OUT).wait()
    g0 = pl.multiple_of((i0 // 16) * 16, 16)
    g1 = pl.multiple_of((i1 // 16) * 16, 16)
    redo0 = i0 < last
    redo1 = i1 < last
    send1 = jnp.logical_and(redo1, g1 != g0)

    def patch(i, gst, yy):
        blk = out_stage[pl.ds(gst, 16), :].astype(f32)
        out_stage[pl.ds(gst, 16), :] = (blk + jnp.where(row16 == i - gst, yy, 0.0)).astype(bf16)

    @pl.when(redo0)
    def _():
        patch(i0, g0, y0)

    @pl.when(redo1)
    def _():
        patch(i1, g1, y1)

    @pl.when(redo0)
    def _():
        out_copy(g0, 16, SEM_P0).start()

    @pl.when(send1)
    def _():
        out_copy(g1, 16, SEM_P1).start()

    out_copy(last, 128, SEM_OUT2).wait()

    @pl.when(redo0)
    def _():
        out_copy(g0, 16, SEM_P0).wait()

    @pl.when(send1)
    def _():
        out_copy(g1, 16, SEM_P1).wait()


@jax.jit
def pallas_parallel_sum__memory_aug_recurrent_mem_tr__moe_arch_mod__prompt_kernel(
    A_x: jax.Array,
    A_mem0: jax.Array,
    A_Wq: jax.Array,
    A_Wk: jax.Array,
    A_Wv: jax.Array,
    A_Wo: jax.Array,
    A_seg_len: jax.Array,
    B_x: jax.Array,
    B_w_r: jax.Array,
    B_w_gate: jax.Array,
    B_w_up: jax.Array,
    B_w_down: jax.Array,
):
    del A_seg_len, B_x
    assert A_x.shape == (1, S, DM) and A_mem0.shape == (1, NMEM, DM)
    assert A_Wq.shape == (DM, H, DH) and A_Wo.shape == (H, DH, DM) and B_w_gate.shape == (DM, FF)
    hbm = pl.BlockSpec(memory_space=pl.ANY)
    vmem = pl.BlockSpec(memory_space=pltpu.VMEM)
    scratch = [
        pltpu.VMEM((S, DM), bf16),
        pltpu.VMEM((S, DM), f32),
        pltpu.VMEM((KT, S // 2, 128), u32),
        pltpu.VMEM((16, DM), f32),
        pltpu.VMEM((48 * DM, 128), u32),
        pltpu.VMEM((3 * H, DM // 2, 128), u32),
        pltpu.VMEM((KT, H * DH // 2, 128), u32),
    ]
    scratch += [pltpu.VMEM((24, RQ // 2, 128), u32)] * NG
    scratch += [pltpu.VMEM((8, RO // 2, 128), u32)] * NG
    scratch += [pltpu.VMEM((8, 16, 128), u32)] * NG
    scratch += [
        pltpu.VMEM((NMEM, DM), f32),
        pltpu.VMEM((16, 128), u32),
        pltpu.VMEM((L2, L2), f32),
        pltpu.VMEM((128 + TOK, 128), f32),
        pltpu.VMEM((S, DM), bf16),
        pltpu.SemaphoreType.DMA((NSEM,)),
    ]
    return pl.pallas_call(
        _kernel,
        out_shape=jax.ShapeDtypeStruct((1, S, DM), bf16),
        in_specs=[hbm, vmem, hbm, hbm, hbm, hbm, vmem, hbm, hbm, hbm],
        out_specs=hbm,
        scratch_shapes=scratch,
        compiler_params=pltpu.CompilerParams(vmem_limit_bytes=110 * 1024 * 1024,
                                             disable_bounds_checks=True),
    )(A_x, A_mem0, A_Wq, A_Wk, A_Wv, A_Wo.reshape(H * DH, DM), B_w_r, B_w_gate, B_w_up, B_w_down)
```
